```python
import jax
import jax.numpy as jnp

def _softmax(x, axis=-1):
    return jax.nn.softmax(x, axis=axis)
def _gelu(x):
    return jax.nn.gelu(x, approximate=True)
def _silu(x):
    return jax.nn.silu(x)
def _sigmoid(x):
    return jax.nn.sigmoid(x)
def _layernorm(x, axis=-1, eps=1e-5):
    m = jnp.mean(x, axis=axis, keepdims=True)
    v = jnp.var(x, axis=axis, keepdims=True)
    return (x - m) / jnp.sqrt(v + eps)
def _scatter_add(tgt, idx, src, axis=0):
    return tgt.at[idx].add(src)
def _segment_sum(src, seg, n):
    return jax.ops.segment_sum(src, seg, n)
class _Rng:
    def __init__(self, key):
        self._k = key
    def _next(self):
        self._k, sub = jax.random.split(self._k)
        return sub
    def normal(self, shape):
        return jax.random.normal(self._next(), shape, dtype=jnp.bfloat16)
    def randint(self, lo, hi, shape):
        return jax.random.randint(self._next(), shape, lo, hi, dtype=jnp.int32)
    def uniform(self, shape, lo=0.0, hi=1.0):
        return jax.random.uniform(self._next(), shape, jnp.bfloat16, lo, hi)
    def permutation(self, n):
        return jax.random.permutation(self._next(), n)


kernel_name = 'gated_mix__linear_kernel_hedgehog__moe_arch_mod__prompt'

def setup_inputs():
    _rng = _Rng(jax.random.key(int.from_bytes(__import__("os").urandom(4), "little")))
    _w = (lambda a: (lambda t: t.astype(jnp.bfloat16) if jnp.issubdtype(t.dtype, jnp.floating) else t)(jnp.asarray(a)))
    def _A_setup():
        B, S, D, H = 1, 2048, 1024, 32
        Dh = D // H
        return {
            "x": _w((lambda *s: _rng.normal(s) * 0.05)(B, S, D)),
            "wqkv": _w((lambda *s: _rng.normal(s) * 0.05)(D, 3 * D)),
            "w_phi": _w((lambda *s: _rng.normal(s) * 0.05)(H, Dh, Dh) * (Dh ** -0.5)),
            "wo": _w((lambda *s: _rng.normal(s) * 0.05)(D, D)),
        }
    _A_in = _A_setup()

    def _B_setup():
        B, S, D, F, C = 1, 2048, 1024, 3584, 1
        return {
            "x": _w((lambda *s: _rng.normal(s) * 0.05)(B, S, D)),
            "w_r": _w((lambda *s: _rng.normal(s) * 0.05)(D)),
            "w_gate": _w((lambda *s: _rng.normal(s) * 0.05)(D, F)),
            "w_up": _w((lambda *s: _rng.normal(s) * 0.05)(D, F)),
            "w_down": _w((lambda *s: _rng.normal(s) * 0.05)(F, D)),
        }
    _B_in = _B_setup()

    return {
        "A_x": _A_in["x"],
        "A_wqkv": _A_in["wqkv"],
        "A_w_phi": _A_in["w_phi"],
        "A_wo": _A_in["wo"],
        "B_x": _B_in["x"],
        "B_w_r": _B_in["w_r"],
        "B_w_gate": _B_in["w_gate"],
        "B_w_up": _B_in["w_up"],
        "B_w_down": _B_in["w_down"],
        "gate_w": _w((lambda *s: _rng.normal(s) * 0.05)(1024)),
    }

def reference(A_x, A_wqkv, A_w_phi, A_wo, B_x, B_w_r, B_w_gate, B_w_up, B_w_down, gate_w):
    def _A_ref(x, wqkv, w_phi, wo):
        B, S, D = x.shape
        H = 32; Dh = D // H
        qkv = (lambda x, *d: x.transpose(*d))((x @ wqkv).reshape(B, S, 3, H, Dh), 2, 0, 3, 1, 4)
        q, k, v = qkv[0], qkv[1], qkv[2]
        pq = jnp.einsum("bhsd,hdf->bhsf", q, w_phi)
        pk = jnp.einsum("bhsd,hdf->bhsf", k, w_phi)
        phi_q = jnp.concatenate([_softmax(pq, axis=-1), _softmax(-pq, axis=-1)], axis=-1)
        phi_k = jnp.concatenate([_softmax(pk, axis=-1), _softmax(-pk, axis=-1)], axis=-1)
        kv = jnp.einsum("bhsf,bhsd->bhfd", phi_k, v)
        z  = jnp.einsum("bhsf->bhf", phi_k)
        num = jnp.einsum("bhqf,bhfd->bhqd", phi_q, kv)
        den = jnp.einsum("bhqf,bhf->bhq", phi_q, z)[..., None] + 1e-6
        o = num / den
        return (lambda x, *d: x.transpose(*d))(o, 0, 2, 1, 3).reshape(B, S, D) @ wo

    def _B_ref(x, w_r, w_gate, w_up, w_down):
        B, S, D = x.shape
        C = 1
        r = x @ w_r
        idx = jnp.argsort(-r, axis=-1)[:, :C]
        idx_e = jnp.repeat(idx.reshape(B, C, 1), D, axis=2)
        x_sel = jnp.take_along_axis(x, idx_e, axis=1)
        g = _silu(x_sel @ w_gate)
        u = x_sel @ w_up
        y = (g * u) @ w_down
        r_sel = _sigmoid(jnp.take_along_axis(r, idx, axis=1))
        y = y * r_sel.reshape(B, C, 1)
        b_off = (jnp.arange(B) * S).reshape(B, 1)
        flat_idx = (idx + b_off).reshape(B * C)
        zero = (x * 0.0).reshape(B * S, D)
        upd = _scatter_add(zero, flat_idx, y.reshape(B * C, D), axis=0)
        return x + upd.reshape(B, S, D)

    x = A_x
    g = _sigmoid((x * gate_w).sum(-1, keepdims=True))
    a = _A_ref(x, A_wqkv, A_w_phi, A_wo)
    b = _B_ref(x, B_w_r, B_w_gate, B_w_up, B_w_down)
    return g * a + (1 - g) * b
```

```python
import jax
import jax.numpy as jnp
import numpy as np
from jax import lax
import jax.experimental.pallas as pl
import jax.experimental.pallas.tpu as pltpu

S, D, H, DH, F = 2048, 1024, 32, 32, 3584
T = 256
NC = S // T
NG = 8
FC = 512
NF = F // FC
f32, bf16 = jnp.float32, jnp.bfloat16
NT = (((1,), (1,)), ((), ()))


def _feat(p):
    outs = []
    for h in range(4):
        ph = p[h * DH:(h + 1) * DH]
        mx = jnp.max(ph, axis=0, keepdims=True)
        mn = jnp.min(ph, axis=0, keepdims=True)
        e1 = jnp.exp(ph - mx)
        e2 = jnp.exp(mn - ph)
        r1 = 1.0 / jnp.sum(e1, axis=0, keepdims=True)
        r2 = 1.0 / jnp.sum(e2, axis=0, keepdims=True)
        outs.append((e1 * r1).astype(bf16))
        outs.append((e2 * r2).astype(bf16))
    return outs


def _kernel(x_hbm, wqkv_hbm, wphi_hbm, wo_hbm, bx_hbm, wr_hbm, wg_hbm, wu_hbm, wd_hbm, gw_hbm,
            out_hbm,
            x_v, wqkv_v, wphi_v, wo_v, bx_v, wr_v, wg_v, wu_v, wd_v, gw_v,
            wt_v, phiq_v, acc_v, kvz_v, out_v, xcol_v, y_v, r_v, sm, sems, xsem, bsem, osem):
    def cp(src, dst, sem):
        return pltpu.make_async_copy(src, dst, sem)

    c_wphi = cp(wphi_hbm, wphi_v, sems.at[0])
    c_wqkv = cp(wqkv_hbm, wqkv_v, sems.at[1])
    c_wr = cp(wr_hbm, wr_v, sems.at[2])
    c_gw = cp(gw_hbm, gw_v, sems.at[3])
    c_wo = cp(wo_hbm, wo_v, sems.at[4])
    c_wg = cp(wg_hbm, wg_v, sems.at[5])
    c_wu = cp(wu_hbm, wu_v, sems.at[6])
    c_wd = cp(wd_hbm, wd_v, sems.at[7])
    c_x = lambda i: cp(x_hbm.at[pl.ds(i * T, T)], x_v.at[pl.ds(i * T, T)], xsem.at[i])
    c_b = lambda i: cp(bx_hbm.at[pl.ds(i * T, T)], bx_v.at[pl.ds(i * T, T)], bsem.at[i])
    c_o = lambda i: cp(out_v.at[pl.ds(i * T, T)], out_hbm.at[pl.ds(i * T, T)], osem.at[i])

    c_wphi.start(); c_wqkv.start(); c_wr.start(); c_gw.start()
    for i in range(NC):
        c_x(i).start()
    c_wo.start(); c_wg.start(); c_wu.start(); c_wd.start()

    c_wphi.wait(); c_wqkv.wait()
    row = lax.broadcasted_iota(jnp.int32, (128, 128), 0)
    col = lax.broadcasted_iota(jnp.int32, (128, 128), 1)
    diag = (row // DH) == (col // DH)
    rep = ((lax.broadcasted_iota(jnp.int32, (DH, 128), 1) % DH) == lax.broadcasted_iota(jnp.int32, (DH, 128), 0)).astype(bf16)
    for g in range(NG):
        w = wphi_v[g * 128:(g + 1) * 128, :]
        wt = jnp.dot(w, rep, preferred_element_type=f32)
        bd = jnp.where(diag, wt, 0.0)
        bdt = bd.T.astype(bf16)
        for j in range(2):
            wj = wqkv_v[:, j * D + g * 128: j * D + (g + 1) * 128]
            wt_v[g * 384 + j * 128: g * 384 + (j + 1) * 128, :] = lax.dot_general(
                bdt, wj, NT, preferred_element_type=f32).astype(bf16)
        wv = wqkv_v[:, 2 * D + g * 128: 2 * D + (g + 1) * 128]
        wt_v[g * 384 + 256: (g + 1) * 384, :] = wv.astype(f32).T.astype(bf16)

    acc_v[...] = jnp.zeros_like(acc_v)
    c_wr.wait(); c_gw.wait()
    ones = jnp.ones((16, T), bf16)

    def p1(i, carry):
        best, bidx = carry
        c_x(i).wait()
        t0 = pl.multiple_of(i * T, T)
        xc = x_v[pl.ds(t0, T), :]
        for g in range(NG):
            pt = lax.dot_general(wt_v[g * 384:(g + 1) * 384, :], xc, NT, preferred_element_type=f32)
            fq = _feat(pt[0:128])
            fk = _feat(pt[128:256])
            vt = pt[256:384].astype(bf16)
            for j in range(8):
                phiq_v[i, g * 256 + j * 32: g * 256 + (j + 1) * 32, :] = fq[j]
            for p in range(2):
                lhs = jnp.concatenate([vt[p * 64:(p + 1) * 64], ones], axis=0)
                rhs = jnp.concatenate(fk[4 * p:4 * p + 4], axis=0)
                acc_v[2 * g + p] += lax.dot_general(lhs, rhs, NT, preferred_element_type=f32)
        r = jnp.sum(x_v[pl.ds(t0, T), :].astype(f32) * wr_v[...].astype(f32), axis=1, keepdims=True)
        r = r.astype(bf16).astype(f32)
        m = jnp.max(r)
        ids = lax.broadcasted_iota(jnp.int32, (T, 1), 0) + i * T
        mi = jnp.min(jnp.where(r == m, ids, S - 1))
        better = m > best
        return jnp.where(better, m, best), jnp.where(better, mi, bidx)

    _, idx = lax.fori_loop(0, NC, p1, (jnp.float32(-jnp.inf), jnp.int32(0)))
    best = _

    r80 = lax.broadcasted_iota(jnp.int32, (80, 128), 0)
    c80 = lax.broadcasted_iota(jnp.int32, (80, 128), 1)
    rh = jnp.where(r80 < 64, r80 // 32, (r80 - 64) // 8)
    keep = rh == (c80 // 64)
    for p in range(2 * NG):
        kvz_v[p] = jnp.where(keep, acc_v[p], 0.0).astype(bf16)

    c_wo.wait(); c_wg.wait(); c_wu.wait(); c_wd.wait()
    base = pl.multiple_of((idx // 16) * 16, 16)
    tile = x_v[pl.ds(base, 16), :].astype(f32)
    sel = lax.broadcasted_iota(jnp.int32, (16, D), 0) == (idx - base)
    xs = jnp.sum(jnp.where(sel, tile, 0.0), axis=0, keepdims=True)
    for k in range(D // 128):
        xcol_v[k * 128:(k + 1) * 128, :] = jnp.broadcast_to(xs[:, k * 128:(k + 1) * 128], (128, 128)).T
    rs = jax.nn.sigmoid(jnp.full((1, 128), best, f32))[:, 0:1]
    y_v[...] = jnp.zeros_like(y_v)
    last = idx // T

    def p2(j, _):
        i = (last + 1 + j) % NC
        t0 = pl.multiple_of(i * T, T)
        ot = []
        for p in range(2 * NG):
            nd = jnp.dot(kvz_v[p], phiq_v[i, p * 128:(p + 1) * 128, :], preferred_element_type=f32)
            for a in range(2):
                rden = 1.0 / (nd[64 + 8 * a:72 + 8 * a] + 1e-6)
                o = nd[32 * a:32 * a + 32].reshape(4, 8, T) * rden[None]
                ot.append(o.reshape(32, T).astype(bf16))
        o = jnp.concatenate(ot, axis=0).T
        a = jnp.dot(o, wo_v[...], preferred_element_type=f32)
        gs = jnp.sum(x_v[pl.ds(t0, T), :].astype(f32) * gw_v[...].astype(f32), axis=1, keepdims=True)
        gate = jax.nn.sigmoid(gs)
        xb = x_v[pl.ds(t0, T), :].astype(f32)
        yrow = jnp.sum(y_v[...], axis=0, keepdims=True) * rs
        hit = (lax.broadcasted_iota(jnp.int32, (T, D), 0) + t0) == idx
        b = xb + (xb * 0.0 + jnp.where(hit, yrow, 0.0))
        out_v[pl.ds(t0, T), :] = (gate * a + (1.0 - gate) * b).astype(bf16)
        c_o(i).start()
        fj = jnp.minimum(j, NF - 1)
        f0 = pl.multiple_of(fj * FC, FC)
        xc = xcol_v[...]
        ynew = jnp.zeros((8, D), f32)
        for c in range(FC // 128):
            fs = pl.ds(f0 + c * 128, 128)
            gg = jnp.sum((wg_v[:, fs].astype(f32) * xc).reshape(D // 8, 8, 128), axis=0)
            uu = jnp.sum((wu_v[:, fs].astype(f32) * xc).reshape(D // 8, 8, 128), axis=0)
            gg = jnp.sum(gg, axis=0, keepdims=True)
            uu = jnp.sum(uu, axis=0, keepdims=True)
            hh = (gg * jax.nn.sigmoid(gg)) * uu
            hcol = jnp.broadcast_to(hh, (128, 128)).T
            wd = wd_v[fs, :].astype(f32)
            ynew = ynew + jnp.concatenate(
                [jnp.sum((wd[:, k * 128:(k + 1) * 128] * hcol).reshape(16, 8, 128), axis=0)
                 for k in range(D // 128)], axis=1)
        y_v[...] += jnp.where(j < NF, ynew, 0.0)
        return 0

    lax.fori_loop(0, NC, p2, 0)
    for i in range(NC):
        c_o(i).wait()


@jax.jit
def pallas_gated_mix__linear_kernel_hedgehog__moe_arch_mod__prompt_kernel(A_x, A_wqkv, A_w_phi, A_wo, B_x, B_w_r, B_w_gate, B_w_up, B_w_down, gate_w):
    anyspec = pl.BlockSpec(memory_space=pl.ANY)
    out = pl.pallas_call(
        _kernel,
        out_shape=jax.ShapeDtypeStruct((S, D), bf16),
        in_specs=[anyspec] * 10,
        out_specs=anyspec,
        scratch_shapes=[
            pltpu.VMEM((S, D), bf16), pltpu.VMEM((D, 3 * D), bf16), pltpu.VMEM((D, DH), bf16),
            pltpu.VMEM((D, D), bf16), pltpu.VMEM((S, D), bf16), pltpu.VMEM((1, D), bf16),
            pltpu.VMEM((D, F), bf16), pltpu.VMEM((D, F), bf16), pltpu.VMEM((F, D), bf16),
            pltpu.VMEM((1, D), bf16),
            pltpu.VMEM((3 * D, D), bf16), pltpu.VMEM((NC, 2 * D, T), bf16),
            pltpu.VMEM((2 * NG, 80, 128), f32), pltpu.VMEM((2 * NG, 80, 128), bf16),
            pltpu.VMEM((S, D), bf16), pltpu.VMEM((D, 128), f32), pltpu.VMEM((8, D), f32),
            pltpu.VMEM((S, 1), f32),
            pltpu.SMEM((4,), jnp.int32),
            pltpu.SemaphoreType.DMA((8,)), pltpu.SemaphoreType.DMA((NC,)),
            pltpu.SemaphoreType.DMA((NC,)), pltpu.SemaphoreType.DMA((NC,)),
        ],
        compiler_params=pltpu.CompilerParams(vmem_limit_bytes=110 * 2**20),
    )(A_x.reshape(S, D), A_wqkv, A_w_phi.reshape(D, DH), A_wo, B_x.reshape(S, D),
      B_w_r.reshape(1, D), B_w_gate, B_w_up, B_w_down, gate_w.reshape(1, D))
    return out.reshape(1, S, D)
```

```python
import jax
import jax.numpy as jnp
import numpy as np
from jax import lax
import jax.experimental.pallas as pl
import jax.experimental.pallas.tpu as pltpu

S, D, H, DH, F = 2048, 1024, 32, 32, 3584
T = 256
NC = S // T
NG = 8
FC = 512
NF = F // FC
FFN0 = 35
f32, bf16 = jnp.float32, jnp.bfloat16
NT = (((1,), (1,)), ((), ()))
LOG2E = 1.4426950408889634


def _rcp(x):
    r = pl.reciprocal(x, approx=True)
    return r * (2.0 - x * r)


def _feat(p):
    outs = []
    for h in range(4):
        ph = p[h * DH:(h + 1) * DH]
        mx = jnp.max(ph, axis=0, keepdims=True)
        mn = jnp.min(ph, axis=0, keepdims=True)
        e1 = jnp.exp2(ph - mx)
        e2 = jnp.exp2(mn - ph)
        r1 = _rcp(jnp.sum(e1, axis=0, keepdims=True))
        r2 = _rcp(jnp.sum(e2, axis=0, keepdims=True))
        outs.append(e1 * r1)
        outs.append(e2 * r2)
    return jnp.concatenate(outs, axis=0).astype(bf16)


def _kernel(x_hbm, wqkv_hbm, wphi_hbm, wo_hbm, wr_hbm, wg_hbm, wu_hbm, wd_hbm, gw_hbm,
            out_hbm,
            x_v, wraw_v, wphi_v, wo_v, wr_v, gw_v, wg_v, wu_v, wd_v,
            wq_v, wkv_v, phiq_v, acc_v, kvz_v, out_v, xcol_v, gate_v, bd_v, rg_v,
            sems):
    cp = pltpu.make_async_copy
    c_wphi = cp(wphi_hbm, wphi_v, sems.at[0])
    c_wr = cp(wr_hbm, wr_v, sems.at[1])
    c_gw = cp(gw_hbm, gw_v, sems.at[2])
    c_wo = [cp(wo_hbm.at[pl.ds(j * 256, 256)], wo_v.at[pl.ds(j * 256, 256)], sems.at[3 + j]) for j in range(4)]
    c_w = [[cp(wqkv_hbm.at[:, pl.ds(j * D + g * 128, 128)], wraw_v[j][g], sems.at[7 + j * NG + g])
            for g in range(NG)] for j in range(3)]
    c_x = [cp(x_hbm.at[pl.ds(i * T, T)], x_v[i], sems.at[31 + i]) for i in range(NC)]
    c_f = [[cp(wg_hbm.at[:, pl.ds(j * FC, FC)], wg_v[j], sems.at[39 + 3 * j]),
            cp(wu_hbm.at[:, pl.ds(j * FC, FC)], wu_v[j], sems.at[40 + 3 * j]),
            cp(wd_hbm.at[pl.ds(j * FC, FC)], wd_v[j], sems.at[41 + 3 * j])] for j in range(NF)]
    c_o = [cp(out_v[i], out_hbm.at[pl.ds(i * T, T)], sems.at[60 + i]) for i in range(NC)]

    c_wphi.start()
    c_w[1][0].start()
    c_x[0].start()
    c_w[2][0].start()
    for g in range(1, NG):
        c_w[1][g].start()
        c_w[2][g].start()
    c_wr.start(); c_gw.start()
    c_x[1].start()
    for g in range(NG):
        c_w[0][g].start()
    for i in range(2, NC):
        c_x[i].start()

    row = lax.broadcasted_iota(jnp.int32, (128, 128), 0)
    col = lax.broadcasted_iota(jnp.int32, (128, 128), 1)
    diag = (row // DH) == (col // DH)
    rep = ((lax.broadcasted_iota(jnp.int32, (DH, 128), 1) % DH)
           == lax.broadcasted_iota(jnp.int32, (DH, 128), 0)).astype(bf16)
    acc_v[...] = jnp.zeros_like(acc_v)
    c_wphi.wait()
    for g in range(NG):
        wt = jnp.dot(wphi_v[g * 128:(g + 1) * 128, :], rep, preferred_element_type=f32)
        bd_v[g] = jnp.where(diag, wt, 0.0).T.astype(bf16)

    def fold(j, g):
        c_w[j][g].wait()
        w = lax.dot_general(bd_v[g], wraw_v[j][g][...], NT, preferred_element_type=f32) * LOG2E
        if j == 0:
            wq_v[g][...] = w.astype(bf16)
        else:
            wkv_v[g][0:128, :] = w.astype(bf16)

    def prep_kv(g):
        fold(1, g)
        c_w[2][g].wait()
        wkv_v[g][128:256, :] = wraw_v[2][g][...].astype(f32).T.astype(bf16)

    ones = jnp.ones((16, T), bf16)

    def proj(w, i):
        return lax.dot_general(w, x_v[i][...], NT, preferred_element_type=f32)

    def soft_kv(pkv):
        fk = _feat(pkv[0:128])
        return fk, pkv[128:256].astype(bf16)

    def kv(g, fk, vt):
        for p in range(2):
            lhs = jnp.concatenate([vt[p * 64:(p + 1) * 64], ones], axis=0)
            acc_v[2 * g + p] += lax.dot_general(lhs, fk[p * 128:(p + 1) * 128], NT,
                                                preferred_element_type=f32)

    st = {}

    def tie(a, dep):
        if dep is None:
            return a
        r = 8 if a.dtype == f32 else 16
        blk = a[0:r, 0:128]
        if a.dtype == f32:
            blk = jnp.where(st["never"], dep, blk)
        else:
            blk = pltpu.bitcast(jnp.where(st["never"], dep, pltpu.bitcast(blk, f32)), bf16)
        top = jnp.concatenate([blk, a[0:r, 128:]], axis=1) if a.shape[1] > 128 else blk
        return jnp.concatenate([top, a[r:]], axis=0) if a.shape[0] > r else top

    def router(i, dep):
        best, bidx = st["best"], st["bidx"]
        side = None
        for b in range(T // 16):
            rows = slice(b * 16, (b + 1) * 16)
            ra = ga = None
            for k in range(D // 128):
                ks = slice(k * 128, (k + 1) * 128)
                xf = x_v[i][rows, ks].astype(f32)
                if b == 0 and k == 0:
                    xf = tie(xf, dep)
                pr, pg = xf * rg_v[0:16, ks], xf * rg_v[16:32, ks]
                ra, ga = (pr, pg) if k == 0 else (ra + pr, ga + pg)
            r = jnp.sum(ra, axis=1, keepdims=True).astype(bf16).astype(f32)
            gs = jnp.broadcast_to(jnp.sum(ga, axis=1, keepdims=True), (16, 128))
            gate_v[i, rows, :] = gs
            r = jnp.broadcast_to(r, (16, 128))
            for k in range(2):
                rk = r[k * 8:(k + 1) * 8]
                if best is None:
                    best, bidx = rk, jnp.zeros((8, 128), jnp.int32)
                else:
                    better = rk > best
                    best = jnp.where(better, rk, best)
                    bidx = jnp.where(better, i * T + b * 16 + k * 8, bidx)
            side = gs[0:8]
        st["best"], st["bidx"] = best, bidx
        return best + side

    def select():
        best, bidx = st["best"], st["bidx"]
        m = jnp.max(best, axis=0, keepdims=True)
        cand = jnp.where(best == m, bidx + lax.broadcasted_iota(jnp.int32, (8, 128), 0), S - 1)
        idxv = jnp.min(cand, axis=0, keepdims=True)
        idx = idxv[0, 0]
        st["idxv"] = idxv
        st["rs"] = jax.nn.sigmoid(m)
        base = pl.multiple_of(((idx % T) // 16) * 16, 16)
        tile = x_v[0][pl.ds(base, 16), :].astype(f32)
        for i in range(1, NC):
            tile = jnp.where(idx // T == i, x_v[i][pl.ds(base, 16), :].astype(f32), tile)
        sel = lax.broadcasted_iota(jnp.int32, (16, D), 0) == (idx % 16)
        xs = jnp.sum(jnp.where(sel, tile, 0.0), axis=0, keepdims=True)
        for k in range(D // 128):
            xcol_v[k * 128:(k + 1) * 128, :] = jnp.broadcast_to(xs[:, k * 128:(k + 1) * 128], (128, 128)).T
        st["y"] = [None] * (D // 128)

    def chain(w_ref, r0, nblk, cols, col_of, dep):
        acc = None
        for k in range(nblk):
            p = w_ref[r0 + k * 16:r0 + (k + 1) * 16, cols].astype(f32) * col_of(k)
            acc = tie(p[0:8], dep) if acc is None else acc + p[0:8]
            acc = acc + p[8:16]
        return acc

    def ffn_up(c, dep):
        j, cc = divmod(c, FC // 128)
        fs = slice(cc * 128, (cc + 1) * 128)
        xc = lambda k: xcol_v[k * 16:(k + 1) * 16, :]
        gg = chain(wg_v[j], 0, D // 16, fs, xc, dep)
        uu = chain(wu_v[j], 0, D // 16, fs, xc, gg)
        side = uu
        gg = jnp.sum(gg, axis=0, keepdims=True)
        uu = jnp.sum(uu, axis=0, keepdims=True)
        hh = (gg * jax.nn.sigmoid(gg)) * uu
        st["hcol"] = jnp.broadcast_to(hh, (128, 128)).T
        return side

    def ffn_down(c, dep):
        j, cc = divmod(c, FC // 128)
        hcol = st["hcol"]
        ys = st["y"]
        for n in range(D // 128):
            dep = chain(wd_v[j], cc * 128, 128 // 16, slice(n * 128, (n + 1) * 128),
                        lambda k: hcol[k * 16:(k + 1) * 16], dep)
            ys[n] = dep if ys[n] is None else ys[n] + dep
        return dep

    pend = None
    prep_kv(0)
    for g in range(NG):
        if g + 1 < NG:
            prep_kv(g + 1)
        else:
            fold(0, 0)
        if g == 0:
            c_x[0].wait()
        pkv = proj(wkv_v[g][...], 0)
        if pend is not None:
            kv(*pend)
        pend = (g,) + soft_kv(pkv)

    for j in range(NF):
        for d in c_f[j]:
            d.start()
    for d in c_wo:
        d.start()

    side = prev = None
    for i in range(1, NC):
        if i == 1:
            c_x[1].wait()
        if i == 2:
            for k in range(2, NC):
                c_x[k].wait()
            c_wr.wait(); c_gw.wait()
            st["wr"] = wr_v[...].reshape(1, D).astype(f32)
            rg_v[0:16, :] = jnp.broadcast_to(st["wr"], (16, D))
            rg_v[16:32, :] = jnp.broadcast_to(gw_v[...].reshape(1, D).astype(f32), (16, D))
            st["best"] = st["bidx"] = None
            st["never"] = jnp.broadcast_to((pltpu.bitcast(st["wr"][:, 0:128], jnp.int32) | 1) == 0, (8, 128))
        for g in range(NG):
            if i == 1 and g + 1 < NG:
                fold(0, g + 1)
            pt = proj(tie(jnp.concatenate([wq_v[g][...], wkv_v[g][...]], axis=0), side), i)
            slot = i * NG + g
            side = None
            if i == 2:
                side = router(g, prev)
            elif slot == 3 * NG:
                select()
            c = slot - FFN0
            if c in (0, 16):
                for j in range(c // 4, min(c // 4 + 4, NF)):
                    for d in c_f[j]:
                        d.wait()
            if 0 < c <= F // 128:
                side = ffn_down(c - 1, prev)
            if 0 <= c < F // 128:
                side = ffn_up(c, prev if side is None else side)
            kv(*pend)
            phiq_v[i][g * 256:(g + 1) * 256, :] = _feat(pt[0:128])
            pend = (g,) + soft_kv(pt[128:384])
            prev = pt[0:8, 0:128]

    for g2 in range(NG // 2):
        pq = proj(jnp.concatenate([wq_v[2 * g2][...], wq_v[2 * g2 + 1][...]], axis=0), 0)
        if g2 == 0:
            kv(*pend)
            r80 = lax.broadcasted_iota(jnp.int32, (80, 128), 0)
            c80 = lax.broadcasted_iota(jnp.int32, (80, 128), 1)
            keep = jnp.where(r80 < 64, r80 // 32, (r80 - 64) // 8) == (c80 // 64)
            for p in range(2 * NG):
                a = acc_v[p]
                kvz_v[p] = jnp.where(keep, jnp.concatenate([a[0:72], a[64:72]], axis=0), 0.0).astype(bf16)
        for a in range(2):
            g = 2 * g2 + a
            phiq_v[0][g * 256:(g + 1) * 256, :] = _feat(pq[a * 128:(a + 1) * 128])

    yrow = jnp.concatenate([jnp.sum(y, axis=0, keepdims=True) * st["rs"] for y in st["y"]], axis=1)
    for d in c_wo:
        d.wait()

    def attn(i):
        ot = []
        for p in range(2 * NG):
            nd = jnp.dot(kvz_v[p], phiq_v[i][p * 128:(p + 1) * 128, :], preferred_element_type=f32)
            for a in range(2):
                rden = 1.0 / (nd[64 + 8 * a:72 + 8 * a] + 1e-6)
                o = nd[32 * a:32 * a + 32].reshape(4, 8, T) * rden[None]
                ot.append(o.reshape(32, T))
        return jnp.concatenate(ot, axis=0).astype(bf16).T

    def finish(i, o):
        a = jnp.dot(o, wo_v[...], preferred_element_type=f32)
        gate = jax.nn.sigmoid(gate_v[i])
        hit = (lax.broadcasted_iota(jnp.int32, (T, 128), 0) + i * T) == st["idxv"]
        xb = x_v[i][...].astype(f32)
        for k in range(D // 128):
            ks = slice(k * 128, (k + 1) * 128)
            b = xb[:, ks] + (xb[:, ks] * 0.0 + jnp.where(hit, yrow[:, ks], 0.0))
            out_v[i][:, ks] = (gate * a[:, ks] + (1.0 - gate) * b).astype(bf16)
        c_o[i].start()

    order = list(range(1, NC)) + [0]
    o_prev = attn(order[0])
    for n, i in enumerate(order):
        o_next = attn(order[n + 1]) if n + 1 < NC else None
        finish(i, o_prev)
        o_prev = o_next
    for i in order:
        c_o[i].wait()


@jax.jit
def pallas_gated_mix__linear_kernel_hedgehog__moe_arch_mod__prompt_kernel(A_x, A_wqkv, A_w_phi, A_wo, B_x, B_w_r, B_w_gate, B_w_up, B_w_down, gate_w):
    anyspec = pl.BlockSpec(memory_space=pl.ANY)
    V = pltpu.VMEM
    out = pl.pallas_call(
        _kernel,
        out_shape=jax.ShapeDtypeStruct((S, D), bf16),
        in_specs=[anyspec] * 9,
        out_specs=anyspec,
        scratch_shapes=[
            [V((T, D), bf16) for _ in range(NC)],
            [[V((D, 128), bf16) for _ in range(NG)] for _ in range(3)],
            V((D, DH), bf16), V((D, D), bf16), V((D,), bf16), V((D,), bf16),
            [V((D, FC), bf16) for _ in range(NF)], [V((D, FC), bf16) for _ in range(NF)],
            [V((FC, D), bf16) for _ in range(NF)],
            [V((128, D), bf16) for _ in range(NG)], [V((256, D), bf16) for _ in range(NG)],
            [V((2 * D, T), bf16) for _ in range(NC)],
            V((2 * NG, 80, 128), f32), V((2 * NG, 80, 128), bf16),
            [V((T, D), bf16) for _ in range(NC)],
            V((D, 128), f32), V((NC, T, 128), f32), V((NG, 128, 128), bf16), V((32, D), f32),
            pltpu.SemaphoreType.DMA((68,)),
        ],
        compiler_params=pltpu.CompilerParams(vmem_limit_bytes=110 * 2**20),
    )(A_x.reshape(S, D), A_wqkv, A_w_phi.reshape(D, DH), A_wo,
      B_w_r, B_w_gate, B_w_up, B_w_down, gate_w)
    return out.reshape(1, S, D)
```

```python
import jax
import jax.numpy as jnp
import numpy as np
from jax import lax
import jax.experimental.pallas as pl
import jax.experimental.pallas.tpu as pltpu

S, D, H, DH, F = 2048, 1024, 32, 32, 3584
T = 256
NC = S // T
NG = 8
FC = 512
NF = F // FC
FFN0 = 35
f32, bf16, u32 = jnp.float32, jnp.bfloat16, jnp.uint32
NT = (((1,), (1,)), ((), ()))
LOG2E = 1.4426950408889634


def _ld(ref, r0, r1, cols=slice(None)):
    return pltpu.bitcast(ref[r0 // 2:r1 // 2, cols], bf16)


def _st(ref, r0, r1, cols, val):
    ref[r0 // 2:r1 // 2, cols] = pltpu.bitcast(val, u32)


ALL = slice(None)


def _rcp(x):
    r = pl.reciprocal(x, approx=True)
    return r * (2.0 - x * r)


def _feat(p):
    outs = []
    for h in range(4):
        ph = p[h * DH:(h + 1) * DH]
        mx = jnp.max(ph, axis=0, keepdims=True)
        mn = jnp.min(ph, axis=0, keepdims=True)
        e1 = jnp.exp2(ph - mx)
        e2 = jnp.exp2(mn - ph)
        r1 = _rcp(jnp.sum(e1, axis=0, keepdims=True))
        r2 = _rcp(jnp.sum(e2, axis=0, keepdims=True))
        outs.append(e1 * r1)
        outs.append(e2 * r2)
    return jnp.concatenate(outs, axis=0).astype(bf16)


def _kernel(x_hbm, wqkv_hbm, wphi_hbm, wo_hbm, wr_hbm, wg_hbm, wu_hbm, wd_hbm, gw_hbm,
            out_hbm,
            x_v, wraw_v, wphi_v, wo_v, wr_v, gw_v, wg_v, wu_v, wd_v,
            wq_v, wkv_v, phiq_v, acc_v, kvz_v, out_v, xcol_v, gate_v, bd_v, rg_v,
            sems):
    cp = pltpu.make_async_copy
    c_wphi = cp(wphi_hbm, wphi_v, sems.at[0])
    c_wr = cp(wr_hbm, wr_v, sems.at[1])
    c_gw = cp(gw_hbm, gw_v, sems.at[2])
    c_wo = [cp(wo_hbm.at[pl.ds(j * 256, 256)], wo_v.bitcast(bf16).at[pl.ds(j * 256, 256)], sems.at[3 + j]) for j in range(4)]
    c_w = [[cp(wqkv_hbm.at[:, pl.ds(j * D + g * 128, 128)], wraw_v[j][g].bitcast(bf16), sems.at[7 + j * NG + g])
            for g in range(NG)] for j in range(3)]
    c_x = [cp(x_hbm.at[pl.ds(i * T, T)], x_v[i].bitcast(bf16), sems.at[31 + i]) for i in range(NC)]
    c_f = [[cp(wg_hbm.at[:, pl.ds(j * FC, FC)], wg_v[j].bitcast(bf16), sems.at[39 + 3 * j]),
            cp(wu_hbm.at[:, pl.ds(j * FC, FC)], wu_v[j].bitcast(bf16), sems.at[40 + 3 * j]),
            cp(wd_hbm.at[pl.ds(j * FC, FC)], wd_v[j].bitcast(bf16), sems.at[41 + 3 * j])] for j in range(NF)]
    c_o = [[cp(out_v[i].bitcast(bf16), out_hbm.at[pl.ds(i * T, T)], sems.at[60 + i])] for i in range(NC)]
    c_o[0] = [cp(out_v[0].bitcast(bf16).at[:, pl.ds(c * 256, 256)], out_hbm.at[pl.ds(0, T), pl.ds(c * 256, 256)],
                 sems.at[68 + c]) for c in range(4)]

    c_wphi.start()
    c_w[1][0].start()
    c_x[0].start()
    c_w[2][0].start()
    for g in range(1, NG):
        c_w[1][g].start()
        c_w[2][g].start()
    c_wr.start(); c_gw.start()
    c_x[1].start()
    for g in range(NG):
        c_w[0][g].start()
    for i in range(2, NC):
        c_x[i].start()

    row = lax.broadcasted_iota(jnp.int32, (128, 128), 0)
    col = lax.broadcasted_iota(jnp.int32, (128, 128), 1)
    diag = (row // DH) == (col // DH)
    rep = ((lax.broadcasted_iota(jnp.int32, (DH, 128), 1) % DH)
           == lax.broadcasted_iota(jnp.int32, (DH, 128), 0)).astype(bf16)
    acc_v[...] = jnp.zeros_like(acc_v)
    c_wphi.wait()
    for g in range(NG):
        wt = jnp.dot(wphi_v[g * 128:(g + 1) * 128, :], rep, preferred_element_type=f32)
        _st(bd_v, g * 128, (g + 1) * 128, ALL, jnp.where(diag, wt, 0.0).T.astype(bf16))

    def fold(j, g):
        w = lax.dot_general(_ld(bd_v, g * 128, (g + 1) * 128), _ld(wraw_v[j][g], 0, D), NT, preferred_element_type=f32) * LOG2E
        if j == 0:
            wq_v[g][...] = w.astype(bf16)
        else:
            wkv_v[g][0:128, :] = w.astype(bf16)

    def prep_kv(g):
        fold(1, g)
        wkv_v[g][128:256, :] = _ld(wraw_v[2][g], 0, D).T

    ones = jnp.ones((16, T), bf16)

    def proj(w, i):
        return lax.dot_general(w, _ld(x_v[i], 0, T), NT, preferred_element_type=f32)

    def soft_kv(pkv):
        fk = _feat(pkv[0:128])
        return fk, pkv[128:256].astype(bf16)

    def kv(g, fk, vt):
        for p in range(2):
            lhs = jnp.concatenate([vt[p * 64:(p + 1) * 64], ones], axis=0)
            acc_v[2 * g + p] += lax.dot_general(lhs, fk[p * 128:(p + 1) * 128], NT,
                                                preferred_element_type=f32)

    st = {}

    def tie(a, dep):
        if dep is None:
            return a
        r = 8 if a.dtype == f32 else 16
        blk = a[0:r, 0:128]
        if a.dtype == f32:
            blk = jnp.where(st["never"], dep, blk)
        else:
            blk = pltpu.bitcast(jnp.where(st["never"], dep, pltpu.bitcast(blk, f32)), bf16)
        top = jnp.concatenate([blk, a[0:r, 128:]], axis=1) if a.shape[1] > 128 else blk
        return jnp.concatenate([top, a[r:]], axis=0) if a.shape[0] > r else top

    def router(i, dep):
        best, bidx = st["best"], st["bidx"]
        side = None
        for b in range(T // 16):
            rows = slice(b * 16, (b + 1) * 16)
            xf = [_ld(x_v[i], b * 16, (b + 1) * 16, slice(k * 128, (k + 1) * 128)).astype(f32)
                  for k in range(D // 128)]
            acc = []
            for w in range(2):
                for hf in range(2):
                    a = None
                    for k in range(D // 128):
                        p = xf[k][hf * 8:(hf + 1) * 8] * rg_v[w * 8:(w + 1) * 8, k * 128:(k + 1) * 128]
                        a = tie(p, dep) if k == 0 else a + p
                    acc.append(a)
                    dep = a
            ra, ga = jnp.concatenate(acc[0:2], axis=0), jnp.concatenate(acc[2:4], axis=0)
            r = jnp.sum(ra, axis=1, keepdims=True).astype(bf16).astype(f32)
            gs = jnp.broadcast_to(jnp.sum(ga, axis=1, keepdims=True), (16, 128))
            gate_v[i, rows, :] = gs
            r = jnp.broadcast_to(r, (16, 128))
            for k in range(2):
                rk = r[k * 8:(k + 1) * 8]
                if best is None:
                    best, bidx = rk, jnp.zeros((8, 128), jnp.int32)
                else:
                    better = rk > best
                    best = jnp.where(better, rk, best)
                    bidx = jnp.where(better, i * T + b * 16 + k * 8, bidx)
        st["best"], st["bidx"] = best, bidx
        return dep

    def select():
        best, bidx = st["best"], st["bidx"]
        m = jnp.max(best, axis=0, keepdims=True)
        cand = jnp.where(best == m, bidx + lax.broadcasted_iota(jnp.int32, (8, 128), 0), S - 1)
        idxv = jnp.min(cand, axis=0, keepdims=True)
        idx = idxv[0, 0]
        st["idxv"] = idxv
        st["rs"] = jax.nn.sigmoid(m)
        base = pl.multiple_of(((idx % T) // 16) * 8, 8)
        tile = x_v[0][pl.ds(base, 8), :]
        for i in range(1, NC):
            tile = jnp.where(idx // T == i, x_v[i][pl.ds(base, 8), :], tile)
        tile = pltpu.bitcast(tile, bf16).astype(f32)
        sel = lax.broadcasted_iota(jnp.int32, (16, D), 0) == (idx % 16)
        xs = jnp.sum(jnp.where(sel, tile, 0.0), axis=0, keepdims=True)
        for k in range(D // 128):
            xcol_v[k * 128:(k + 1) * 128, :] = jnp.broadcast_to(xs[:, k * 128:(k + 1) * 128], (128, 128)).T
        st["y"] = [None] * (D // 128)

    def chain(w_ref, r0, nblk, cols, col_of, dep):
        acc = None
        for k in range(nblk):
            p = _ld(w_ref, r0 + k * 16, r0 + (k + 1) * 16, cols).astype(f32) * col_of(k)
            acc = tie(p[0:8], dep) if acc is None else acc + p[0:8]
            acc = acc + p[8:16]
        return acc

    def ffn_up(c, dep):
        j, cc = divmod(c, FC // 128)
        fs = slice(cc * 128, (cc + 1) * 128)
        xc = lambda k: xcol_v[k * 16:(k + 1) * 16, :]
        gg = chain(wg_v[j], 0, D // 16, fs, xc, dep)
        uu = chain(wu_v[j], 0, D // 16, fs, xc, gg)
        side = uu
        gg = jnp.sum(gg, axis=0, keepdims=True)
        uu = jnp.sum(uu, axis=0, keepdims=True)
        hh = (gg * jax.nn.sigmoid(gg)) * uu
        st["hcol"] = jnp.broadcast_to(hh, (128, 128)).T
        return side

    def ffn_down(c, dep):
        j, cc = divmod(c, FC // 128)
        hcol = st["hcol"]
        ys = st["y"]
        for n in range(D // 128):
            dep = chain(wd_v[j], cc * 128, 128 // 16, slice(n * 128, (n + 1) * 128),
                        lambda k: hcol[k * 16:(k + 1) * 16], dep)
            ys[n] = dep if ys[n] is None else ys[n] + dep
        return dep

    def wait_kv(gs):
        for g in gs:
            c_w[1][g].wait()
            c_w[2][g].wait()
        for g in gs:
            prep_kv(g)

    pend = None
    c_x[0].wait()
    wait_kv([0])
    nxt = {0: [1], 1: [2, 3], 3: [4, 5], 5: [6, 7]}
    for g in range(NG):
        pkv = proj(wkv_v[g][...], 0)
        if g in nxt:
            wait_kv(nxt[g])
        if g == NG - 1:
            c_x[1].wait()
            for k in range(4):
                c_w[0][k].wait()
            fold(0, 0)
        if pend is not None:
            kv(*pend)
        pend = (g,) + soft_kv(pkv)

    for j in range(NF):
        for d in c_f[j]:
            d.start()
    for d in c_wo:
        d.start()

    side = prev = None
    for i in range(1, NC):
        for g in range(NG):
            if i == 1 and g + 1 < NG:
                fold(0, g + 1)
            pt = proj(tie(jnp.concatenate([wq_v[g][...], wkv_v[g][...]], axis=0), side), i)
            slot = i * NG + g
            if slot == NG + 1:
                for k in range(4, NG):
                    c_w[0][k].wait()
            if slot == 2 * NG - 1:
                for k in range(2, NC):
                    c_x[k].wait()
                c_wr.wait(); c_gw.wait()
                st["wr"] = wr_v[...].reshape(1, D).astype(f32)
                rg_v[0:8, :] = jnp.broadcast_to(st["wr"], (8, D))
                rg_v[8:16, :] = jnp.broadcast_to(gw_v[...].reshape(1, D).astype(f32), (8, D))
                st["best"] = st["bidx"] = None
                st["never"] = jnp.broadcast_to((pltpu.bitcast(st["wr"][:, 0:128], jnp.int32) | 1) == 0, (8, 128))
            side = None
            if i == 2:
                side = router(g, prev)
            elif slot == 3 * NG:
                select()
            c = slot - FFN0
            if c in (-1, 15):
                for j in range((c + 1) // 4, min((c + 1) // 4 + 4, NF)):
                    for d in c_f[j]:
                        d.wait()
            if 0 < c <= F // 128:
                side = ffn_down(c - 1, prev)
            if 0 <= c < F // 128:
                side = ffn_up(c, prev if side is None else side)
            kv(*pend)
            _st(phiq_v[i], g * 256, (g + 1) * 256, ALL, _feat(pt[0:128]))
            pend = (g,) + soft_kv(pt[128:384])
            prev = pt[0:8, 0:128]

    for g2 in range(NG // 2):
        pq = proj(jnp.concatenate([wq_v[2 * g2][...], wq_v[2 * g2 + 1][...]], axis=0), 0)
        if g2 == 0:
            kv(*pend)
            r80 = lax.broadcasted_iota(jnp.int32, (80, 128), 0)
            c80 = lax.broadcasted_iota(jnp.int32, (80, 128), 1)
            keep = jnp.where(r80 < 64, r80 // 32, (r80 - 64) // 8) == (c80 // 64)
            for p in range(2 * NG):
                a = acc_v[p]
                _st(kvz_v, p * 80, (p + 1) * 80, ALL, jnp.where(keep, jnp.concatenate([a[0:72], a[64:72]], axis=0), 0.0).astype(bf16))
        for a in range(2):
            g = 2 * g2 + a
            _st(phiq_v[0], g * 256, (g + 1) * 256, ALL, _feat(pq[a * 128:(a + 1) * 128]))

    yrow = jnp.concatenate([jnp.sum(y, axis=0, keepdims=True) * st["rs"] for y in st["y"]], axis=1)
    for d in c_wo:
        d.wait()

    def attn(i):
        ot = []
        for p in range(2 * NG):
            nd = jnp.dot(_ld(kvz_v, p * 80, (p + 1) * 80), _ld(phiq_v[i], p * 128, (p + 1) * 128), preferred_element_type=f32)
            for a in range(2):
                rden = 1.0 / (nd[64 + 8 * a:72 + 8 * a] + 1e-6)
                o = nd[32 * a:32 * a + 32].reshape(4, 8, T) * rden[None]
                ot.append(o.reshape(32, T))
        return jnp.concatenate(ot, axis=0).astype(bf16).T

    def finish(i, o, nsplit):
        gate = jax.nn.sigmoid(gate_v[i])
        omg = 1.0 - gate
        hit = (lax.broadcasted_iota(jnp.int32, (T, 128), 0) + i * T) == st["idxv"]
        w = D // nsplit
        for c in range(nsplit):
            a = jnp.dot(o, _ld(wo_v, 0, D, slice(c * w, (c + 1) * w)), preferred_element_type=f32)
            for k in range(w // 128):
                ks = slice(c * w + k * 128, c * w + (k + 1) * 128)
                xb = _ld(x_v[i], 0, T, ks).astype(f32)
                b = xb + (xb * 0.0 + jnp.where(hit, yrow[:, ks], 0.0))
                _st(out_v[i], 0, T, ks, (gate * a[:, k * 128:(k + 1) * 128] + omg * b).astype(bf16))
            c_o[i][c].start()

    order = list(range(1, NC)) + [0]
    o_prev = attn(order[0])
    for n, i in enumerate(order):
        o_next = attn(order[n + 1]) if n + 1 < NC else None
        finish(i, o_prev, len(c_o[i]))
        o_prev = o_next
    for i in order:
        for d in c_o[i]:
            d.wait()


@jax.jit
def pallas_gated_mix__linear_kernel_hedgehog__moe_arch_mod__prompt_kernel(A_x, A_wqkv, A_w_phi, A_wo, B_x, B_w_r, B_w_gate, B_w_up, B_w_down, gate_w):
    anyspec = pl.BlockSpec(memory_space=pl.ANY)
    V = pltpu.VMEM
    P = lambda r, c: V((r // 2, c), u32)
    out = pl.pallas_call(
        _kernel,
        out_shape=jax.ShapeDtypeStruct((S, D), bf16),
        in_specs=[anyspec] * 9,
        out_specs=anyspec,
        scratch_shapes=[
            [P(T, D) for _ in range(NC)],
            [[P(D, 128) for _ in range(NG)] for _ in range(3)],
            V((D, DH), bf16), P(D, D), V((D,), bf16), V((D,), bf16),
            [P(D, FC) for _ in range(NF)], [P(D, FC) for _ in range(NF)],
            [P(FC, D) for _ in range(NF)],
            [V((128, D), bf16) for _ in range(NG)], [V((256, D), bf16) for _ in range(NG)],
            [P(2 * D, T) for _ in range(NC)],
            V((2 * NG, 80, 128), f32), P(2 * NG * 80, 128),
            [P(T, D) for _ in range(NC)],
            V((D, 128), f32), V((NC, T, 128), f32), P(NG * 128, 128), V((16, D), f32),
            pltpu.SemaphoreType.DMA((72,)),
        ],
        compiler_params=pltpu.CompilerParams(vmem_limit_bytes=110 * 2**20),
    )(A_x.reshape(S, D), A_wqkv, A_w_phi.reshape(D, DH), A_wo,
      B_w_r, B_w_gate, B_w_up, B_w_down, gate_w)
    return out.reshape(1, S, D)
```

```python
import jax
import jax.numpy as jnp
import numpy as np
from jax import lax
import jax.experimental.pallas as pl
import jax.experimental.pallas.tpu as pltpu

S, D, H, DH, F = 2048, 1024, 32, 32, 3584
T = 256
NC = S // T
NG = 8
NP = NG // 2
HD = D // 2
FC = 512
NF = F // FC
NB = F // 128
FFN0 = 31
FFN_WAIT = {30: (0, 1), 38: (2, 3), 46: (4, 5), 54: (6,)}
f32, bf16, u32 = jnp.float32, jnp.bfloat16, jnp.uint32
NT = (((1,), (1,)), ((), ()))
LOG2E = 1.4426950408889634
ALL = slice(None)


def _ld(ref, r0, r1, cols=ALL):
    return pltpu.bitcast(ref[r0 // 2:r1 // 2, cols], bf16)


def _st(ref, r0, r1, cols, val):
    ref[r0 // 2:r1 // 2, cols] = pltpu.bitcast(val, u32)


def _rcp(x):
    r = pl.reciprocal(x, approx=True)
    return r * (2.0 - x * r)


def _feat(p):
    outs = []
    for h in range(4):
        ph = p[h * DH:(h + 1) * DH]
        mx = jnp.max(ph, axis=0, keepdims=True)
        mn = jnp.min(ph, axis=0, keepdims=True)
        e1 = jnp.exp2(ph - mx)
        e2 = jnp.exp2(mn - ph)
        r1 = _rcp(jnp.sum(e1, axis=0, keepdims=True))
        r2 = _rcp(jnp.sum(e2, axis=0, keepdims=True))
        outs.append(e1 * r1)
        outs.append(e2 * r2)
    return jnp.concatenate(outs, axis=0).astype(bf16)


def _left(a11, a12, a21, a22):
    return (a11 + a22, a21 + a22, a11, a22, a11 + a12, a21 - a11, a12 - a22)


def _right(k, b11, b12, b21, b22):
    if k == 1:
        return b11()
    if k == 4:
        return b22()
    p, q, sub = {0: (b11, b22, False), 2: (b12, b22, True), 3: (b21, b11, True),
                 5: (b11, b12, False), 6: (b21, b22, False)}[k]
    p, q = p().astype(f32), q().astype(f32)
    return (p - q if sub else p + q).astype(bf16)


def _kernel(x_hbm, wqkv_hbm, wphi_hbm, wo_hbm, wr_hbm, wg_hbm, wu_hbm, wd_hbm, gw_hbm,
            out_hbm,
            x_v, wraw_v, wphi_v, wo_v, wr_v, gw_v, wg_v, wu_v, wd_v,
            sq_v, skv_v, xt_v, wot_v, phiq_v, acc_v, kvz_v, out_v, xcol_v, gate_v, bd_v, rg_v,
            sems):
    cp = pltpu.make_async_copy
    c_wphi = cp(wphi_hbm, wphi_v, sems.at[0])
    c_wr = cp(wr_hbm, wr_v, sems.at[1])
    c_gw = cp(gw_hbm, gw_v, sems.at[2])
    c_wo = cp(wo_hbm, wo_v.bitcast(bf16), sems.at[3])
    c_w = [[cp(wqkv_hbm.at[:, pl.ds(j * D + g * 128, 128)], wraw_v[j][g].bitcast(bf16), sems.at[4 + j * NG + g])
            for g in range(NG)] for j in range(3)]
    c_x = [cp(x_hbm.at[pl.ds(i * T, T)], x_v[i].bitcast(bf16), sems.at[28 + i]) for i in range(NC)]
    c_f = [[cp(wg_hbm.at[:, pl.ds(j * FC, FC)], wg_v[j].bitcast(bf16), sems.at[36 + 3 * j]),
            cp(wu_hbm.at[:, pl.ds(j * FC, FC)], wu_v[j].bitcast(bf16), sems.at[37 + 3 * j]),
            cp(wd_hbm.at[pl.ds(j * FC, FC)], wd_v[j].bitcast(bf16), sems.at[38 + 3 * j])] for j in range(NF)]
    c_o = [cp(out_v[i].bitcast(bf16), out_hbm.at[pl.ds(i * T, T)], sems.at[57 + i]) for i in range(NC)]

    c_wphi.start()
    for g in range(NG):
        c_w[1][g].start()
        c_w[2][g].start()
        if g == 1:
            c_x[0].start()
    c_wr.start(); c_gw.start()
    c_x[1].start()
    for g in range(NG):
        c_w[0][g].start()
    for i in range(2, NC):
        c_x[i].start()

    row = lax.broadcasted_iota(jnp.int32, (128, 128), 0)
    col = lax.broadcasted_iota(jnp.int32, (128, 128), 1)
    diag = (row // DH) == (col // DH)
    rep = ((lax.broadcasted_iota(jnp.int32, (DH, 128), 1) % DH)
           == lax.broadcasted_iota(jnp.int32, (DH, 128), 0)).astype(bf16)
    acc_v[...] = jnp.zeros_like(acc_v)
    c_wphi.wait()
    for g in range(NG):
        wt = jnp.dot(wphi_v[g * 128:(g + 1) * 128, :], rep, preferred_element_type=f32)
        _st(bd_v, g * 128, (g + 1) * 128, ALL, jnp.where(diag, wt, 0.0).T.astype(bf16))

    def prep(j, pp):
        w = []
        for g in (2 * pp, 2 * pp + 1):
            raw = _ld(wraw_v[j][g], 0, D)
            if j < 2:
                w.append(lax.dot_general(_ld(bd_v, g * 128, (g + 1) * 128), raw, NT,
                                         preferred_element_type=f32) * LOG2E)
            else:
                w.append(raw.T.astype(f32))
        dst, r0 = (sq_v, 0) if j == 0 else (skv_v, (j - 1) * 128)
        for k, s in enumerate(_left(w[0][:, :HD], w[0][:, HD:], w[1][:, :HD], w[1][:, HD:])):
            _st(dst[pp][k], r0, r0 + 128, ALL, s.astype(bf16))

    ones = jnp.ones((16, T), f32)
    st = {"side": None, "prev": None}

    def tie(a, dep):
        if dep is None:
            return a
        if a.dtype == f32:
            return jnp.where(st["never"], dep, a)
        blk = pltpu.bitcast(jnp.where(st["never"], dep, pltpu.bitcast(a[0:16, 0:128], f32)), bf16)
        return jnp.concatenate([jnp.concatenate([blk, a[0:16, 128:]], axis=1), a[16:]], axis=0)

    def xright(i, k, fresh):
        blk = lambda r, c: (lambda: _ld(x_v[i], r * 128, (r + 1) * 128, slice(c * HD, (c + 1) * HD)))
        if k in (1, 4) or fresh:
            val = _right(k, blk(0, 0), blk(1, 0), blk(0, 1), blk(1, 1))
            if k not in (1, 4):
                _st(xt_v[i], k * 128, (k + 1) * 128, ALL, val)
            return val
        return _ld(xt_v[i], k * 128, (k + 1) * 128)

    def project(lhs, i, fresh, use, mid, hook):
        def m(k, tied=False):
            w = lhs(k)
            if tied:
                w = tie(w, st["side"])
                st["side"] = None
            out = lax.dot_general(w, xright(i, k, fresh), NT, preferred_element_type=f32)
            return out
        m5 = m(4, True)
        m3 = m(2)
        use(0, 1, m3 + m5)
        mid()
        m2 = m(1)
        hook(0)
        st["prev"] = m2[0:8]
        m4 = m(3, True)
        use(1, 0, m2 + m4)
        m1 = m(0)
        c11 = m1 + m4 - m5
        c22 = m1 - m2 + m3
        use(0, 0, c11 + m(6))
        m6 = m(5)
        hook(1)
        st["prev"] = m6[0:8]
        use(1, 1, c22 + m6)

    pend = []

    def kv_flush():
        for g, fk, vt in pend:
            fk = jnp.concatenate(fk, axis=1)
            vt = jnp.concatenate(vt, axis=1)
            for p in range(2):
                lhs = jnp.concatenate([vt[p * 64:(p + 1) * 64], ones], axis=0).astype(bf16)
                acc_v[2 * g + p] += lax.dot_general(lhs, fk[p * 128:(p + 1) * 128], NT,
                                                    preferred_element_type=f32)
        pend.clear()

    def router(i, dep):
        best, bidx = st["best"], st["bidx"]
        for b in range(T // 16):
            rows = slice(b * 16, (b + 1) * 16)
            xf = [_ld(x_v[i], b * 16, (b + 1) * 16, slice(k * 128, (k + 1) * 128)).astype(f32)
                  for k in range(D // 128)]
            acc = []
            for w in range(2):
                for hf in range(2):
                    a = None
                    for k in range(D // 128):
                        p = xf[k][hf * 8:(hf + 1) * 8] * rg_v[w * 8:(w + 1) * 8, k * 128:(k + 1) * 128]
                        a = tie(p, dep) if k == 0 else a + p
                    acc.append(a)
                    dep = a
            ra, ga = jnp.concatenate(acc[0:2], axis=0), jnp.concatenate(acc[2:4], axis=0)
            r = jnp.sum(ra, axis=1, keepdims=True).astype(bf16).astype(f32)
            gate_v[i, rows, :] = jnp.broadcast_to(jnp.sum(ga, axis=1, keepdims=True), (16, 128))
            r = jnp.broadcast_to(r, (16, 128))
            for k in range(2):
                rk = r[k * 8:(k + 1) * 8]
                if best is None:
                    best, bidx = rk, jnp.zeros((8, 128), jnp.int32)
                else:
                    better = rk > best
                    best = jnp.where(better, rk, best)
                    bidx = jnp.where(better, i * T + b * 16 + k * 8, bidx)
        st["best"], st["bidx"] = best, bidx
        return dep

    def select():
        best, bidx = st["best"], st["bidx"]
        m = jnp.max(best, axis=0, keepdims=True)
        cand = jnp.where(best == m, bidx + lax.broadcasted_iota(jnp.int32, (8, 128), 0), S - 1)
        idxv = jnp.min(cand, axis=0, keepdims=True)
        idx = idxv[0, 0]
        st["idxv"] = idxv
        st["rs"] = jax.nn.sigmoid(m)
        base = pl.multiple_of(((idx % T) // 16) * 8, 8)
        tile = x_v[0][pl.ds(base, 8), :]
        for i in range(1, NC):
            tile = jnp.where(idx // T == i, x_v[i][pl.ds(base, 8), :], tile)
        tile = pltpu.bitcast(tile, bf16).astype(f32)
        sel = lax.broadcasted_iota(jnp.int32, (16, D), 0) == (idx % 16)
        xs = jnp.sum(jnp.where(sel, tile, 0.0), axis=0, keepdims=True)
        for k in range(D // 128):
            xcol_v[k * 128:(k + 1) * 128, :] = jnp.broadcast_to(xs[:, k * 128:(k + 1) * 128], (128, 128)).T
        st["y"] = [None] * (D // 128)

    def chain(w_ref, r0, nblk, cols, col_of, dep):
        acc = None
        for k in range(nblk):
            p = _ld(w_ref, r0 + k * 16, r0 + (k + 1) * 16, cols).astype(f32) * col_of(k)
            acc = tie(p[0:8], dep) if acc is None else acc + p[0:8]
            acc = acc + p[8:16]
        return acc

    def ffn_up(c, dep):
        j, cc = divmod(c, FC // 128)
        fs = slice(cc * 128, (cc + 1) * 128)
        xc = lambda k: xcol_v[k * 16:(k + 1) * 16, :]
        gg = chain(wg_v[j], 0, D // 16, fs, xc, dep)
        uu = chain(wu_v[j], 0, D // 16, fs, xc, gg)
        side = uu
        gg = jnp.sum(gg, axis=0, keepdims=True)
        uu = jnp.sum(uu, axis=0, keepdims=True)
        hh = (gg * jax.nn.sigmoid(gg)) * uu
        st["hcol"] = jnp.broadcast_to(hh, (128, 128)).T
        return side

    def ffn_down(c, dep):
        j, cc = divmod(c, FC // 128)
        hcol = st["hcol"]
        ys = st["y"]
        for n in range(D // 128):
            dep = chain(wd_v[j], cc * 128, 128 // 16, slice(n * 128, (n + 1) * 128),
                        lambda k: hcol[k * 16:(k + 1) * 16], dep)
            ys[n] = dep if ys[n] is None else ys[n] + dep
        return dep

    def wo_right(k):
        blk = lambda r, c: (lambda: _ld(wo_v, r * HD, (r + 1) * HD, slice(c * HD, (c + 1) * HD)))
        return _right(k, blk(0, 0), blk(0, 1), blk(1, 0), blk(1, 1))

    def side_work(hs):
        prev, side = st["prev"], None
        if 24 <= hs < 32:
            side = router(hs - 24, prev)
            if hs == 31:
                select()
        c = hs - FFN0 - 1
        if 0 < c <= NB:
            side = ffn_down(c - 1, prev)
        if 0 <= c < NB:
            side = ffn_up(c, prev if side is None else side)
        st["side"] = side
        if hs == 9:
            for g in range(4, NG):
                c_w[0][g].wait()
            c_x[2].wait()
        if hs == 22:
            for k in range(3, NC):
                c_x[k].wait()
            c_wr.wait(); c_gw.wait()
            wr = wr_v[...].reshape(1, D).astype(f32)
            rg_v[0:8, :] = jnp.broadcast_to(wr, (8, D))
            rg_v[8:16, :] = jnp.broadcast_to(gw_v[...].reshape(1, D).astype(f32), (8, D))
            st["best"] = st["bidx"] = None
            st["never"] = jnp.broadcast_to((pltpu.bitcast(wr[:, 0:128], jnp.int32) | 1) == 0, (8, 128))
        for j in FFN_WAIT.get(hs, ()):
            for d in c_f[j]:
                d.wait()
            if j == NF - 1:
                c_wo.wait()
        if 59 <= hs < 64:
            k = (0, 2, 3, 5, 6)[hs - 59]
            _st(wot_v, k * HD, (k + 1) * HD, ALL, wo_right(k))

    def wait_kv(pp):
        for g in (2 * pp, 2 * pp + 1):
            c_w[1][g].wait()
            c_w[2][g].wait()

    wait_kv(0)
    prep(1, 0); prep(2, 0)
    c_x[0].wait()
    for pp in range(NP):
        new = [(2 * pp + a, [None, None], [None, None]) for a in range(2)]

        def use(a, t, c, new=new):
            new[a][1][t] = _feat(c[0:128])
            new[a][2][t] = c[128:256]

        def hook(h, pp=pp):
            if h == 1 and pp + 1 < NP:
                wait_kv(pp + 1)
                prep(1, pp + 1); prep(2, pp + 1)
            elif h == 1:
                c_x[1].wait()
                for g in range(4):
                    c_w[0][g].wait()
                prep(0, 0)

        project(lambda k, pp=pp: _ld(skv_v[pp][k], 0, 256), 0, pp == 0, use, kv_flush, hook)
        pend.extend(new)

    for j in range(NF):
        for d in c_f[j]:
            d.start()
    c_wo.start()

    for i in range(1, NC):
        for pp in range(NP):
            new = [(2 * pp + a, [None, None], [None, None]) for a in range(2)]

            def use(a, t, c, new=new, i=i, pp=pp):
                g = 2 * pp + a
                _st(phiq_v[i], g * 256, (g + 1) * 256, slice(t * 128, (t + 1) * 128), _feat(c[0:128]))
                new[a][1][t] = _feat(c[128:256])
                new[a][2][t] = c[256:384]

            def hook(h, i=i, pp=pp):
                side_work(i * 8 + pp * 2 + h)
                if i == 1 and h == 1 and pp + 1 < NP:
                    prep(0, pp + 1)

            project(lambda k, pp=pp: jnp.concatenate([_ld(sq_v[pp][k], 0, 128), _ld(skv_v[pp][k], 0, 256)], axis=0),
                    i, pp == 0, use, kv_flush, hook)
            pend.extend(new)

    def finalize():
        if pend:
            kv_flush()
            r80 = lax.broadcasted_iota(jnp.int32, (80, 128), 0)
            c80 = lax.broadcasted_iota(jnp.int32, (80, 128), 1)
            keep = jnp.where(r80 < 64, r80 // 32, (r80 - 64) // 8) == (c80 // 64)
            for p in range(2 * NG):
                _st(kvz_v, p * 80, (p + 1) * 80, ALL, jnp.where(keep, acc_v[p], 0.0).astype(bf16))

    for q in range(NP // 2):
        def use(a, t, c, q=q):
            for e in range(2):
                g = 2 * (2 * q + e) + a
                _st(phiq_v[0], g * 256, (g + 1) * 256, slice(t * 128, (t + 1) * 128), _feat(c[e * 128:(e + 1) * 128]))

        project(lambda k, q=q: jnp.concatenate([_ld(sq_v[2 * q][k], 0, 128), _ld(sq_v[2 * q + 1][k], 0, 128)], axis=0),
                0, False, use, finalize, lambda h: None)

    yrow = jnp.concatenate([jnp.sum(y, axis=0, keepdims=True) * st["rs"] for y in st["y"]], axis=1)

    def attn(i):
        ot = []
        for p in range(2 * NG):
            nd = jnp.dot(_ld(kvz_v, p * 80, (p + 1) * 80), _ld(phiq_v[i], p * 128, (p + 1) * 128),
                         preferred_element_type=f32)
            for a in range(2):
                rden = 1.0 / (nd[64 + 8 * a:72 + 8 * a] + 1e-6)
                o = nd[32 * a:32 * a + 32].reshape(4, 8, T) * rden[None]
                ot.append(o.reshape(32, T))
        ot = jnp.concatenate(ot, axis=0)
        return [s.astype(bf16).T for s in _left(ot[:HD, :128], ot[HD:, :128], ot[:HD, 128:], ot[HD:, 128:])]

    def finish(i, o):
        def m(k):
            rhs = wo_right(k) if k in (1, 4) else _ld(wot_v, k * HD, (k + 1) * HD)
            return jnp.dot(o[k], rhs, preferred_element_type=f32)

        def mix(t, c, a):
            rows = slice(t * 128, (t + 1) * 128)
            gate = jax.nn.sigmoid(gate_v[i, rows, :])
            omg = 1.0 - gate
            hit = (lax.broadcasted_iota(jnp.int32, (128, 128), 0) + (i * T + t * 128)) == st["idxv"]
            for k in range(HD // 128):
                ks = slice(c * HD + k * 128, c * HD + (k + 1) * 128)
                xb = _ld(x_v[i], t * 128, (t + 1) * 128, ks).astype(f32)
                b = xb + (xb * 0.0 + jnp.where(hit, yrow[:, ks], 0.0))
                _st(out_v[i], t * 128, (t + 1) * 128, ks,
                    (gate * a[:, k * 128:(k + 1) * 128] + omg * b).astype(bf16))

        m5 = m(4)
        m3 = m(2)
        mix(0, 1, m3 + m5)
        m2 = m(1)
        m4 = m(3)
        mix(1, 0, m2 + m4)
        m1 = m(0)
        c11 = m1 + m4 - m5
        c22 = m1 - m2 + m3
        mix(0, 0, c11 + m(6))
        mix(1, 1, c22 + m(5))
        c_o[i].start()

    order = list(range(1, NC)) + [0]
    o_prev = attn(order[0])
    for n, i in enumerate(order):
        o_next = attn(order[n + 1]) if n + 1 < NC else None
        finish(i, o_prev)
        o_prev = o_next
    for i in order:
        c_o[i].wait()


@jax.jit
def pallas_gated_mix__linear_kernel_hedgehog__moe_arch_mod__prompt_kernel(A_x, A_wqkv, A_w_phi, A_wo, B_x, B_w_r, B_w_gate, B_w_up, B_w_down, gate_w):
    anyspec = pl.BlockSpec(memory_space=pl.ANY)
    V = pltpu.VMEM
    P = lambda r, c: V((r // 2, c), u32)
    out = pl.pallas_call(
        _kernel,
        out_shape=jax.ShapeDtypeStruct((S, D), bf16),
        in_specs=[anyspec] * 9,
        out_specs=anyspec,
        scratch_shapes=[
            [P(T, D) for _ in range(NC)],
            [[P(D, 128) for _ in range(NG)] for _ in range(3)],
            V((D, DH), bf16), P(D, D), V((D,), bf16), V((D,), bf16),
            [P(D, FC) for _ in range(NF)], [P(D, FC) for _ in range(NF)], [P(FC, D) for _ in range(NF)],
            [[P(128, HD) for _ in range(7)] for _ in range(NP)],
            [[P(256, HD) for _ in range(7)] for _ in range(NP)],
            [P(7 * 128, HD) for _ in range(NC)], P(7 * HD, HD),
            [P(2 * D, T) for _ in range(NC)],
            V((2 * NG, 80, 128), f32), P(2 * NG * 80, 128),
            [P(T, D) for _ in range(NC)],
            V((D, 128), f32), V((NC, T, 128), f32), P(NG * 128, 128), V((16, D), f32),
            pltpu.SemaphoreType.DMA((65,)),
        ],
        compiler_params=pltpu.CompilerParams(vmem_limit_bytes=120 * 2**20),
    )(A_x.reshape(S, D), A_wqkv, A_w_phi.reshape(D, DH), A_wo,
      B_w_r, B_w_gate, B_w_up, B_w_down, gate_w)
    return out.reshape(1, S, D)
```

```python
import functools

import jax
import jax.numpy as jnp
import numpy as np
from jax import lax
import jax.experimental.pallas as pl
import jax.experimental.pallas.tpu as pltpu

S, D, H, DH, F = 2048, 1024, 32, 32, 3584
T = 256
NC = S // T
NG = 8
NP = NG // 2
HD = D // 2
FC = 512
NF = F // FC
NB = F // 128
NDOT = 28 * NC + 14
LAG = 3
FFN0 = 111
GAP = 5
FFN_WAIT = {0: (0, 1), 8: (2, 3), 16: (4, 5), 24: (6,)}
f32, bf16, u32 = jnp.float32, jnp.bfloat16, jnp.uint32
NT = (((1,), (1,)), ((), ()))
LOG2E = 1.4426950408889634
ALL = slice(None)


def _ld(ref, r0, r1, cols=ALL):
    return pltpu.bitcast(ref[r0 // 2:r1 // 2, cols], bf16)


def _st(ref, r0, r1, cols, val):
    ref[r0 // 2:r1 // 2, cols] = pltpu.bitcast(val, u32)


def _rcp(x):
    r = pl.reciprocal(x, approx=True)
    return r * (2.0 - x * r)


def _feat(p):
    outs = []
    for h in range(4):
        ph = p[h * DH:(h + 1) * DH]
        mx = jnp.max(ph, axis=0, keepdims=True)
        mn = jnp.min(ph, axis=0, keepdims=True)
        e1 = jnp.exp2(ph - mx)
        e2 = jnp.exp2(mn - ph)
        r1 = _rcp(jnp.sum(e1, axis=0, keepdims=True))
        r2 = _rcp(jnp.sum(e2, axis=0, keepdims=True))
        outs.append(e1 * r1)
        outs.append(e2 * r2)
    return jnp.concatenate(outs, axis=0).astype(bf16)


def _left(a11, a12, a21, a22):
    return (a11 + a22, a21 + a22, a11, a22, a11 + a12, a21 - a11, a12 - a22)


def _right(k, b11, b12, b21, b22):
    if k == 1:
        return b11()
    if k == 4:
        return b22()
    p, q, sub = {0: (b11, b22, False), 2: (b12, b22, True), 3: (b21, b11, True),
                 5: (b11, b12, False), 6: (b21, b22, False)}[k]
    p, q = p().astype(f32), q().astype(f32)
    return (p - q if sub else p + q).astype(bf16)


def _kernel(x_hbm, wqkv_hbm, wphi_hbm, wo_hbm, wr_hbm, wg_hbm, wu_hbm, wd_hbm, gw_hbm,
            out_hbm,
            x_v, wraw_v, wphi_v, wo_v, wr_v, gw_v, wg_v, wu_v, wd_v,
            sq_v, skv_v, xt_v, wot_v, phiq_v, acc_v, kvz_v, out_v, xcol_v, gate_v, bd_v, rg_v,
            sems):
    cp = pltpu.make_async_copy
    c_wphi = cp(wphi_hbm, wphi_v, sems.at[0])
    c_wr = cp(wr_hbm, wr_v, sems.at[6])
    c_gw = cp(gw_hbm, gw_v, sems.at[6])
    c_w = [[cp(wqkv_hbm.at[:, pl.ds(j * D + g * 128, 128)], wraw_v[j][g].bitcast(bf16),
               sems.at[1 + g // 2 if j else 5 + g // 4]) for g in range(NG)] for j in range(3)]
    c_x = [cp(x_hbm.at[pl.ds(i * T, T)], x_v[i].bitcast(bf16), sems.at[(1, 5, 6, 7)[min(i, 3)]])
           for i in range(NC)]
    fsem = {j: n for n, js in enumerate(FFN_WAIT.values()) for j in js}
    c_f = [[cp(wg_hbm.at[:, pl.ds(j * FC, FC)], wg_v[j].bitcast(bf16), sems.at[fsem[j]]),
            cp(wu_hbm.at[:, pl.ds(j * FC, FC)], wu_v[j].bitcast(bf16), sems.at[fsem[j]]),
            cp(wd_hbm.at[pl.ds(j * FC, FC)], wd_v[j].bitcast(bf16), sems.at[fsem[j]])] for j in range(NF)]
    c_wo = cp(wo_hbm, wo_v.bitcast(bf16), sems.at[fsem[NF - 1]])
    c_o = [cp(out_v[i].bitcast(bf16), out_hbm.at[pl.ds(i * T, T)], sems.at[4]) for i in range(1, NC)]
    c_o0 = {(t, c): cp(out_v[0].bitcast(bf16).at[pl.ds(t * 128, 128), pl.ds(c * HD, HD)],
                       out_hbm.at[pl.ds(t * 128, 128), pl.ds(c * HD, HD)], sems.at[4])
            for t in range(2) for c in range(2)}

    c_wphi.start()
    for g in range(NG):
        c_w[1][g].start()
        c_w[2][g].start()
        if g == 1:
            c_x[0].start()
    c_wr.start(); c_gw.start()
    c_x[1].start()
    for g in range(NG):
        c_w[0][g].start()
    for i in range(2, NC):
        c_x[i].start()

    row = lax.broadcasted_iota(jnp.int32, (128, 128), 0)
    col = lax.broadcasted_iota(jnp.int32, (128, 128), 1)
    diag = (row // DH) == (col // DH)
    rep = ((lax.broadcasted_iota(jnp.int32, (DH, 128), 1) % DH)
           == lax.broadcasted_iota(jnp.int32, (DH, 128), 0)).astype(bf16)
    acc_v[...] = jnp.zeros_like(acc_v)
    c_wphi.wait()
    for g in range(NG):
        wt = jnp.dot(wphi_v[g * 128:(g + 1) * 128, :], rep, preferred_element_type=f32)
        _st(bd_v, g * 128, (g + 1) * 128, ALL, jnp.where(diag, wt, 0.0).T.astype(bf16))

    def prep(j, pp):
        w = []
        for g in (2 * pp, 2 * pp + 1):
            raw = _ld(wraw_v[j][g], 0, D)
            if j < 2:
                w.append(lax.dot_general(_ld(bd_v, g * 128, (g + 1) * 128), raw, NT,
                                         preferred_element_type=f32) * LOG2E)
            else:
                w.append(raw.T.astype(f32))
        dst, r0 = (sq_v, 0) if j == 0 else (skv_v, (j - 1) * 128)
        for k, s in enumerate(_left(w[0][:, :HD], w[0][:, HD:], w[1][:, :HD], w[1][:, HD:])):
            _st(dst[pp][k], r0, r0 + 128, ALL, s.astype(bf16))

    ones = jnp.ones((16, T), f32)
    st = {"n": 0}

    def tie(a, dep):
        if dep is None:
            return a
        if a.dtype == f32:
            return jnp.where(st["never"], dep, a)
        blk = pltpu.bitcast(jnp.where(st["never"], dep, pltpu.bitcast(a[0:16, 0:128], f32)), bf16)
        return jnp.concatenate([jnp.concatenate([blk, a[0:16, 128:]], axis=1), a[16:]], axis=0)

    def xright(i, k, fresh):
        blk = lambda r, c: (lambda: _ld(x_v[i], r * 128, (r + 1) * 128, slice(c * HD, (c + 1) * HD)))
        if k in (1, 4) or fresh:
            val = _right(k, blk(0, 0), blk(1, 0), blk(0, 1), blk(1, 1))
            if k not in (1, 4):
                _st(xt_v[i], k * 128, (k + 1) * 128, ALL, val)
            return val
        return _ld(xt_v[i], k * 128, (k + 1) * 128)

    jobs = {}
    after = {}
    ties = {}

    def project(lhs, i, fresh, use, mid):
        def m(k):
            n = st["n"]
            st["n"] = n + 1
            out = lax.dot_general(tie(lhs(k), ties.pop(n, None)), xright(i, k, fresh), NT,
                                  preferred_element_type=f32)
            if n in after:
                after.pop(n)()
            if n in jobs:
                res = jobs.pop(n)(out[0:8])
                if res is not None and n + LAG < NDOT:
                    ties[n + LAG] = res
            return out
        m5 = m(4)
        m3 = m(2)
        use(0, 1, m3 + m5)
        mid()
        m2 = m(1)
        m4 = m(3)
        use(1, 0, m2 + m4)
        m1 = m(0)
        c11 = m1 + m4 - m5
        c22 = m1 - m2 + m3
        use(0, 0, c11 + m(6))
        use(1, 1, c22 + m(5))

    pend = []

    def kv_flush():
        for g, fk, vt in pend:
            fk = jnp.concatenate(fk, axis=1)
            vt = jnp.concatenate(vt, axis=1)
            for p in range(2):
                lhs = jnp.concatenate([vt[p * 64:(p + 1) * 64], ones], axis=0).astype(bf16)
                acc_v[2 * g + p] += lax.dot_general(lhs, fk[p * 128:(p + 1) * 128], NT,
                                                    preferred_element_type=f32)
        pend.clear()

    def router(i, part, dep):
        best, bidx = st["best"], st["bidx"]
        for b in range(part * 4, part * 4 + 4):
            rows = slice(b * 16, (b + 1) * 16)
            xf = [_ld(x_v[i], b * 16, (b + 1) * 16, slice(k * 128, (k + 1) * 128)).astype(f32)
                  for k in range(D // 128)]
            acc = []
            for w in range(2):
                for hf in range(2):
                    a = None
                    for k in range(D // 128):
                        p = xf[k][hf * 8:(hf + 1) * 8] * rg_v[w * 8:(w + 1) * 8, k * 128:(k + 1) * 128]
                        a = tie(p, dep) if k == 0 else a + p
                    acc.append(a)
                    dep = a
            ra, ga = jnp.concatenate(acc[0:2], axis=0), jnp.concatenate(acc[2:4], axis=0)
            r = jnp.sum(ra, axis=1, keepdims=True).astype(bf16).astype(f32)
            gate_v[i, rows, :] = jnp.broadcast_to(jnp.sum(ga, axis=1, keepdims=True), (16, 128))
            r = jnp.broadcast_to(r, (16, 128))
            for k in range(2):
                rk = r[k * 8:(k + 1) * 8]
                if best is None:
                    best, bidx = rk, jnp.zeros((8, 128), jnp.int32)
                else:
                    better = rk > best
                    best = jnp.where(better, rk, best)
                    bidx = jnp.where(better, i * T + b * 16 + k * 8, bidx)
        st["best"], st["bidx"] = best, bidx
        return dep

    def select():
        best, bidx = st["best"], st["bidx"]
        m = jnp.max(best, axis=0, keepdims=True)
        cand = jnp.where(best == m, bidx + lax.broadcasted_iota(jnp.int32, (8, 128), 0), S - 1)
        idxv = jnp.min(cand, axis=0, keepdims=True)
        idx = idxv[0, 0]
        st["idxv"] = idxv
        st["rs"] = jax.nn.sigmoid(m)
        base = pl.multiple_of(((idx % T) // 16) * 8, 8)
        tile = x_v[0][pl.ds(base, 8), :]
        for i in range(1, NC):
            tile = jnp.where(idx // T == i, x_v[i][pl.ds(base, 8), :], tile)
        tile = pltpu.bitcast(tile, bf16).astype(f32)
        sel = lax.broadcasted_iota(jnp.int32, (16, D), 0) == (idx % 16)
        xs = jnp.sum(jnp.where(sel, tile, 0.0), axis=0, keepdims=True)
        for k in range(D // 128):
            xcol_v[k * 128:(k + 1) * 128, :] = jnp.broadcast_to(xs[:, k * 128:(k + 1) * 128], (128, 128)).T
        st["y"] = [None] * (D // 128)

    def chain(w_ref, r0, nblk, cols, col_of, dep):
        acc = None
        for k in range(nblk):
            p = _ld(w_ref, r0 + k * 16, r0 + (k + 1) * 16, cols).astype(f32) * col_of(k)
            acc = tie(p[0:8], dep) if acc is None else acc + p[0:8]
            acc = acc + p[8:16]
        return acc

    def ffn_in(w, c, dep):
        j, cc = divmod(c, FC // 128)
        acc = chain((wg_v, wu_v)[w][j], 0, D // 16, slice(cc * 128, (cc + 1) * 128),
                    lambda k: xcol_v[k * 16:(k + 1) * 16, :], dep)
        v = jnp.sum(acc, axis=0, keepdims=True)
        if w == 0:
            st["g", c] = v * jax.nn.sigmoid(v)
        else:
            st["h", c] = jnp.broadcast_to(st.pop(("g", c)) * v, (128, 128)).T
        return acc

    def ffn_down(c, dep):
        j, cc = divmod(c, FC // 128)
        hcol = st.pop(("h", c))
        ys = st["y"]
        for n in range(D // 128):
            dep = chain(wd_v[j], cc * 128, 128 // 16, slice(n * 128, (n + 1) * 128),
                        lambda k: hcol[k * 16:(k + 1) * 16], dep)
            ys[n] = dep if ys[n] is None else ys[n] + dep
        return dep

    def wo_right(k):
        blk = lambda r, c: (lambda: _ld(wo_v, r * HD, (r + 1) * HD, slice(c * HD, (c + 1) * HD)))
        return _right(k, blk(0, 0), blk(0, 1), blk(1, 0), blk(1, 1))

    def wo_job(k, dep):
        _st(wot_v, k * HD, (k + 1) * HD, ALL, wo_right(k))

    def wait_rest():
        for k in range(3, NC):
            c_x[k].wait()

    def wait_kv(pp):
        for g in (2 * pp, 2 * pp + 1):
            c_w[1][g].wait()
            c_w[2][g].wait()
        if pp == 0:
            c_x[0].wait()
        prep(1, pp); prep(2, pp)

    def wait_q(half):
        c_x[1 + half].wait()
        for g in range(4 * half, 4 * half + 4):
            c_w[0][g].wait()
        prep(0, 2 * half)
        if half:
            c_wr.wait(); c_gw.wait()
            wr = wr_v[...].reshape(1, D).astype(f32)
            rg_v[0:8, :] = jnp.broadcast_to(wr, (8, D))
            rg_v[8:16, :] = jnp.broadcast_to(gw_v[...].reshape(1, D).astype(f32), (8, D))
            st["best"] = st["bidx"] = None
            st["never"] = jnp.broadcast_to((pltpu.bitcast(wr[:, 0:128], jnp.int32) | 1) == 0, (8, 128))

    def wait_ffn(js):
        for j in js:
            for d in c_f[j]:
                d.wait()
            if j == NF - 1:
                c_wo.wait()

    for pp in range(1, NP):
        after[7 * pp - 1] = functools.partial(wait_kv, pp)
    after[27] = functools.partial(wait_q, 0)
    after[34] = functools.partial(prep, 0, 1)
    after[41] = functools.partial(wait_q, 1)
    after[48] = functools.partial(prep, 0, 3)
    after[83] = wait_rest
    for r in range(4 * NC):
        jobs[56 + 2 * r if r < 12 else 72 + r] = functools.partial(router, r // 4, r % 4)
    jobs[106] = lambda dep: select()
    units = []
    for c in range(NB + 1):
        if c < NB:
            units += [(c, functools.partial(ffn_in, 0, c)), (c, functools.partial(ffn_in, 1, c))]
        if c > 0:
            units.append((-1, functools.partial(ffn_down, c - 1)))
    n, waits = FFN0, dict(FFN_WAIT)
    for c, u in units:
        if c in waits:
            n += 0 if c == 0 else LAG - 1
            after[n] = functools.partial(wait_ffn, waits.pop(c))
        jobs[n] = u
        n += 1 if n % 7 == 6 or c < 0 or (n * 5) % 29 > GAP else 2
    assert n <= 28 * NC + 6
    for e, k in enumerate((2, 3, 0, 6, 5)):
        jobs[28 * NC + 7 + e] = functools.partial(wo_job, k)

    wait_kv(0)
    for pp in range(NP):
        new = [(2 * pp + a, [None, None], [None, None]) for a in range(2)]

        def use(a, t, c, new=new):
            new[a][1][t] = _feat(c[0:128])
            new[a][2][t] = c[128:256]

        project(lambda k, pp=pp: _ld(skv_v[pp][k], 0, 256), 0, pp == 0, use, kv_flush)
        pend.extend(new)

    for j in range(NF):
        for d in c_f[j]:
            d.start()
    c_wo.start()

    for i in range(1, NC):
        for pp in range(NP):
            new = [(2 * pp + a, [None, None], [None, None]) for a in range(2)]

            def use(a, t, c, new=new, i=i, pp=pp):
                g = 2 * pp + a
                _st(phiq_v[i], g * 256, (g + 1) * 256, slice(t * 128, (t + 1) * 128), _feat(c[0:128]))
                new[a][1][t] = _feat(c[128:256])
                new[a][2][t] = c[256:384]

            project(lambda k, pp=pp: jnp.concatenate([_ld(sq_v[pp][k], 0, 128), _ld(skv_v[pp][k], 0, 256)], axis=0),
                    i, pp == 0, use, kv_flush)
            pend.extend(new)

    def finalize():
        if pend:
            kv_flush()
            r80 = lax.broadcasted_iota(jnp.int32, (80, 128), 0)
            c80 = lax.broadcasted_iota(jnp.int32, (80, 128), 1)
            keep = jnp.where(r80 < 64, r80 // 32, (r80 - 64) // 8) == (c80 // 64)
            for p in range(2 * NG):
                _st(kvz_v, p * 80, (p + 1) * 80, ALL, jnp.where(keep, acc_v[p], 0.0).astype(bf16))

    for q in range(NP // 2):
        def use(a, t, c, q=q):
            for e in range(2):
                g = 2 * (2 * q + e) + a
                _st(phiq_v[0], g * 256, (g + 1) * 256, slice(t * 128, (t + 1) * 128), _feat(c[e * 128:(e + 1) * 128]))

        project(lambda k, q=q: jnp.concatenate([_ld(sq_v[2 * q][k], 0, 128), _ld(sq_v[2 * q + 1][k], 0, 128)], axis=0),
                0, False, use, finalize)

    yrow = jnp.concatenate([jnp.sum(y, axis=0, keepdims=True) * st["rs"] for y in st["y"]], axis=1)

    def attn(i):
        ot = []
        for p in range(2 * NG):
            nd = jnp.dot(_ld(kvz_v, p * 80, (p + 1) * 80), _ld(phiq_v[i], p * 128, (p + 1) * 128),
                         preferred_element_type=f32)
            for a in range(2):
                rden = _rcp(nd[64 + 8 * a:72 + 8 * a] + 1e-6)
                o = nd[32 * a:32 * a + 32].reshape(4, 8, T) * rden[None]
                ot.append(o.reshape(32, T))
        ot = jnp.concatenate(ot, axis=0)
        return [s.astype(bf16).T for s in _left(ot[:HD, :128], ot[HD:, :128], ot[:HD, 128:], ot[HD:, 128:])]

    def finish(i, o):
        def m(k):
            rhs = wo_right(k) if k in (1, 4) else _ld(wot_v, k * HD, (k + 1) * HD)
            return jnp.dot(o[k], rhs, preferred_element_type=f32)

        def mix(t, c, a):
            rows = slice(t * 128, (t + 1) * 128)
            gate = jax.nn.sigmoid(gate_v[i, rows, :])
            omg = 1.0 - gate
            hit = (lax.broadcasted_iota(jnp.int32, (128, 128), 0) + (i * T + t * 128)) == st["idxv"]
            for k in range(HD // 128):
                ks = slice(c * HD + k * 128, c * HD + (k + 1) * 128)
                xb = _ld(x_v[i], t * 128, (t + 1) * 128, ks).astype(f32)
                b = xb + (xb * 0.0 + jnp.where(hit, yrow[:, ks], 0.0))
                _st(out_v[i], t * 128, (t + 1) * 128, ks,
                    (gate * a[:, k * 128:(k + 1) * 128] + omg * b).astype(bf16))
            if i == 0:
                c_o0[t, c].start()

        m5 = m(4)
        m3 = m(2)
        mix(0, 1, m3 + m5)
        m2 = m(1)
        m4 = m(3)
        mix(1, 0, m2 + m4)
        m1 = m(0)
        c11 = m1 + m4 - m5
        c22 = m1 - m2 + m3
        mix(0, 0, c11 + m(6))
        mix(1, 1, c22 + m(5))
        if i:
            c_o[i - 1].start()

    order = list(range(1, NC)) + [0]
    o_prev = attn(order[0])
    for n, i in enumerate(order):
        o_next = attn(order[n + 1]) if n + 1 < NC else None
        finish(i, o_prev)
        o_prev = o_next
    for d in c_o + list(c_o0.values()):
        d.wait()


@jax.jit
def pallas_gated_mix__linear_kernel_hedgehog__moe_arch_mod__prompt_kernel(A_x, A_wqkv, A_w_phi, A_wo, B_x, B_w_r, B_w_gate, B_w_up, B_w_down, gate_w):
    anyspec = pl.BlockSpec(memory_space=pl.ANY)
    V = pltpu.VMEM
    P = lambda r, c: V((r // 2, c), u32)
    out = pl.pallas_call(
        _kernel,
        out_shape=jax.ShapeDtypeStruct((S, D), bf16),
        in_specs=[anyspec] * 9,
        out_specs=anyspec,
        scratch_shapes=[
            [P(T, D) for _ in range(NC)],
            [[P(D, 128) for _ in range(NG)] for _ in range(3)],
            V((D, DH), bf16), P(D, D), V((D,), bf16), V((D,), bf16),
            [P(D, FC) for _ in range(NF)], [P(D, FC) for _ in range(NF)], [P(FC, D) for _ in range(NF)],
            [[P(128, HD) for _ in range(7)] for _ in range(NP)],
            [[P(256, HD) for _ in range(7)] for _ in range(NP)],
            [P(7 * 128, HD) for _ in range(NC)], P(7 * HD, HD),
            [P(2 * D, T) for _ in range(NC)],
            V((2 * NG, 80, 128), f32), P(2 * NG * 80, 128),
            [P(T, D) for _ in range(NC)],
            V((D, 128), f32), V((NC, T, 128), f32), P(NG * 128, 128), V((16, D), f32),
            pltpu.SemaphoreType.DMA((8,)),
        ],
        compiler_params=pltpu.CompilerParams(vmem_limit_bytes=120 * 2**20),
    )(A_x.reshape(S, D), A_wqkv, A_w_phi.reshape(D, DH), A_wo,
      B_w_r, B_w_gate, B_w_up, B_w_down, gate_w)
    return out.reshape(1, S, D)
```

```python
import functools

import jax
import jax.numpy as jnp
import numpy as np
from jax import lax
import jax.experimental.pallas as pl
import jax.experimental.pallas.tpu as pltpu

S, D, H, DH, F = 2048, 1024, 32, 32, 3584
T = 256
NC = S // T
NG = 8
NP = NG // 2
HD = D // 2
FC = 512
NF = F // FC
NB = F // 128
NDOT = 28 * NC + 14
LAG = 4
GU0 = 2
W1, W2 = 150, 203
f32, bf16, u32 = jnp.float32, jnp.bfloat16, jnp.uint32
NT = (((1,), (1,)), ((), ()))
LOG2E = 1.4426950408889634
ALL = slice(None)


def _ld(ref, r0, r1, cols=ALL):
    return pltpu.bitcast(ref[r0 // 2:r1 // 2, cols], bf16)


def _st(ref, r0, r1, cols, val):
    ref[r0 // 2:r1 // 2, cols] = pltpu.bitcast(val, u32)


def _rcp(x):
    r = pl.reciprocal(x, approx=True)
    return r * (2.0 - x * r)


def _heads(v, op):
    r = v[0]
    for j in range(1, 8):
        r = op(r, v[j])
    r = op(r, pltpu.roll(r, 4, 0))
    return op(r, pltpu.roll(r, 2, 0))


def _feat(p):
    outs = []
    for h in range(2):
        ph = p[h * 64:(h + 1) * 64].reshape(8, 8, p.shape[1])
        e1 = jnp.exp2(ph - _heads(ph, jnp.maximum)[None])
        e2 = jnp.exp2(_heads(ph, jnp.minimum)[None] - ph)
        for e in (e1, e2):
            outs.append((e * _rcp(_heads(e, jnp.add))[None]).reshape(64, p.shape[1]))
    return jnp.concatenate(outs, axis=0)


def _left(a11, a12, a21, a22):
    return (a11 + a22, a21 + a22, a11, a22, a11 + a12, a21 - a11, a12 - a22)


def _right(k, b11, b12, b21, b22):
    if k == 1:
        return b11()
    if k == 4:
        return b22()
    p, q, sub = {0: (b11, b22, False), 2: (b12, b22, True), 3: (b21, b11, True),
                 5: (b11, b12, False), 6: (b21, b22, False)}[k]
    p, q = p().astype(f32), q().astype(f32)
    return (p - q if sub else p + q).astype(bf16)


def _kernel(x_hbm, wqkv_hbm, wphi_hbm, wo_hbm, wr_hbm, wg_hbm, wu_hbm, wd_hbm, gw_hbm,
            out_hbm,
            x_v, wraw_v, wphi_v, wo_v, wr_v, gw_v, wg_v, wu_v, wd_v,
            sq_v, skv_v, xt_v, wot_v, phiq_v, acc_v, kvz_v, out_v, out0_v, xcol_v, gate_v, bd_v, rg_v, h_v,
            sems):
    cp = pltpu.make_async_copy
    c_wphi = cp(wphi_hbm, wphi_v, sems.at[0])
    c_wr = cp(wr_hbm, wr_v, sems.at[9])
    c_gw = cp(gw_hbm, gw_v, sems.at[9])
    wsem = lambda j, g: 1 + g // 2 if j else (5, 9)[g // 4]
    c_w = [[cp(wqkv_hbm.at[:, pl.ds(j * D + g * 128, 128)], wraw_v[j][g].bitcast(bf16), sems.at[wsem(j, g)])
            for g in range(NG)] for j in range(3)]
    c_x = [cp(x_hbm.at[pl.ds(i * T, T)], x_v[i].bitcast(bf16), sems.at[(1, 5, 9, 6)[min(i, 3)]])
           for i in range(NC)]
    c_gu = [cp(w.at[:, pl.ds(j * FC, FC)], v[j].bitcast(bf16), sems.at[6 if j < GU0 else 7])
            for j in range(NF) for w, v in ((wg_hbm, wg_v), (wu_hbm, wu_v))]
    c_d = [cp(wd_hbm.at[pl.ds(j * FC, FC)], wd_v[j].bitcast(bf16), sems.at[8]) for j in range(NF)]
    c_d.append(cp(wo_hbm, wo_v.bitcast(bf16), sems.at[8]))
    c_o = [cp(out_v[i - 1].bitcast(bf16), out_hbm.at[pl.ds(i * T, T)], sems.at[2]) for i in range(1, NC)]
    c_o0 = {(t, c): cp(out0_v[t][c].bitcast(bf16), out_hbm.at[pl.ds(t * 128, 128), pl.ds(c * HD, HD)], sems.at[2])
            for t in range(2) for c in range(2)}

    for d in [c_wphi, c_w[1][0], c_w[1][1], c_w[2][0], c_w[2][1], c_x[0]]:
        d.start()
    for g in range(2, NG):
        c_w[1][g].start()
        c_w[2][g].start()
    for d in [c_x[1]] + c_w[0][:4] + [c_wr, c_gw] + c_w[0][4:] + c_x[2:] + c_gu + c_d:
        d.start()

    row = lax.broadcasted_iota(jnp.int32, (128, 128), 0)
    col = lax.broadcasted_iota(jnp.int32, (128, 128), 1)
    diag = (row // DH) == (col // 64) * 2 + col % 2
    rep = (((lax.broadcasted_iota(jnp.int32, (DH, 128), 1) % 64) // 2)
           == lax.broadcasted_iota(jnp.int32, (DH, 128), 0)).astype(bf16)
    acc_v[...] = jnp.zeros_like(acc_v)
    ones = jnp.ones((16, T), bf16)
    c_wphi.wait()
    for g in range(NG):
        wt = jnp.dot(wphi_v[g * 128:(g + 1) * 128, :], rep, preferred_element_type=f32)
        _st(bd_v, g * 128, (g + 1) * 128, ALL, jnp.where(diag, wt, 0.0).T.astype(bf16))

    def prep(j, pp):
        w = []
        for g in (2 * pp, 2 * pp + 1):
            raw = _ld(wraw_v[j][g], 0, D)
            if j < 2:
                w.append(lax.dot_general(_ld(bd_v, g * 128, (g + 1) * 128), raw, NT,
                                         preferred_element_type=f32) * LOG2E)
            else:
                w.append(raw.T.astype(f32))
        dst, r0 = (sq_v, 0) if j == 0 else (skv_v, (j - 1) * 128)
        for k, s in enumerate(_left(w[0][:, :HD], w[0][:, HD:], w[1][:, :HD], w[1][:, HD:])):
            _st(dst[pp][k], r0, r0 + 128, ALL, s.astype(bf16))

    st = {"n": 0}

    def tie(a, dep):
        if dep is None:
            return a
        if a.dtype == f32:
            return jnp.where(st["never"], dep, a)
        blk = pltpu.bitcast(jnp.where(st["never"], dep, pltpu.bitcast(a[0:16, 0:128], f32)), bf16)
        return jnp.concatenate([jnp.concatenate([blk, a[0:16, 128:]], axis=1), a[16:]], axis=0)

    def xright(i, k, fresh):
        blk = lambda r, c: (lambda: _ld(x_v[i], r * 128, (r + 1) * 128, slice(c * HD, (c + 1) * HD)))
        if k in (1, 4) or fresh:
            val = _right(k, blk(0, 0), blk(1, 0), blk(0, 1), blk(1, 1))
            if k not in (1, 4):
                _st(xt_v[i], k * 128, (k + 1) * 128, ALL, val)
            return val
        return _ld(xt_v[i], k * 128, (k + 1) * 128)

    jobs = {}
    after = {}
    ties = {}

    def project(lhs, i, fresh, use, mid):
        def m(k):
            n = st["n"]
            st["n"] = n + 1
            out = lax.dot_general(tie(lhs(k), ties.pop(n, None)), xright(i, k, fresh), NT,
                                  preferred_element_type=f32)
            if n in after:
                after.pop(n)()
            if n in jobs:
                res = jobs.pop(n)(out[0:8])
                if res is not None and n + LAG < NDOT:
                    ties[n + LAG] = res
            return out
        m5 = m(4)
        m3 = m(2)
        use(0, 1, m3 + m5)
        mid()
        m2 = m(1)
        m4 = m(3)
        use(1, 0, m2 + m4)
        m1 = m(0)
        c11 = m1 + m4 - m5
        c22 = m1 - m2 + m3
        use(0, 0, c11 + m(6))
        use(1, 1, c22 + m(5))

    pend = []

    def feat_k(g, p):
        fk = _feat(p)
        return fk.astype(bf16)

    def kv_flush():
        for g, fk, vt in pend:
            fk = jnp.concatenate(fk, axis=1)
            vt = jnp.concatenate(vt, axis=1)
            for p in range(2):
                lhs = jnp.concatenate([vt[p * 64:(p + 1) * 64], ones], axis=0)
                acc_v[2 * g + p] += lax.dot_general(lhs, fk[p * 128:(p + 1) * 128], NT,
                                                    preferred_element_type=f32)
        pend.clear()

    def router(i, part, dep):
        best, bidx = st["best"], st["bidx"]
        for b in range(part * 4, part * 4 + 4):
            rows = slice(b * 16, (b + 1) * 16)
            xf = [_ld(x_v[i], b * 16, (b + 1) * 16, slice(k * 128, (k + 1) * 128)).astype(f32)
                  for k in range(D // 128)]
            acc = []
            for w in range(2):
                for hf in range(2):
                    a = None
                    for k in range(D // 128):
                        p = xf[k][hf * 8:(hf + 1) * 8] * rg_v[w * 8:(w + 1) * 8, k * 128:(k + 1) * 128]
                        a = tie(p, dep) if k == 0 else a + p
                    acc.append(a)
                    dep = a
            ra, ga = jnp.concatenate(acc[0:2], axis=0), jnp.concatenate(acc[2:4], axis=0)
            r = jnp.sum(ra, axis=1, keepdims=True).astype(bf16).astype(f32)
            gate_v[i, rows, :] = jnp.broadcast_to(jnp.sum(ga, axis=1, keepdims=True), (16, 128))
            r = jnp.broadcast_to(r, (16, 128))
            for k in range(2):
                rk = r[k * 8:(k + 1) * 8]
                if best is None:
                    best, bidx = rk, jnp.zeros((8, 128), jnp.int32)
                else:
                    better = rk > best
                    best = jnp.where(better, rk, best)
                    bidx = jnp.where(better, i * T + b * 16 + k * 8, bidx)
        st["best"], st["bidx"] = best, bidx
        return dep

    def select():
        best, bidx = st["best"], st["bidx"]
        m = jnp.max(best, axis=0, keepdims=True)
        cand = jnp.where(best == m, bidx + lax.broadcasted_iota(jnp.int32, (8, 128), 0), S - 1)
        idxv = jnp.min(cand, axis=0, keepdims=True)
        idx = idxv[0, 0]
        st["idxv"] = idxv
        st["rs"] = jax.nn.sigmoid(m)
        base = pl.multiple_of(((idx % T) // 16) * 8, 8)
        tile = x_v[0][pl.ds(base, 8), :]
        for i in range(1, NC):
            tile = jnp.where(idx // T == i, x_v[i][pl.ds(base, 8), :], tile)
        tile = pltpu.bitcast(tile, bf16).astype(f32)
        sel = lax.broadcasted_iota(jnp.int32, (16, D), 0) == (idx % 16)
        xs = jnp.sum(jnp.where(sel, tile, 0.0), axis=0, keepdims=True)
        for k in range(D // 128):
            xcol_v[k * 128:(k + 1) * 128, :] = jnp.broadcast_to(xs[:, k * 128:(k + 1) * 128], (128, 128)).T
        st["y"] = [None] * (D // 128)

    def chain(w_ref, r0, nblk, cols, col_of, dep):
        acc = None
        for k in range(nblk):
            p = _ld(w_ref, r0 + k * 16, r0 + (k + 1) * 16, cols).astype(f32) * col_of(k)
            acc = tie(p[0:8], dep) if acc is None else acc + p[0:8]
            acc = acc + p[8:16]
        return acc

    def ffn_in(w, c, dep):
        j, cc = divmod(c, FC // 128)
        acc = chain((wg_v, wu_v)[w][j], 0, D // 16, slice(cc * 128, (cc + 1) * 128),
                    lambda k: xcol_v[k * 16:(k + 1) * 16, :], dep)
        v = jnp.sum(acc, axis=0, keepdims=True)
        if w == 0:
            st["g", c] = v * jax.nn.sigmoid(v)
        else:
            h_v[c] = jnp.broadcast_to(st.pop(("g", c)) * v, (8, 128))
        return acc

    def ffn_down(c, dep):
        j, cc = divmod(c, FC // 128)
        hcol = jnp.concatenate([h_v[c]] * 16, axis=0).T
        ys = st["y"]
        for n in range(D // 128):
            dep = chain(wd_v[j], cc * 128, 128 // 16, slice(n * 128, (n + 1) * 128),
                        lambda k: hcol[k * 16:(k + 1) * 16], dep)
            ys[n] = dep if ys[n] is None else ys[n] + dep
        return dep

    def wo_right(k):
        blk = lambda r, c: (lambda: _ld(wo_v, r * HD, (r + 1) * HD, slice(c * HD, (c + 1) * HD)))
        return _right(k, blk(0, 0), blk(0, 1), blk(1, 0), blk(1, 1))

    def wo_job(k, dep):
        _st(wot_v, k * HD, (k + 1) * HD, ALL, wo_right(k))

    def wait_kv(pp):
        for g in (2 * pp, 2 * pp + 1):
            c_w[1][g].wait()
            c_w[2][g].wait()
        if pp == 0:
            c_x[0].wait()
        prep(1, pp)
        prep(2, pp)

    def wait_q(half):
        for d in [c_x[1 + half]] + c_w[0][4 * half:4 * half + 4] + [c_wr, c_gw][:2 * half]:
            d.wait()
        prep(0, 2 * half)
        if half:
            wr = wr_v[...].reshape(1, D).astype(f32)
            rg_v[0:8, :] = jnp.broadcast_to(wr, (8, D))
            rg_v[8:16, :] = jnp.broadcast_to(gw_v[...].reshape(1, D).astype(f32), (8, D))
            st["best"] = st["bidx"] = None
            st["never"] = jnp.broadcast_to((pltpu.bitcast(wr[:, 0:128], jnp.int32) | 1) == 0, (8, 128))

    def wait_all(ds):
        for d in ds:
            d.wait()

    for pp in range(1, NP):
        after[7 * pp - 1] = functools.partial(wait_kv, pp)
    after[27] = functools.partial(wait_q, 0)
    after[34] = functools.partial(prep, 0, 1)
    after[41] = functools.partial(wait_q, 1)
    after[48] = functools.partial(prep, 0, 3)
    after[83] = functools.partial(wait_all, c_x[3:] + c_gu[:2 * GU0])
    for r in range(4 * NC):
        jobs[56 + 2 * r if r < 12 else 72 + r] = functools.partial(router, r // 4, r % 4)
    jobs[106] = lambda dep: select()
    n0 = 8 * GU0
    for u in range(2 * NB):
        pos = 111 + (u * (W1 - LAG - 111)) // n0 if u < n0 else W1 + 1 + ((u - n0) * (W2 - LAG - W1)) // (2 * NB - n0)
        assert pos not in jobs
        jobs[pos] = functools.partial(ffn_in, u % 2, u // 2)
    after[W1] = functools.partial(wait_all, c_gu[2 * GU0:])
    after[W2] = functools.partial(wait_all, c_d)
    for c in range(NB):
        jobs[W2 + 1 + c] = functools.partial(ffn_down, c)
    for e, k in enumerate((2, 3, 0, 6, 5)):
        jobs[W2 + 1 + NB + e] = functools.partial(wo_job, k)

    wait_kv(0)
    for i, pp in [(i, pp) for i in range(NC) for pp in range(NP)]:
        new = [(2 * pp + a, [None, None], [None, None]) for a in range(2)]

        def use(a, t, c, new=new, i=i, pp=pp):
            g = 2 * pp + a
            if i >= 1:
                _st(phiq_v[i], g * 256, (g + 1) * 256, slice(t * 128, (t + 1) * 128), _feat(c[0:128]).astype(bf16))
            new[a][1][t] = feat_k(g, c[-256:-128])
            new[a][2][t] = c[-128:].astype(bf16)

        def lhs(k, i=i, pp=pp):
            kvw = _ld(skv_v[pp][k], 0, 256)
            return jnp.concatenate([_ld(sq_v[pp][k], 0, 128), kvw], axis=0) if i >= 1 else kvw

        project(lhs, i, pp == 0, use, kv_flush)
        pend.extend(new)

    def finalize():
        if pend:
            kv_flush()
            r80 = lax.broadcasted_iota(jnp.int32, (80, 128), 0)
            c80 = lax.broadcasted_iota(jnp.int32, (80, 128), 1)
            keep = jnp.where(r80 < 64, r80 // 32, (r80 - 64) // 8) == (c80 % 2)
            for p in range(2 * NG):
                kvz = acc_v[p]
                _st(kvz_v, p * 80, (p + 1) * 80, ALL, jnp.where(keep, kvz, 0.0).astype(bf16))

    for i, q in ((0, 0), (0, 1)):
        def use(a, t, c, i=i, q=q):
            for e in range(2):
                g = 2 * (2 * q + e) + a
                _st(phiq_v[i], g * 256, (g + 1) * 256, slice(t * 128, (t + 1) * 128),
                    _feat(c[e * 128:(e + 1) * 128]).astype(bf16))

        project(lambda k, q=q: jnp.concatenate([_ld(sq_v[2 * q][k], 0, 128), _ld(sq_v[2 * q + 1][k], 0, 128)], axis=0),
                i, False, use, finalize)

    yrow = jnp.concatenate([jnp.sum(y, axis=0, keepdims=True) * st["rs"] for y in st["y"]], axis=1)

    def attn(i):
        ot = []
        for p in range(2 * NG):
            nd = jnp.dot(_ld(kvz_v, p * 80, (p + 1) * 80), _ld(phiq_v[i], p * 128, (p + 1) * 128),
                         preferred_element_type=f32)
            for a in range(2):
                rden = _rcp(nd[64 + 8 * a:72 + 8 * a] + 1e-6)
                o = nd[32 * a:32 * a + 32].reshape(4, 8, T) * rden[None]
                ot.append(o.reshape(32, T))
        ot = jnp.concatenate(ot, axis=0)
        return [s.astype(bf16).T for s in _left(ot[:HD, :128], ot[HD:, :128], ot[:HD, 128:], ot[HD:, 128:])]

    def finish(i, o):
        def m(k):
            rhs = wo_right(k) if k in (1, 4) else _ld(wot_v, k * HD, (k + 1) * HD)
            return jnp.dot(o[k], rhs, preferred_element_type=f32)

        def mix(t, c, a):
            rows = slice(t * 128, (t + 1) * 128)
            gate = jax.nn.sigmoid(gate_v[i, rows, :])
            omg = 1.0 - gate
            hit = (lax.broadcasted_iota(jnp.int32, (128, 128), 0) + (i * T + t * 128)) == st["idxv"]
            for k in range(HD // 128):
                ks = slice(c * HD + k * 128, c * HD + (k + 1) * 128)
                xb = _ld(x_v[i], t * 128, (t + 1) * 128, ks).astype(f32)
                b = xb + (xb * 0.0 + jnp.where(hit, yrow[:, ks], 0.0))
                res = (gate * a[:, k * 128:(k + 1) * 128] + omg * b).astype(bf16)
                if i:
                    _st(out_v[i - 1], t * 128, (t + 1) * 128, ks, res)
                else:
                    _st(out0_v[t][c], 0, 128, slice(k * 128, (k + 1) * 128), res)
            if i == 0:
                c_o0[t, c].start()

        m5 = m(4)
        m3 = m(2)
        mix(0, 1, m3 + m5)
        m2 = m(1)
        m4 = m(3)
        mix(1, 0, m2 + m4)
        m1 = m(0)
        c11 = m1 + m4 - m5
        c22 = m1 - m2 + m3
        mix(0, 0, c11 + m(6))
        mix(1, 1, c22 + m(5))
        if i:
            c_o[i - 1].start()

    order = list(range(1, NC)) + [0]
    o_prev = attn(order[0])
    for n, i in enumerate(order):
        o_next = attn(order[n + 1]) if n + 1 < NC else None
        finish(i, o_prev)
        o_prev = o_next
    for d in c_o + list(c_o0.values()):
        d.wait()


@jax.jit
def pallas_gated_mix__linear_kernel_hedgehog__moe_arch_mod__prompt_kernel(A_x, A_wqkv, A_w_phi, A_wo, B_x, B_w_r, B_w_gate, B_w_up, B_w_down, gate_w):
    anyspec = pl.BlockSpec(memory_space=pl.ANY)
    V = pltpu.VMEM
    P = lambda r, c: V((r // 2, c), u32)
    out = pl.pallas_call(
        _kernel,
        out_shape=jax.ShapeDtypeStruct((S, D), bf16),
        in_specs=[anyspec] * 9,
        out_specs=anyspec,
        scratch_shapes=[
            [P(T, D) for _ in range(NC)],
            [[P(D, 128) for _ in range(NG)] for _ in range(3)],
            V((D, DH), bf16), P(D, D), V((D,), bf16), V((D,), bf16),
            [P(D, FC) for _ in range(NF)], [P(D, FC) for _ in range(NF)], [P(FC, D) for _ in range(NF)],
            [[P(128, HD) for _ in range(7)] for _ in range(NP)],
            [[P(256, HD) for _ in range(7)] for _ in range(NP)],
            [P(7 * 128, HD) for _ in range(NC)], P(7 * HD, HD),
            [P(2 * D, T) for _ in range(NC)],
            V((2 * NG, 80, 128), f32), P(2 * NG * 80, 128),
            [P(T, D) for _ in range(NC - 1)], [[P(128, HD) for _ in range(2)] for _ in range(2)],
            V((D, 128), f32), V((NC, T, 128), f32), P(NG * 128, 128), V((16, D), f32), V((NB, 8, 128), f32),
            pltpu.SemaphoreType.DMA((10,)),
        ],
        compiler_params=pltpu.CompilerParams(vmem_limit_bytes=120 * 2**20),
    )(A_x.reshape(S, D), A_wqkv, A_w_phi.reshape(D, DH), A_wo,
      B_w_r, B_w_gate, B_w_up, B_w_down, gate_w)
    return out.reshape(1, S, D)
```

```python
import functools

import jax
import jax.numpy as jnp
import numpy as np
from jax import lax
import jax.experimental.pallas as pl
import jax.experimental.pallas.tpu as pltpu

S, D, H, DH, F = 2048, 1024, 32, 32, 3584
T = 256
NC = S // T
NG = 8
NP = NG // 2
HD = D // 2
FC = 512
NF = F // FC
NB = F // 128
NDOT = 28 * NC + 14
LAG = 4
GU0 = 2
W1, W2 = 143, 190
f32, bf16, u32 = jnp.float32, jnp.bfloat16, jnp.uint32
NT = (((1,), (1,)), ((), ()))
LOG2E = 1.4426950408889634
ALL = slice(None)


def _ld(ref, r0, r1, cols=ALL):
    return pltpu.bitcast(ref[r0 // 2:r1 // 2, cols], bf16)


def _st(ref, r0, r1, cols, val):
    ref[r0 // 2:r1 // 2, cols] = pltpu.bitcast(val, u32)


def _rcp(x):
    r = pl.reciprocal(x, approx=True)
    return r * (2.0 - x * r)


def _heads(v, op):
    r = v[0]
    for j in range(1, 8):
        r = op(r, v[j])
    r = op(r, pltpu.roll(r, 4, 0))
    return op(r, pltpu.roll(r, 2, 0))


def _feat(p):
    outs = []
    for h in range(2):
        ph = p[h * 64:(h + 1) * 64].reshape(8, 8, p.shape[1])
        e1 = jnp.exp2(ph - _heads(ph, jnp.maximum)[None])
        e2 = jnp.exp2(_heads(ph, jnp.minimum)[None] - ph)
        for e in (e1, e2):
            outs.append((e * _rcp(_heads(e, jnp.add))[None]).reshape(64, p.shape[1]))
    return jnp.concatenate(outs, axis=0)


def _left(a11, a12, a21, a22):
    return (a11 + a22, a21 + a22, a11, a22, a11 + a12, a21 - a11, a12 - a22)


def _right(k, b11, b12, b21, b22):
    if k == 1:
        return b11()
    if k == 4:
        return b22()
    p, q, sub = {0: (b11, b22, False), 2: (b12, b22, True), 3: (b21, b11, True),
                 5: (b11, b12, False), 6: (b21, b22, False)}[k]
    p, q = p().astype(f32), q().astype(f32)
    return (p - q if sub else p + q).astype(bf16)


def _kernel(x_hbm, wqkv_hbm, wphi_hbm, wo_hbm, wr_hbm, wg_hbm, wu_hbm, wd_hbm, gw_hbm,
            out_hbm,
            x_v, wraw_v, wphi_v, wo_v, wr_v, gw_v, wg_v, wu_v, wd_v,
            sq_v, skv_v, xt_v, wot_v, phiq_v, acc_v, kvz_v, out_v, out0_v, xcol_v, gate_v, bd_v, rg_v, h_v,
            sems):
    cp = pltpu.make_async_copy
    c_wphi = cp(wphi_hbm, wphi_v, sems.at[0])
    c_wr = cp(wr_hbm, wr_v, sems.at[9])
    c_gw = cp(gw_hbm, gw_v, sems.at[9])
    wsem = lambda j, g: 1 + g // 2 if j else (5, 9)[g // 4]
    c_w = [[cp(wqkv_hbm.at[:, pl.ds(j * D + g * 128, 128)], wraw_v[j][g].bitcast(bf16), sems.at[wsem(j, g)])
            for g in range(NG)] for j in range(3)]
    c_x = [cp(x_hbm.at[pl.ds(i * T, T)], x_v[i].bitcast(bf16), sems.at[(1, 5, 9, 6)[min(i, 3)]])
           for i in range(NC)]
    c_gu = [cp(w.at[:, pl.ds(j * FC, FC)], v[j].bitcast(bf16), sems.at[6 if j < GU0 else 7])
            for j in range(NF) for w, v in ((wg_hbm, wg_v), (wu_hbm, wu_v))]
    c_d = [cp(wd_hbm.at[pl.ds(j * FC, FC)], wd_v[j].bitcast(bf16), sems.at[8]) for j in range(NF)]
    c_d.append(cp(wo_hbm, wo_v.bitcast(bf16), sems.at[8]))
    c_o = [cp(out_v[i - 1].bitcast(bf16), out_hbm.at[pl.ds(i * T, T)], sems.at[2]) for i in range(1, NC)]
    c_o0 = {(t, c): cp(out0_v[t][c].bitcast(bf16), out_hbm.at[pl.ds(t * 128, 128), pl.ds(c * HD, HD)], sems.at[2])
            for t in range(2) for c in range(2)}

    for d in [c_wphi, c_w[1][0], c_w[1][1], c_w[2][0], c_w[2][1], c_x[0]]:
        d.start()
    for g in range(2, NG):
        c_w[1][g].start()
        c_w[2][g].start()
    for d in [c_x[1]] + c_w[0][:4] + [c_wr, c_gw] + c_w[0][4:] + c_x[2:] + c_gu + c_d:
        d.start()

    row = lax.broadcasted_iota(jnp.int32, (128, 128), 0)
    col = lax.broadcasted_iota(jnp.int32, (128, 128), 1)
    diag = (row // DH) == (col // 64) * 2 + col % 2
    rep = (((lax.broadcasted_iota(jnp.int32, (DH, 128), 1) % 64) // 2)
           == lax.broadcasted_iota(jnp.int32, (DH, 128), 0)).astype(bf16)
    acc_v[...] = jnp.zeros_like(acc_v)
    ones = jnp.ones((16, T), bf16)
    c_wphi.wait()
    for g in range(NG):
        wt = jnp.dot(wphi_v[g * 128:(g + 1) * 128, :], rep, preferred_element_type=f32)
        _st(bd_v, g * 128, (g + 1) * 128, ALL, jnp.where(diag, wt, 0.0).T.astype(bf16))

    def prep(j, pp):
        w = []
        for g in (2 * pp, 2 * pp + 1):
            raw = _ld(wraw_v[j][g], 0, D)
            if j < 2:
                w.append(lax.dot_general(_ld(bd_v, g * 128, (g + 1) * 128), raw, NT,
                                         preferred_element_type=f32) * LOG2E)
            else:
                w.append(raw.T.astype(f32))
        dst, r0 = (sq_v, 0) if j == 0 else (skv_v, (j - 1) * 128)
        for k, s in enumerate(_left(w[0][:, :HD], w[0][:, HD:], w[1][:, :HD], w[1][:, HD:])):
            _st(dst[pp][k], r0, r0 + 128, ALL, s.astype(bf16))

    st = {"n": 0}

    def tie(a, dep):
        if dep is None:
            return a
        if a.dtype == f32:
            blk = jnp.where(st["never"], dep, a[0:8])
            return jnp.concatenate([blk, a[8:]], axis=0) if a.shape[0] > 8 else blk
        blk = pltpu.bitcast(jnp.where(st["never"], dep, pltpu.bitcast(a[0:16, 0:128], f32)), bf16)
        if a.shape[1] > 128:
            blk = jnp.concatenate([blk, a[0:16, 128:]], axis=1)
        return jnp.concatenate([blk, a[16:]], axis=0)

    def xright(i, k, fresh):
        blk = lambda r, c: (lambda: _ld(x_v[i], r * 128, (r + 1) * 128, slice(c * HD, (c + 1) * HD)))
        if k in (1, 4) or fresh:
            val = _right(k, blk(0, 0), blk(1, 0), blk(0, 1), blk(1, 1))
            if k not in (1, 4):
                _st(xt_v[i], k * 128, (k + 1) * 128, ALL, val)
            return val
        return _ld(xt_v[i], k * 128, (k + 1) * 128)

    jobs = {}
    after = {}
    ties = {}

    def project(lhs, i, fresh, use, mid):
        def m(k):
            n = st["n"]
            st["n"] = n + 1
            out = lax.dot_general(tie(lhs(k), ties.pop(n, None)), xright(i, k, fresh), NT,
                                  preferred_element_type=f32)
            if n in after:
                after.pop(n)()
            if n in jobs:
                res = jobs.pop(n)(out[0:8])
                if res is not None and n + LAG < NDOT:
                    ties[n + LAG] = res
            return out
        m5 = m(4)
        late()
        m3 = m(2)
        m2 = m(1)
        use(0, 1, m3 + m5)
        mid()
        m4 = m(3)
        m1 = m(0)
        use(1, 0, m2 + m4)
        c11 = m1 + m4 - m5
        c22 = m1 - m2 + m3
        c11 = c11 + m(6)
        m6 = m(5)
        use(0, 0, c11)
        st["late"] = lambda: use(1, 1, c22 + m6)

    def late():
        st.pop("late", lambda: None)()

    pend = []

    def feat_k(g, p):
        fk = _feat(p)
        return fk.astype(bf16)

    def kv_flush():
        for g, fk, vt in pend:
            fk = jnp.concatenate(fk, axis=1)
            vt = jnp.concatenate(vt, axis=1)
            for p in range(2):
                lhs = jnp.concatenate([vt[p * 64:(p + 1) * 64], ones], axis=0)
                acc_v[2 * g + p] += lax.dot_general(lhs, fk[p * 128:(p + 1) * 128], NT,
                                                    preferred_element_type=f32)
        pend.clear()

    def router(i, part, dep):
        best, bidx = st["best"], st["bidx"]
        for b in range(part * 4, part * 4 + 4):
            rows = slice(b * 16, (b + 1) * 16)
            xf = [_ld(x_v[i], b * 16, (b + 1) * 16, slice(k * 128, (k + 1) * 128)).astype(f32)
                  for k in range(D // 128)]
            acc = []
            for w in range(2):
                for hf in range(2):
                    a = None
                    for k in range(D // 128):
                        p = xf[k][hf * 8:(hf + 1) * 8] * rg_v[w * 8:(w + 1) * 8, k * 128:(k + 1) * 128]
                        a = tie(p, dep) if k == 0 else a + p
                    acc.append(a)
                    dep = a
            ra, ga = jnp.concatenate(acc[0:2], axis=0), jnp.concatenate(acc[2:4], axis=0)
            r = jnp.sum(ra, axis=1, keepdims=True).astype(bf16).astype(f32)
            gate_v[i, rows, :] = jnp.broadcast_to(jnp.sum(ga, axis=1, keepdims=True), (16, 128))
            r = jnp.broadcast_to(r, (16, 128))
            for k in range(2):
                rk = r[k * 8:(k + 1) * 8]
                if best is None:
                    best, bidx = rk, jnp.zeros((8, 128), jnp.int32)
                else:
                    better = rk > best
                    best = jnp.where(better, rk, best)
                    bidx = jnp.where(better, i * T + b * 16 + k * 8, bidx)
        st["best"], st["bidx"] = best, bidx
        return dep

    def select():
        best, bidx = st["best"], st["bidx"]
        m = jnp.max(best, axis=0, keepdims=True)
        cand = jnp.where(best == m, bidx + lax.broadcasted_iota(jnp.int32, (8, 128), 0), S - 1)
        idxv = jnp.min(cand, axis=0, keepdims=True)
        idx = idxv[0, 0]
        st["idxv"] = idxv
        st["rs"] = jax.nn.sigmoid(m)
        base = pl.multiple_of(((idx % T) // 16) * 8, 8)
        tile = x_v[0][pl.ds(base, 8), :]
        for i in range(1, NC):
            tile = jnp.where(idx // T == i, x_v[i][pl.ds(base, 8), :], tile)
        tile = pltpu.bitcast(tile, bf16).astype(f32)
        sel = lax.broadcasted_iota(jnp.int32, (16, D), 0) == (idx % 16)
        xs = jnp.sum(jnp.where(sel, tile, 0.0), axis=0, keepdims=True)
        for k in range(D // 128):
            xcol_v[k * 128:(k + 1) * 128, :] = jnp.broadcast_to(xs[:, k * 128:(k + 1) * 128], (128, 128)).T
        st["y"] = [None] * (D // 128)

    def chain(w_ref, r0, nblk, cols, col_of, dep):
        acc = None
        for k in range(nblk):
            p = _ld(w_ref, r0 + k * 16, r0 + (k + 1) * 16, cols).astype(f32) * col_of(k)
            acc = tie(p[0:8], dep) if acc is None else acc + p[0:8]
            acc = acc + p[8:16]
        return acc

    def ffn_in(w, c, dep):
        j, cc = divmod(c, FC // 128)
        acc = chain((wg_v, wu_v)[w][j], 0, D // 16, slice(cc * 128, (cc + 1) * 128),
                    lambda k: xcol_v[k * 16:(k + 1) * 16, :], dep)
        v = jnp.sum(acc, axis=0, keepdims=True)
        if w == 0:
            st["g", c] = v * jax.nn.sigmoid(v)
        else:
            h_v[c] = jnp.broadcast_to(st.pop(("g", c)) * v, (8, 128))
        return acc

    def ffn_down(c, dep):
        j, cc = divmod(c, FC // 128)
        hcol = jnp.concatenate([h_v[c]] * 16, axis=0).T
        ys = st["y"]
        for n in range(D // 128):
            dep = chain(wd_v[j], cc * 128, 128 // 16, slice(n * 128, (n + 1) * 128),
                        lambda k: hcol[k * 16:(k + 1) * 16], dep)
            ys[n] = dep if ys[n] is None else ys[n] + dep
        return dep

    def wo_right(k):
        blk = lambda r, c: (lambda: _ld(wo_v, r * HD, (r + 1) * HD, slice(c * HD, (c + 1) * HD)))
        return _right(k, blk(0, 0), blk(0, 1), blk(1, 0), blk(1, 1))

    def wo_job(r, e, dep):
        def blk(a, b):
            r0, c0 = b * HD + e * 128, a * HD + r * 128
            return _ld(wo_v, r0, r0 + 128, slice(c0, c0 + 128)).T.astype(f32)
        for k, v in enumerate(_left(blk(0, 0), blk(0, 1), blk(1, 0), blk(1, 1))):
            _st(wot_v, k * HD + r * 128, k * HD + (r + 1) * 128, slice(e * 128, (e + 1) * 128), v.astype(bf16))
            dep = jnp.maximum(dep, v[120:128])
        return dep

    def wait_kv(pp):
        for g in (2 * pp, 2 * pp + 1):
            c_w[1][g].wait()
            c_w[2][g].wait()
        if pp == 0:
            c_x[0].wait()
        prep(1, pp)
        prep(2, pp)

    def wait_q(half):
        for d in [c_x[1 + half]] + c_w[0][4 * half:4 * half + 4] + [c_wr, c_gw][:2 * half]:
            d.wait()
        prep(0, 2 * half)
        if half:
            wr = wr_v[...].reshape(1, D).astype(f32)
            rg_v[0:8, :] = jnp.broadcast_to(wr, (8, D))
            rg_v[8:16, :] = jnp.broadcast_to(gw_v[...].reshape(1, D).astype(f32), (8, D))
            st["best"] = st["bidx"] = None
            st["never"] = jnp.broadcast_to((pltpu.bitcast(wr[:, 0:128], jnp.int32) | 1) == 0, (8, 128))

    def wait_all(ds):
        for d in ds:
            d.wait()

    for pp in range(1, NP):
        after[7 * pp - 1] = functools.partial(wait_kv, pp)
    after[27] = functools.partial(wait_q, 0)
    after[34] = functools.partial(prep, 0, 1)
    after[41] = functools.partial(wait_q, 1)
    after[48] = functools.partial(prep, 0, 3)
    after[83] = functools.partial(wait_all, c_x[3:] + c_gu[:2 * GU0])
    for r in range(4 * NC):
        jobs[56 + 2 * r if r < 12 else 72 + r] = functools.partial(router, r // 4, r % 4)
    jobs[106] = lambda dep: select()
    n0 = 8 * GU0
    for u in range(2 * NB):
        pos = 111 + (u * (W1 - LAG - 111)) // n0 if u < n0 else W1 + 1 + ((u - n0) * (W2 - LAG - W1)) // (2 * NB - n0)
        assert pos not in jobs
        jobs[pos] = functools.partial(ffn_in, u % 2, u // 2)
    after[W1] = functools.partial(wait_all, c_gu[2 * GU0:])
    after[W2] = functools.partial(wait_all, c_d)
    tail = sorted([(c / NB, functools.partial(ffn_down, c)) for c in range(NB)]
                  + [((w + 0.5) / 16, functools.partial(wo_job, w // 4, w % 4)) for w in range(16)], key=lambda e: e[0])
    for pos, (_, job) in enumerate(tail):
        jobs[W2 + 1 + pos] = job

    wait_kv(0)
    for i, pp in [(i, pp) for i in range(NC) for pp in range(NP)]:
        new = [(2 * pp + a, [None, None], [None, None]) for a in range(2)]

        def use(a, t, c, new=new, i=i, pp=pp):
            g = 2 * pp + a
            if i >= 1:
                _st(phiq_v[i], g * 256, (g + 1) * 256, slice(t * 128, (t + 1) * 128), _feat(c[0:128]).astype(bf16))
            new[a][1][t] = feat_k(g, c[-256:-128])
            new[a][2][t] = c[-128:].astype(bf16)

        def lhs(k, i=i, pp=pp):
            kvw = _ld(skv_v[pp][k], 0, 256)
            return jnp.concatenate([_ld(sq_v[pp][k], 0, 128), kvw], axis=0) if i >= 1 else kvw

        project(lhs, i, pp == 0, use, kv_flush)
        pend.extend(new)

    def finalize():
        if pend:
            kv_flush()
            r80 = lax.broadcasted_iota(jnp.int32, (80, 128), 0)
            c80 = lax.broadcasted_iota(jnp.int32, (80, 128), 1)
            keep = jnp.where(r80 < 64, r80 // 32, (r80 - 64) // 8) == (c80 % 2)
            for p in range(2 * NG):
                kvz = acc_v[p]
                _st(kvz_v, p * 80, (p + 1) * 80, ALL, jnp.where(keep, kvz, 0.0).astype(bf16))

    for i, q in ((0, 0), (0, 1)):
        def use(a, t, c, i=i, q=q):
            for e in range(2):
                g = 2 * (2 * q + e) + a
                _st(phiq_v[i], g * 256, (g + 1) * 256, slice(t * 128, (t + 1) * 128),
                    _feat(c[e * 128:(e + 1) * 128]).astype(bf16))

        project(lambda k, q=q: jnp.concatenate([_ld(sq_v[2 * q][k], 0, 128), _ld(sq_v[2 * q + 1][k], 0, 128)], axis=0),
                i, False, use, finalize)

    late()
    yrow = jnp.concatenate([jnp.sum(y, axis=0, keepdims=True) * st["rs"] for y in st["y"]], axis=1)

    def attn(i, dep):
        ot = []
        for p in range(2 * NG):
            nd = jnp.dot(tie(_ld(kvz_v, p * 80, (p + 1) * 80), dep), _ld(phiq_v[i], p * 128, (p + 1) * 128),
                         preferred_element_type=f32)
            for a in range(2):
                rden = _rcp(nd[64 + 8 * a:72 + 8 * a] + 1e-6)
                o = nd[32 * a:32 * a + 32].reshape(4, 8, T) * rden[None]
                ot.append(o.reshape(32, T))
        ot = jnp.concatenate(ot, axis=0)
        b11, b12, b21, b22 = ot[:HD, :128], ot[:HD, 128:], ot[HD:, :128], ot[HD:, 128:]
        return [s.astype(bf16) for s in (b11 + b22, b11, b12 - b22, b21 - b11, b22, b11 + b12, b21 + b22)]

    def finish(i, o, nxt):
        def m(k):
            return jnp.dot(_ld(wot_v, k * HD, (k + 1) * HD), o[k], preferred_element_type=f32)

        def mix(c, t, a):
            a = a.T
            rows = slice(t * 128, (t + 1) * 128)
            gate = jax.nn.sigmoid(gate_v[i, rows, :])
            omg = 1.0 - gate
            hit = (lax.broadcasted_iota(jnp.int32, (128, 128), 0) + (i * T + t * 128)) == st["idxv"]
            for k in range(HD // 128):
                ks = slice(c * HD + k * 128, c * HD + (k + 1) * 128)
                xb = _ld(x_v[i], t * 128, (t + 1) * 128, ks).astype(f32)
                b = xb + (xb * 0.0 + jnp.where(hit, yrow[:, ks], 0.0))
                res = (gate * a[:, k * 128:(k + 1) * 128] + omg * b).astype(bf16)
                if i:
                    _st(out_v[i - 1], t * 128, (t + 1) * 128, ks, res)
                else:
                    _st(out0_v[t][c], 0, 128, slice(k * 128, (k + 1) * 128), res)
            if i == 0:
                c_o0[t, c].start()

        m5 = m(4)
        o_next = None if nxt is None else attn(nxt, None)
        m3 = m(2)
        mix(0, 1, m3 + m5)
        m2 = m(1)
        m4 = m(3)
        mix(1, 0, m2 + m4)
        m1 = m(0)
        c11 = m1 + m4 - m5
        c22 = m1 - m2 + m3
        mix(0, 0, c11 + m(6))
        mix(1, 1, c22 + m(5))
        if i:
            c_o[i - 1].start()
        return o_next

    order = list(range(1, NC)) + [0]
    o = attn(order[0], None)
    for n, i in enumerate(order):
        o = finish(i, o, order[n + 1] if n + 1 < NC else None)
    for d in c_o + list(c_o0.values()):
        d.wait()


@jax.jit
def pallas_gated_mix__linear_kernel_hedgehog__moe_arch_mod__prompt_kernel(A_x, A_wqkv, A_w_phi, A_wo, B_x, B_w_r, B_w_gate, B_w_up, B_w_down, gate_w):
    anyspec = pl.BlockSpec(memory_space=pl.ANY)
    V = pltpu.VMEM
    P = lambda r, c: V((r // 2, c), u32)
    out = pl.pallas_call(
        _kernel,
        out_shape=jax.ShapeDtypeStruct((S, D), bf16),
        in_specs=[anyspec] * 9,
        out_specs=anyspec,
        scratch_shapes=[
            [P(T, D) for _ in range(NC)],
            [[P(D, 128) for _ in range(NG)] for _ in range(3)],
            V((D, DH), bf16), P(D, D), V((D,), bf16), V((D,), bf16),
            [P(D, FC) for _ in range(NF)], [P(D, FC) for _ in range(NF)], [P(FC, D) for _ in range(NF)],
            [[P(128, HD) for _ in range(7)] for _ in range(NP)],
            [[P(256, HD) for _ in range(7)] for _ in range(NP)],
            [P(7 * 128, HD) for _ in range(NC)], P(7 * HD, HD),
            [P(2 * D, T) for _ in range(NC)],
            V((2 * NG, 80, 128), f32), P(2 * NG * 80, 128),
            [P(T, D) for _ in range(NC - 1)], [[P(128, HD) for _ in range(2)] for _ in range(2)],
            V((D, 128), f32), V((NC, T, 128), f32), P(NG * 128, 128), V((16, D), f32), V((NB, 8, 128), f32),
            pltpu.SemaphoreType.DMA((10,)),
        ],
        compiler_params=pltpu.CompilerParams(vmem_limit_bytes=120 * 2**20),
    )(A_x.reshape(S, D), A_wqkv, A_w_phi.reshape(D, DH), A_wo,
      B_w_r, B_w_gate, B_w_up, B_w_down, gate_w)
    return out.reshape(1, S, D)
```

```python
import functools

import jax
import jax.numpy as jnp
import numpy as np
from jax import lax
import jax.experimental.pallas as pl
import jax.experimental.pallas.tpu as pltpu

S, D, H, DH, F = 2048, 1024, 32, 32, 3584
T = 256
NC = S // T
NG = 8
NP = NG // 2
HD = D // 2
FC = 512
NF = F // FC
NB = F // 128
NDOT = 28 * NC + 14
LAG = 4
GU0 = 2
W1, W2 = 143, 190
f32, bf16, u32 = jnp.float32, jnp.bfloat16, jnp.uint32
NT = (((1,), (1,)), ((), ()))
LOG2E = 1.4426950408889634
ALL = slice(None)


def _ld(ref, r0, r1, cols=ALL):
    return pltpu.bitcast(ref[r0 // 2:r1 // 2, cols], bf16)


def _st(ref, r0, r1, cols, val):
    ref[r0 // 2:r1 // 2, cols] = pltpu.bitcast(val, u32)


def _rcp(x):
    r = pl.reciprocal(x, approx=True)
    return r * (2.0 - x * r)


def _heads(v, op):
    r = v[0]
    for j in range(1, v.shape[0]):
        r = op(r, v[j])
    r = op(r, pltpu.roll(r, 4, 0))
    return op(r, pltpu.roll(r, 2, 0))


def _feat(p):
    outs = []
    for h in range(2):
        ph = p[h * 64:(h + 1) * 64].reshape(8, 8, p.shape[1])
        e1 = jnp.exp2(ph - _heads(ph, jnp.maximum)[None])
        e2 = jnp.exp2(_heads(ph, jnp.minimum)[None] - ph)
        for e in (e1, e2):
            outs.append((e * _rcp(_heads(e, jnp.add))[None]).reshape(64, p.shape[1]))
    return jnp.concatenate(outs, axis=0)


def _left(a11, a12, a21, a22):
    return (a11 + a22, a21 + a22, a11, a22, a11 + a12, a21 - a11, a12 - a22)


def _right(k, b11, b12, b21, b22):
    if k == 1:
        return b11()
    if k == 4:
        return b22()
    p, q, sub = {0: (b11, b22, False), 2: (b12, b22, True), 3: (b21, b11, True),
                 5: (b11, b12, False), 6: (b21, b22, False)}[k]
    p, q = p().astype(f32), q().astype(f32)
    return (p - q if sub else p + q).astype(bf16)


def _kernel(x_hbm, wqkv_hbm, wphi_hbm, wo_hbm, wr_hbm, wg_hbm, wu_hbm, wd_hbm, gw_hbm,
            out_hbm,
            x_v, wraw_v, wphi_v, wo_v, wr_v, gw_v, wg_v, wu_v, wd_v,
            sq_v, skv_v, xt_v, wot_v, phiq_v, acc_v, kvz_v, zc_v, out_v, out0_v, xcol_v, gate_v, bd_v, rg_v, h_v,
            sems):
    cp = pltpu.make_async_copy
    c_wphi = cp(wphi_hbm, wphi_v, sems.at[0])
    c_wr = cp(wr_hbm, wr_v, sems.at[9])
    c_gw = cp(gw_hbm, gw_v, sems.at[9])
    wsem = lambda j, g: 1 + g // 2 if j else (5, 9)[g // 4]
    c_w = [[cp(wqkv_hbm.at[:, pl.ds(j * D + g * 128, 128)], wraw_v[j][g].bitcast(bf16), sems.at[wsem(j, g)])
            for g in range(NG)] for j in range(3)]
    c_x = [cp(x_hbm.at[pl.ds(i * T, T)], x_v[i].bitcast(bf16), sems.at[(1, 5, 9, 6)[min(i, 3)]])
           for i in range(NC)]
    c_gu = [cp(w.at[:, pl.ds(j * FC, FC)], v[j].bitcast(bf16), sems.at[6 if j < GU0 else 7])
            for j in range(NF) for w, v in ((wg_hbm, wg_v), (wu_hbm, wu_v))]
    c_d = [cp(wd_hbm.at[pl.ds(j * FC, FC)], wd_v[j].bitcast(bf16), sems.at[8]) for j in range(NF)]
    c_d.append(cp(wo_hbm, wo_v.bitcast(bf16), sems.at[8]))
    c_o = [cp(out_v[i - 1].bitcast(bf16), out_hbm.at[pl.ds(i * T, T)], sems.at[2]) for i in range(1, NC)]
    c_o0 = {(t, c): cp(out0_v[t][c].bitcast(bf16), out_hbm.at[pl.ds(t * 128, 128), pl.ds(c * HD, HD)], sems.at[2])
            for t in range(2) for c in range(2)}

    for d in [c_wphi, c_w[1][0], c_w[1][1], c_w[2][0], c_w[2][1], c_x[0]]:
        d.start()
    for g in range(2, NG):
        c_w[1][g].start()
        c_w[2][g].start()
    for d in [c_x[1]] + c_w[0][:4] + [c_wr, c_gw] + c_w[0][4:] + c_x[2:] + c_gu + c_d:
        d.start()

    row = lax.broadcasted_iota(jnp.int32, (128, 128), 0)
    col = lax.broadcasted_iota(jnp.int32, (128, 128), 1)
    diag = (row // DH) == (col // 64) * 2 + col % 2
    rep = (((lax.broadcasted_iota(jnp.int32, (DH, 128), 1) % 64) // 2)
           == lax.broadcasted_iota(jnp.int32, (DH, 128), 0)).astype(bf16)
    acc_v[...] = jnp.zeros_like(acc_v)
    ones = jnp.ones((16, T), bf16)
    c_wphi.wait()
    for g in range(NG):
        wt = jnp.dot(wphi_v[g * 128:(g + 1) * 128, :], rep, preferred_element_type=f32)
        _st(bd_v, g * 128, (g + 1) * 128, ALL, jnp.where(diag, wt, 0.0).T.astype(bf16))

    def prep(j, pp):
        w = []
        for g in (2 * pp, 2 * pp + 1):
            raw = _ld(wraw_v[j][g], 0, D)
            if j < 2:
                w.append(lax.dot_general(_ld(bd_v, g * 128, (g + 1) * 128), raw, NT,
                                         preferred_element_type=f32) * LOG2E)
            else:
                w.append(raw.T.astype(f32))
        dst, r0 = (sq_v, 0) if j == 0 else (skv_v, (j - 1) * 128)
        for k, s in enumerate(_left(w[0][:, :HD], w[0][:, HD:], w[1][:, :HD], w[1][:, HD:])):
            _st(dst[pp][k], r0, r0 + 128, ALL, s.astype(bf16))

    st = {"n": 0}

    def tie(a, dep):
        if dep is None:
            return a
        if a.dtype == f32:
            blk = jnp.where(st["never"], dep, a[0:8])
            return jnp.concatenate([blk, a[8:]], axis=0) if a.shape[0] > 8 else blk
        blk = pltpu.bitcast(jnp.where(st["never"], dep, pltpu.bitcast(a[0:16, 0:128], f32)), bf16)
        if a.shape[1] > 128:
            blk = jnp.concatenate([blk, a[0:16, 128:]], axis=1)
        return jnp.concatenate([blk, a[16:]], axis=0)

    def xright(i, k, fresh):
        blk = lambda r, c: (lambda: _ld(x_v[i], r * 128, (r + 1) * 128, slice(c * HD, (c + 1) * HD)))
        if k in (1, 4) or fresh:
            val = _right(k, blk(0, 0), blk(1, 0), blk(0, 1), blk(1, 1))
            if k not in (1, 4):
                _st(xt_v[i], k * 128, (k + 1) * 128, ALL, val)
            return val
        return _ld(xt_v[i], k * 128, (k + 1) * 128)

    jobs = {}
    after = {}
    ties = {}

    def project(lhs, i, fresh, use, mid):
        def m(k):
            n = st["n"]
            st["n"] = n + 1
            out = lax.dot_general(tie(lhs(k), ties.pop(n, None)), xright(i, k, fresh), NT,
                                  preferred_element_type=f32)
            if n in after:
                after.pop(n)()
            if n in jobs:
                res = jobs.pop(n)(out[0:8])
                if res is not None and n + LAG < NDOT:
                    ties[n + LAG] = res
            return out
        m5 = m(4)
        late()
        m3 = m(2)
        m2 = m(1)
        use(0, 1, m3 + m5)
        mid()
        m4 = m(3)
        m1 = m(0)
        use(1, 0, m2 + m4)
        c11 = m1 + m4 - m5
        c22 = m1 - m2 + m3
        c11 = c11 + m(6)
        m6 = m(5)
        use(0, 0, c11)
        st["late"] = lambda: use(1, 1, c22 + m6)

    def late():
        st.pop("late", lambda: None)()

    pend = []

    def feat_k(g, p):
        fk = _feat(p)
        return fk.astype(bf16)

    def kv_flush():
        for g, fk, vt in pend:
            fk = jnp.concatenate(fk, axis=1)
            vt = jnp.concatenate(vt, axis=1)
            for p in range(2):
                lhs = jnp.concatenate([vt[p * 64:(p + 1) * 64], ones], axis=0)
                acc_v[2 * g + p] += lax.dot_general(lhs, fk[p * 128:(p + 1) * 128], NT,
                                                    preferred_element_type=f32)
        pend.clear()

    def router(i, part, dep):
        best, bidx = st["best"], st["bidx"]
        for b in range(part * 4, part * 4 + 4):
            rows = slice(b * 16, (b + 1) * 16)
            xf = [_ld(x_v[i], b * 16, (b + 1) * 16, slice(k * 128, (k + 1) * 128)).astype(f32)
                  for k in range(D // 128)]
            acc = []
            for w in range(2):
                for hf in range(2):
                    a = None
                    for k in range(D // 128):
                        p = xf[k][hf * 8:(hf + 1) * 8] * rg_v[w * 8:(w + 1) * 8, k * 128:(k + 1) * 128]
                        a = tie(p, dep) if k == 0 else a + p
                    acc.append(a)
                    dep = a
            ra, ga = jnp.concatenate(acc[0:2], axis=0), jnp.concatenate(acc[2:4], axis=0)
            r = jnp.sum(ra, axis=1, keepdims=True).astype(bf16).astype(f32)
            gate_v[i, rows, :] = jnp.broadcast_to(jnp.sum(ga, axis=1, keepdims=True), (16, 128))
            r = jnp.broadcast_to(r, (16, 128))
            for k in range(2):
                rk = r[k * 8:(k + 1) * 8]
                if best is None:
                    best, bidx = rk, jnp.zeros((8, 128), jnp.int32)
                else:
                    better = rk > best
                    best = jnp.where(better, rk, best)
                    bidx = jnp.where(better, i * T + b * 16 + k * 8, bidx)
        st["best"], st["bidx"] = best, bidx
        return dep

    def select():
        best, bidx = st["best"], st["bidx"]
        m = jnp.max(best, axis=0, keepdims=True)
        cand = jnp.where(best == m, bidx + lax.broadcasted_iota(jnp.int32, (8, 128), 0), S - 1)
        idxv = jnp.min(cand, axis=0, keepdims=True)
        idx = idxv[0, 0]
        st["idxv"] = idxv
        st["rs"] = jax.nn.sigmoid(m)
        base = pl.multiple_of(((idx % T) // 16) * 8, 8)
        tile = x_v[0][pl.ds(base, 8), :]
        for i in range(1, NC):
            tile = jnp.where(idx // T == i, x_v[i][pl.ds(base, 8), :], tile)
        tile = pltpu.bitcast(tile, bf16).astype(f32)
        sel = lax.broadcasted_iota(jnp.int32, (16, D), 0) == (idx % 16)
        xs = jnp.sum(jnp.where(sel, tile, 0.0), axis=0, keepdims=True)
        for k in range(D // 128):
            xcol_v[k * 128:(k + 1) * 128, :] = jnp.broadcast_to(xs[:, k * 128:(k + 1) * 128], (128, 128)).T
        st["y"] = [None] * (D // 128)

    def chain(w_ref, r0, nblk, cols, col_of, dep):
        acc = None
        for k in range(nblk):
            p = _ld(w_ref, r0 + k * 16, r0 + (k + 1) * 16, cols).astype(f32) * col_of(k)
            acc = tie(p[0:8], dep) if acc is None else acc + p[0:8]
            acc = acc + p[8:16]
        return acc

    def ffn_in(w, c, dep):
        j, cc = divmod(c, FC // 128)
        acc = chain((wg_v, wu_v)[w][j], 0, D // 16, slice(cc * 128, (cc + 1) * 128),
                    lambda k: xcol_v[k * 16:(k + 1) * 16, :], dep)
        v = jnp.sum(acc, axis=0, keepdims=True)
        if w == 0:
            st["g", c] = v * jax.nn.sigmoid(v)
        else:
            h_v[c] = jnp.broadcast_to(st.pop(("g", c)) * v, (8, 128))
        return acc

    def ffn_down(c, dep):
        j, cc = divmod(c, FC // 128)
        hcol = jnp.concatenate([h_v[c]] * 16, axis=0).T
        ys = st["y"]
        for n in range(D // 128):
            dep = chain(wd_v[j], cc * 128, 128 // 16, slice(n * 128, (n + 1) * 128),
                        lambda k: hcol[k * 16:(k + 1) * 16], dep)
            ys[n] = dep if ys[n] is None else ys[n] + dep
        return dep

    def wo_right(k):
        blk = lambda r, c: (lambda: _ld(wo_v, r * HD, (r + 1) * HD, slice(c * HD, (c + 1) * HD)))
        return _right(k, blk(0, 0), blk(0, 1), blk(1, 0), blk(1, 1))

    def wo_job(r, e, dep):
        def blk(a, b):
            r0, c0 = b * HD + e * 128, a * HD + r * 128
            return _ld(wo_v, r0, r0 + 128, slice(c0, c0 + 128)).T.astype(f32)
        for k, v in enumerate(_left(blk(0, 0), blk(0, 1), blk(1, 0), blk(1, 1))):
            _st(wot_v, k * HD + r * 128, k * HD + (r + 1) * 128, slice(e * 128, (e + 1) * 128), v.astype(bf16))
            dep = jnp.maximum(dep, v[120:128])
        return dep

    def wait_kv(pp):
        for g in (2 * pp, 2 * pp + 1):
            c_w[1][g].wait()
            c_w[2][g].wait()
        if pp == 0:
            c_x[0].wait()
        prep(1, pp)
        prep(2, pp)

    def wait_q(half):
        for d in [c_x[1 + half]] + c_w[0][4 * half:4 * half + 4] + [c_wr, c_gw][:2 * half]:
            d.wait()
        prep(0, 2 * half)
        if half:
            wr = wr_v[...].reshape(1, D).astype(f32)
            rg_v[0:8, :] = jnp.broadcast_to(wr, (8, D))
            rg_v[8:16, :] = jnp.broadcast_to(gw_v[...].reshape(1, D).astype(f32), (8, D))
            st["best"] = st["bidx"] = None
            st["never"] = jnp.broadcast_to((pltpu.bitcast(wr[:, 0:128], jnp.int32) | 1) == 0, (8, 128))

    def wait_all(ds):
        for d in ds:
            d.wait()

    for pp in range(1, NP):
        after[7 * pp - 1] = functools.partial(wait_kv, pp)
    after[27] = functools.partial(wait_q, 0)
    after[34] = functools.partial(prep, 0, 1)
    after[41] = functools.partial(wait_q, 1)
    after[48] = functools.partial(prep, 0, 3)
    after[83] = functools.partial(wait_all, c_x[3:] + c_gu[:2 * GU0])
    for r in range(4 * NC):
        jobs[56 + 2 * r if r < 12 else 72 + r] = functools.partial(router, r // 4, r % 4)
    jobs[106] = lambda dep: select()
    n0 = 8 * GU0
    for u in range(2 * NB):
        pos = 111 + (u * (W1 - LAG - 111)) // n0 if u < n0 else W1 + 1 + ((u - n0) * (W2 - LAG - W1)) // (2 * NB - n0)
        assert pos not in jobs
        jobs[pos] = functools.partial(ffn_in, u % 2, u // 2)
    after[W1] = functools.partial(wait_all, c_gu[2 * GU0:])
    after[W2] = functools.partial(wait_all, c_d)
    tail = sorted([(c / NB, functools.partial(ffn_down, c)) for c in range(NB)]
                  + [((w + 0.5) / 16, functools.partial(wo_job, w // 4, w % 4)) for w in range(16)], key=lambda e: e[0])
    for pos, (_, job) in enumerate(tail):
        jobs[W2 + 1 + pos] = job

    wait_kv(0)
    for i, pp in [(i, pp) for i in range(NC) for pp in range(NP)]:
        new = [(2 * pp + a, [None, None], [None, None]) for a in range(2)]

        def use(a, t, c, new=new, i=i, pp=pp):
            g = 2 * pp + a
            if i >= 1:
                _st(phiq_v[i], g * 256, (g + 1) * 256, slice(t * 128, (t + 1) * 128), _feat(c[0:128]).astype(bf16))
            new[a][1][t] = feat_k(g, c[-256:-128])
            new[a][2][t] = c[-128:].astype(bf16)

        def lhs(k, i=i, pp=pp):
            kvw = _ld(skv_v[pp][k], 0, 256)
            return jnp.concatenate([_ld(sq_v[pp][k], 0, 128), kvw], axis=0) if i >= 1 else kvw

        project(lhs, i, pp == 0, use, kv_flush)
        pend.extend(new)

    def finalize():
        if pend:
            kv_flush()
            keep = (lax.broadcasted_iota(jnp.int32, (64, 128), 0) // 32
                    == lax.broadcasted_iota(jnp.int32, (64, 128), 1) % 2)
            for p in range(2 * NG):
                _st(kvz_v, p * 64, (p + 1) * 64, ALL, jnp.where(keep, acc_v[p, 0:64], 0.0).astype(bf16))
                zc_v[p] = jnp.concatenate([acc_v[p, 64:72]] * 16, axis=0).T

    for i, q in ((0, 0), (0, 1)):
        def use(a, t, c, i=i, q=q):
            for e in range(2):
                g = 2 * (2 * q + e) + a
                _st(phiq_v[i], g * 256, (g + 1) * 256, slice(t * 128, (t + 1) * 128),
                    _feat(c[e * 128:(e + 1) * 128]).astype(bf16))

        project(lambda k, q=q: jnp.concatenate([_ld(sq_v[2 * q][k], 0, 128), _ld(sq_v[2 * q + 1][k], 0, 128)], axis=0),
                i, False, use, finalize)

    late()
    yrow = jnp.concatenate([jnp.sum(y, axis=0, keepdims=True) * st["rs"] for y in st["y"]], axis=1)

    parity = lax.broadcasted_iota(jnp.int32, (8, T), 0) % 2

    def attn(i, dep):
        ot = []
        for p in range(2 * NG):
            phi = _ld(phiq_v[i], p * 128, (p + 1) * 128)
            num = jnp.dot(_ld(kvz_v, p * 64, (p + 1) * 64), phi, preferred_element_type=f32)
            zc = zc_v[p]
            pz = (phi.astype(f32) * jnp.concatenate([zc] * (T // 128), axis=1)).reshape(16, 8, T)
            rden = _rcp(_heads(pz, jnp.add) + 1e-6)
            swapped = pltpu.roll(rden, 1, 0)
            for a in range(2):
                r = jnp.where(parity == a, rden, swapped)
                ot.append((num[32 * a:32 * a + 32].reshape(4, 8, T) * r[None]).reshape(32, T))
        ot = jnp.concatenate(ot, axis=0)
        b11, b12, b21, b22 = ot[:HD, :128], ot[:HD, 128:], ot[HD:, :128], ot[HD:, 128:]
        return [s.astype(bf16) for s in (b11 + b22, b11, b12 - b22, b21 - b11, b22, b11 + b12, b21 + b22)]

    def finish(i, o, nxt):
        def m(k):
            return jnp.dot(_ld(wot_v, k * HD, (k + 1) * HD), o[k], preferred_element_type=f32)

        def mix(c, t, a):
            a = a.T
            rows = slice(t * 128, (t + 1) * 128)
            gate = jax.nn.sigmoid(gate_v[i, rows, :])
            omg = 1.0 - gate
            hit = (lax.broadcasted_iota(jnp.int32, (128, 128), 0) + (i * T + t * 128)) == st["idxv"]
            for k in range(HD // 128):
                ks = slice(c * HD + k * 128, c * HD + (k + 1) * 128)
                xb = _ld(x_v[i], t * 128, (t + 1) * 128, ks).astype(f32)
                b = xb + (xb * 0.0 + jnp.where(hit, yrow[:, ks], 0.0))
                res = (gate * a[:, k * 128:(k + 1) * 128] + omg * b).astype(bf16)
                if i:
                    _st(out_v[i - 1], t * 128, (t + 1) * 128, ks, res)
                else:
                    _st(out0_v[t][c], 0, 128, slice(k * 128, (k + 1) * 128), res)
            if i == 0:
                c_o0[t, c].start()

        m5 = m(4)
        o_next = None if nxt is None else attn(nxt, None)
        m3 = m(2)
        mix(0, 1, m3 + m5)
        m2 = m(1)
        m4 = m(3)
        mix(1, 0, m2 + m4)
        m1 = m(0)
        c11 = m1 + m4 - m5
        c22 = m1 - m2 + m3
        mix(0, 0, c11 + m(6))
        mix(1, 1, c22 + m(5))
        if i:
            c_o[i - 1].start()
        return o_next

    order = list(range(1, NC)) + [0]
    o = attn(order[0], None)
    for n, i in enumerate(order):
        o = finish(i, o, order[n + 1] if n + 1 < NC else None)
    for d in c_o + list(c_o0.values()):
        d.wait()


@jax.jit
def pallas_gated_mix__linear_kernel_hedgehog__moe_arch_mod__prompt_kernel(A_x, A_wqkv, A_w_phi, A_wo, B_x, B_w_r, B_w_gate, B_w_up, B_w_down, gate_w):
    anyspec = pl.BlockSpec(memory_space=pl.ANY)
    V = pltpu.VMEM
    P = lambda r, c: V((r // 2, c), u32)
    out = pl.pallas_call(
        _kernel,
        out_shape=jax.ShapeDtypeStruct((S, D), bf16),
        in_specs=[anyspec] * 9,
        out_specs=anyspec,
        scratch_shapes=[
            [P(T, D) for _ in range(NC)],
            [[P(D, 128) for _ in range(NG)] for _ in range(3)],
            V((D, DH), bf16), P(D, D), V((D,), bf16), V((D,), bf16),
            [P(D, FC) for _ in range(NF)], [P(D, FC) for _ in range(NF)], [P(FC, D) for _ in range(NF)],
            [[P(128, HD) for _ in range(7)] for _ in range(NP)],
            [[P(256, HD) for _ in range(7)] for _ in range(NP)],
            [P(7 * 128, HD) for _ in range(NC)], P(7 * HD, HD),
            [P(2 * D, T) for _ in range(NC)],
            V((2 * NG, 80, 128), f32), P(2 * NG * 64, 128), V((2 * NG, 128, 128), f32),
            [P(T, D) for _ in range(NC - 1)], [[P(128, HD) for _ in range(2)] for _ in range(2)],
            V((D, 128), f32), V((NC, T, 128), f32), P(NG * 128, 128), V((16, D), f32), V((NB, 8, 128), f32),
            pltpu.SemaphoreType.DMA((10,)),
        ],
        compiler_params=pltpu.CompilerParams(vmem_limit_bytes=120 * 2**20),
    )(A_x.reshape(S, D), A_wqkv, A_w_phi.reshape(D, DH), A_wo,
      B_w_r, B_w_gate, B_w_up, B_w_down, gate_w)
    return out.reshape(1, S, D)
```

```python
import functools

import jax
import jax.numpy as jnp
from jax import lax
import jax.experimental.pallas as pl
import jax.experimental.pallas.tpu as pltpu

S, D, DH, F = 2048, 1024, 32, 3584
T = 256
NC = S // T
NG = 8
NP = NG // 2
HD = D // 2
FC = 512
NF = F // FC
NB = F // 128
NDOT = 28 * NC + 14
LAG = 4
SEL, SEL_LAG = 104, 7
GU0 = 2
GU1 = 115
W1, W2 = 146, 192
f32, bf16, u32 = jnp.float32, jnp.bfloat16, jnp.uint32
NT = (((1,), (1,)), ((), ()))
LOG2E = 1.4426950408889634
ALL = slice(None)


def _ld(ref, r0, r1, cols=ALL):
    return pltpu.bitcast(ref[r0 // 2:r1 // 2, cols], bf16)


def _st(ref, r0, r1, cols, val):
    ref[r0 // 2:r1 // 2, cols] = pltpu.bitcast(val, u32)


def _rcp(x):
    r = pl.reciprocal(x, approx=True)
    return r * (2.0 - x * r)


def _heads(v, op):
    r = v[0]
    for j in range(1, v.shape[0]):
        r = op(r, v[j])
    r = op(r, pltpu.roll(r, 4, 0))
    return op(r, pltpu.roll(r, 2, 0))


def _feat(p):
    outs = []
    for h in range(2):
        ph = p[h * 64:(h + 1) * 64].reshape(8, 8, p.shape[1])
        e1 = jnp.exp2(ph - _heads(ph, jnp.maximum)[None])
        e2 = jnp.exp2(_heads(ph, jnp.minimum)[None] - ph)
        for e in (e1, e2):
            outs.append((e * _rcp(_heads(e, jnp.add))[None]).reshape(64, p.shape[1]))
    return jnp.concatenate(outs, axis=0)


def _left(a11, a12, a21, a22):
    return (a11 + a22, a21 + a22, a11, a22, a11 + a12, a21 - a11, a12 - a22)


def _right(k, b11, b12, b21, b22):
    if k == 1:
        return b11()
    if k == 4:
        return b22()
    p, q, sub = {0: (b11, b22, False), 2: (b12, b22, True), 3: (b21, b11, True),
                 5: (b11, b12, False), 6: (b21, b22, False)}[k]
    p, q = p().astype(f32), q().astype(f32)
    return (p - q if sub else p + q).astype(bf16)


def _kernel(x_hbm, wqkv_hbm, wphi_hbm, wo_hbm, wr_hbm, wg_hbm, wu_hbm, wd_hbm, gw_hbm,
            out_hbm,
            x_v, wraw_v, wphi_v, wo_v, wr_v, gw_v, wg_v, wu_v, wd_v,
            sq_v, skv_v, xt_v, wot_v, phiq_v, acc_v, kvz_v, zc_v, out_v, out0_v, xcol_v, gate_v, bd_v, rg_v, h_v,
            sems):
    cp = pltpu.make_async_copy
    c_wphi = cp(wphi_hbm, wphi_v, sems.at[0])
    c_wr = cp(wr_hbm, wr_v, sems.at[9])
    c_gw = cp(gw_hbm, gw_v, sems.at[9])
    wsem = lambda j, g: 1 + g // 2 if j else (5, 9)[g // 4]
    c_w = [[cp(wqkv_hbm.at[:, pl.ds(j * D + g * 128, 128)], wraw_v[j][g].bitcast(bf16), sems.at[wsem(j, g)])
            for g in range(NG)] for j in range(3)]
    c_x = [cp(x_hbm.at[pl.ds(i * T, T)], x_v[i].bitcast(bf16), sems.at[(1, 5, 9, 6)[min(i, 3)]])
           for i in range(NC)]
    c_gu = [cp(w.at[:, pl.ds(j * FC, FC)], v[j].bitcast(bf16), sems.at[6 if j < GU0 else 7])
            for j in range(NF) for w, v in ((wg_hbm, wg_v), (wu_hbm, wu_v))]
    c_d = [cp(wd_hbm.at[pl.ds(j * FC, FC)], wd_v[j].bitcast(bf16), sems.at[8]) for j in range(NF)]
    c_d.append(cp(wo_hbm, wo_v.bitcast(bf16), sems.at[8]))
    c_o = [cp(out_v[i - 1].bitcast(bf16), out_hbm.at[pl.ds(i * T, T)], sems.at[2]) for i in range(1, NC)]
    c_o0 = {(t, c): cp(out0_v[t][c].bitcast(bf16), out_hbm.at[pl.ds(t * 128, 128), pl.ds(c * HD, HD)], sems.at[2])
            for t in range(2) for c in range(2)}

    for d in [c_wphi, c_w[1][0], c_w[1][1], c_w[2][0], c_w[2][1], c_x[0]]:
        d.start()
    for g in range(2, NG):
        c_w[1][g].start()
        c_w[2][g].start()
    for d in [c_x[1]] + c_w[0][:4] + [c_wr, c_gw] + c_w[0][4:] + c_x[2:] + c_gu + c_d:
        d.start()

    row = lax.broadcasted_iota(jnp.int32, (128, 128), 0)
    col = lax.broadcasted_iota(jnp.int32, (128, 128), 1)
    diag = (row // DH) == (col // 64) * 2 + col % 2
    rep = (((lax.broadcasted_iota(jnp.int32, (DH, 128), 1) % 64) // 2)
           == lax.broadcasted_iota(jnp.int32, (DH, 128), 0)).astype(bf16)
    acc_v[...] = jnp.zeros_like(acc_v)
    ones = jnp.ones((16, T), bf16)
    c_wphi.wait()
    for g in range(NG):
        wt = jnp.dot(wphi_v[g * 128:(g + 1) * 128, :], rep, preferred_element_type=f32)
        _st(bd_v, g * 128, (g + 1) * 128, ALL, jnp.where(diag, wt, 0.0).T.astype(bf16))

    def prep(j, pp):
        w = []
        for g in (2 * pp, 2 * pp + 1):
            raw = _ld(wraw_v[j][g], 0, D)
            if j < 2:
                w.append(lax.dot_general(_ld(bd_v, g * 128, (g + 1) * 128), raw, NT,
                                         preferred_element_type=f32) * LOG2E)
            else:
                w.append(raw.T.astype(f32))
        dst, r0 = (sq_v, 0) if j == 0 else (skv_v, (j - 1) * 128)
        for k, s in enumerate(_left(w[0][:, :HD], w[0][:, HD:], w[1][:, :HD], w[1][:, HD:])):
            _st(dst[pp][k], r0, r0 + 128, ALL, s.astype(bf16))

    st = {"n": 0}

    def tie(a, dep):
        if dep is None:
            return a
        if a.dtype == f32:
            blk = jnp.where(st["never"], dep, a[0:8])
            return jnp.concatenate([blk, a[8:]], axis=0) if a.shape[0] > 8 else blk
        blk = pltpu.bitcast(jnp.where(st["never"], dep, pltpu.bitcast(a[0:16, 0:128], f32)), bf16)
        if a.shape[1] > 128:
            blk = jnp.concatenate([blk, a[0:16, 128:]], axis=1)
        return jnp.concatenate([blk, a[16:]], axis=0)

    def xright(i, k, fresh):
        blk = lambda r, c: (lambda: _ld(x_v[i], r * 128, (r + 1) * 128, slice(c * HD, (c + 1) * HD)))
        if k in (1, 4) or fresh:
            val = _right(k, blk(0, 0), blk(1, 0), blk(0, 1), blk(1, 1))
            if k not in (1, 4):
                _st(xt_v[i], k * 128, (k + 1) * 128, ALL, val)
            return val
        return _ld(xt_v[i], k * 128, (k + 1) * 128)

    jobs = {}
    after = {}
    ties = {}

    def project(lhs, i, fresh, use, mid):
        def m(k):
            n = st["n"]
            st["n"] = n + 1
            out = lax.dot_general(tie(lhs(k), ties.pop(n, None)), xright(i, k, fresh), NT,
                                  preferred_element_type=f32)
            if n in after:
                after.pop(n)()
            if n in jobs:
                res = jobs.pop(n)(out[0:8])
                lag = SEL_LAG if n == SEL else LAG
                if n + lag < NDOT:
                    assert n + lag not in ties
                    ties[n + lag] = res
            return out
        m5 = m(4)
        late()
        m3 = m(2)
        m2 = m(1)
        use(0, 1, m3 + m5)
        mid()
        m4 = m(3)
        m1 = m(0)
        use(1, 0, m2 + m4)
        c11 = m1 + m4 - m5
        c22 = m1 - m2 + m3
        c11 = c11 + m(6)
        m6 = m(5)
        use(0, 0, c11)
        st["late"] = lambda: use(1, 1, c22 + m6)

    def late():
        st.pop("late", lambda: None)()

    pend = []

    def kv_flush():
        for g, fk, vt in pend:
            fk = jnp.concatenate(fk, axis=1)
            vt = jnp.concatenate(vt, axis=1)
            for p in range(2):
                lhs = jnp.concatenate([vt[p * 64:(p + 1) * 64], ones], axis=0)
                acc_v[2 * g + p] += lax.dot_general(lhs, fk[p * 128:(p + 1) * 128], NT,
                                                    preferred_element_type=f32)
        pend.clear()

    def router(i, part, dep):
        best, bidx = st["best"], st["bidx"]
        for b in range(part * 4, part * 4 + 4):
            rows = slice(b * 16, (b + 1) * 16)
            xf = [_ld(x_v[i], b * 16, (b + 1) * 16, slice(k * 128, (k + 1) * 128)).astype(f32)
                  for k in range(D // 128)]
            acc = []
            for w in range(2):
                for hf in range(2):
                    a = None
                    for k in range(D // 128):
                        p = xf[k][hf * 8:(hf + 1) * 8] * rg_v[w * 8:(w + 1) * 8, k * 128:(k + 1) * 128]
                        a = tie(p, dep) if k == 0 else a + p
                    acc.append(a)
                    dep = a
            ra, ga = jnp.concatenate(acc[0:2], axis=0), jnp.concatenate(acc[2:4], axis=0)
            r = jnp.sum(ra, axis=1, keepdims=True).astype(bf16).astype(f32)
            gate_v[i, rows, :] = jnp.broadcast_to(jnp.sum(ga, axis=1, keepdims=True), (16, 128))
            r = jnp.broadcast_to(r, (16, 128))
            for k in range(2):
                rk = r[k * 8:(k + 1) * 8]
                if best is None:
                    best, bidx = rk, jnp.zeros((8, 128), jnp.int32)
                else:
                    better = rk > best
                    best = jnp.where(better, rk, best)
                    bidx = jnp.where(better, i * T + b * 16 + k * 8, bidx)
        st["best"], st["bidx"] = best, bidx
        return dep

    def select():
        best, bidx = st["best"], st["bidx"]
        m = jnp.max(best, axis=0, keepdims=True)
        cand = jnp.where(best == m, bidx + lax.broadcasted_iota(jnp.int32, (8, 128), 0), S)
        idxv = jnp.min(cand, axis=0, keepdims=True) & (S - 1)
        idx = idxv[0, 0]
        st["idxv"] = idxv
        st["rs"] = jax.nn.sigmoid(m)
        base = pl.multiple_of(((idx % T) // 16) * 8, 8)
        tile = x_v[0][pl.ds(base, 8), :]
        for i in range(1, NC):
            tile = jnp.where(idx // T == i, x_v[i][pl.ds(base, 8), :], tile)
        tile = pltpu.bitcast(tile, bf16).astype(f32)
        sel = lax.broadcasted_iota(jnp.int32, (16, D), 0) == (idx % 16)
        xs = jnp.sum(jnp.where(sel, tile, 0.0), axis=0, keepdims=True)
        for k in range(D // 128):
            xc = jnp.broadcast_to(xs[:, k * 128:(k + 1) * 128], (128, 128)).T
            xcol_v[k * 128:(k + 1) * 128, :] = xc
            best = jnp.maximum(best, xc[120:128])
        st["y"] = [None] * (D // 128)
        return best

    def chain(w_ref, r0, nblk, cols, col_of, dep):
        acc = None
        for k in range(nblk):
            p = _ld(w_ref, r0 + k * 16, r0 + (k + 1) * 16, cols).astype(f32) * col_of(k)
            acc = tie(p[0:8], dep) if acc is None else acc + p[0:8]
            acc = acc + p[8:16]
        return acc

    def ffn_in(w, c, dep):
        j, cc = divmod(c, FC // 128)
        acc = chain((wg_v, wu_v)[w][j], 0, D // 16, slice(cc * 128, (cc + 1) * 128),
                    lambda k: xcol_v[k * 16:(k + 1) * 16, :], dep)
        v = jnp.sum(acc, axis=0, keepdims=True)
        if w == 0:
            st["g", c] = v * jax.nn.sigmoid(v)
        else:
            h_v[c] = jnp.broadcast_to(st.pop(("g", c)) * v, (8, 128))
        return acc

    def ffn_down(c, dep):
        j, cc = divmod(c, FC // 128)
        hcol = jnp.concatenate([h_v[c]] * 16, axis=0).T
        ys = st["y"]
        for n in range(D // 128):
            dep = chain(wd_v[j], cc * 128, 128 // 16, slice(n * 128, (n + 1) * 128),
                        lambda k: hcol[k * 16:(k + 1) * 16], dep)
            ys[n] = dep if ys[n] is None else ys[n] + dep
        return dep

    def wo_job(r, e, dep):
        def blk(a, b):
            r0, c0 = b * HD + e * 128, a * HD + r * 128
            return _ld(wo_v, r0, r0 + 128, slice(c0, c0 + 128)).T.astype(f32)
        for k, v in enumerate(_left(blk(0, 0), blk(0, 1), blk(1, 0), blk(1, 1))):
            _st(wot_v, k * HD + r * 128, k * HD + (r + 1) * 128, slice(e * 128, (e + 1) * 128), v.astype(bf16))
            dep = jnp.maximum(dep, v[120:128])
        return dep

    def wait_kv(pp):
        for g in (2 * pp, 2 * pp + 1):
            c_w[1][g].wait()
            c_w[2][g].wait()
        if pp == 0:
            c_x[0].wait()
        prep(1, pp)
        prep(2, pp)

    def wait_q(half):
        for d in [c_x[1 + half]] + c_w[0][4 * half:4 * half + 4] + [c_wr, c_gw][:2 * half]:
            d.wait()
        prep(0, 2 * half)
        if half:
            wr = wr_v[...].reshape(1, D).astype(f32)
            rg_v[0:8, :] = jnp.broadcast_to(wr, (8, D))
            rg_v[8:16, :] = jnp.broadcast_to(gw_v[...].reshape(1, D).astype(f32), (8, D))
            st["best"] = st["bidx"] = None
            st["never"] = jnp.broadcast_to((pltpu.bitcast(wr[:, 0:128], jnp.int32) | 1) == 0, (8, 128))

    def wait_all(ds):
        for d in ds:
            d.wait()

    for pp in range(1, NP):
        after[7 * pp - 1] = functools.partial(wait_kv, pp)
    after[26] = functools.partial(wait_q, 0)
    after[33] = functools.partial(prep, 0, 1)
    after[40] = functools.partial(wait_q, 1)
    after[47] = functools.partial(prep, 0, 3)
    after[83] = functools.partial(wait_all, c_x[3:] + c_gu[:2 * GU0])
    for r in range(4 * NC):
        jobs[56 + 2 * r if r < 12 else 72 + r] = functools.partial(router, r // 4, r % 4)
    jobs[SEL] = lambda dep: select()
    n0 = 8 * GU0
    for u in range(2 * NB):
        pos = GU1 + (u * (W1 - LAG - GU1)) // n0 if u < n0 else W1 + 1 + ((u - n0) * (W2 - LAG - W1)) // (2 * NB - n0)
        assert pos not in jobs
        jobs[pos] = functools.partial(ffn_in, u % 2, u // 2)
    after[W1] = functools.partial(wait_all, c_gu[2 * GU0:])
    after[W2] = functools.partial(wait_all, c_d)
    tail = sorted([(c / NB, functools.partial(ffn_down, c)) for c in range(NB)]
                  + [((w + 0.5) / 16, functools.partial(wo_job, w // 4, w % 4)) for w in range(16)], key=lambda e: e[0])
    for pos, (_, job) in enumerate(tail):
        jobs[W2 + 1 + pos] = job

    wait_kv(0)
    for i, pp in [(i, pp) for i in range(NC) for pp in range(NP)]:
        new = [(2 * pp + a, [None, None], [None, None]) for a in range(2)]

        def use(a, t, c, new=new, i=i, pp=pp):
            g = 2 * pp + a
            if i >= 1:
                _st(phiq_v[i], g * 256, (g + 1) * 256, slice(t * 128, (t + 1) * 128), _feat(c[0:128]).astype(bf16))
            new[a][1][t] = _feat(c[-256:-128]).astype(bf16)
            new[a][2][t] = c[-128:].astype(bf16)

        def lhs(k, i=i, pp=pp):
            kvw = _ld(skv_v[pp][k], 0, 256)
            return jnp.concatenate([_ld(sq_v[pp][k], 0, 128), kvw], axis=0) if i >= 1 else kvw

        project(lhs, i, pp == 0, use, kv_flush)
        pend.extend(new)

    def finalize():
        if pend:
            kv_flush()
            keep = (lax.broadcasted_iota(jnp.int32, (64, 128), 0) // 32
                    == lax.broadcasted_iota(jnp.int32, (64, 128), 1) % 2)
            for p in range(2 * NG):
                _st(kvz_v, p * 64, (p + 1) * 64, ALL, jnp.where(keep, acc_v[p, 0:64], 0.0).astype(bf16))
                zc_v[p] = jnp.concatenate([acc_v[p, 64:72]] * 16, axis=0).T

    for q in range(NP // 2):
        def use(a, t, c, q=q):
            for e in range(2):
                g = 2 * (2 * q + e) + a
                _st(phiq_v[0], g * 256, (g + 1) * 256, slice(t * 128, (t + 1) * 128),
                    _feat(c[e * 128:(e + 1) * 128]).astype(bf16))

        project(lambda k, q=q: jnp.concatenate([_ld(sq_v[2 * q][k], 0, 128), _ld(sq_v[2 * q + 1][k], 0, 128)], axis=0),
                0, False, use, finalize)

    late()
    yrow = jnp.concatenate([jnp.sum(y, axis=0, keepdims=True) * st["rs"] for y in st["y"]], axis=1)

    parity = lax.broadcasted_iota(jnp.int32, (8, T), 0) % 2

    def attn(i):
        ot = []
        for p in range(2 * NG):
            phi = _ld(phiq_v[i], p * 128, (p + 1) * 128)
            num = jnp.dot(_ld(kvz_v, p * 64, (p + 1) * 64), phi, preferred_element_type=f32)
            zc = zc_v[p]
            pz = (phi.astype(f32) * jnp.concatenate([zc] * (T // 128), axis=1)).reshape(16, 8, T)
            rden = _rcp(_heads(pz, jnp.add) + 1e-6)
            swapped = pltpu.roll(rden, 1, 0)
            for a in range(2):
                r = jnp.where(parity == a, rden, swapped)
                ot.append((num[32 * a:32 * a + 32].reshape(4, 8, T) * r[None]).reshape(32, T))
        ot = jnp.concatenate(ot, axis=0)
        b11, b12, b21, b22 = ot[:HD, :128], ot[:HD, 128:], ot[HD:, :128], ot[HD:, 128:]
        return [s.astype(bf16) for s in (b11 + b22, b11, b12 - b22, b21 - b11, b22, b11 + b12, b21 + b22)]

    def finish(i, o, nxt):
        def m(k):
            return jnp.dot(_ld(wot_v, k * HD, (k + 1) * HD), o[k], preferred_element_type=f32)

        def mix(c, t, a):
            a = a.T
            rows = slice(t * 128, (t + 1) * 128)
            gate = jax.nn.sigmoid(gate_v[i, rows, :])
            omg = 1.0 - gate
            hit = (lax.broadcasted_iota(jnp.int32, (128, 128), 0) + (i * T + t * 128)) == st["idxv"]
            for k in range(HD // 128):
                ks = slice(c * HD + k * 128, c * HD + (k + 1) * 128)
                xb = _ld(x_v[i], t * 128, (t + 1) * 128, ks).astype(f32)
                b = xb + (xb * 0.0 + jnp.where(hit, yrow[:, ks], 0.0))
                res = (gate * a[:, k * 128:(k + 1) * 128] + omg * b).astype(bf16)
                if i:
                    _st(out_v[i - 1], t * 128, (t + 1) * 128, ks, res)
                else:
                    _st(out0_v[t][c], 0, 128, slice(k * 128, (k + 1) * 128), res)
            if i == 0:
                c_o0[t, c].start()

        m5 = m(4)
        o_next = None if nxt is None else attn(nxt)
        m3 = m(2)
        mix(0, 1, m3 + m5)
        m2 = m(1)
        m4 = m(3)
        mix(1, 0, m2 + m4)
        m1 = m(0)
        c11 = m1 + m4 - m5
        c22 = m1 - m2 + m3
        mix(0, 0, c11 + m(6))
        mix(1, 1, c22 + m(5))
        if i:
            c_o[i - 1].start()
        return o_next

    order = list(range(1, NC)) + [0]
    o = attn(order[0])
    for n, i in enumerate(order):
        o = finish(i, o, order[n + 1] if n + 1 < NC else None)
    for d in c_o + list(c_o0.values()):
        d.wait()


@jax.jit
def pallas_gated_mix__linear_kernel_hedgehog__moe_arch_mod__prompt_kernel(
        A_x, A_wqkv, A_w_phi, A_wo, B_x, B_w_r, B_w_gate, B_w_up, B_w_down, gate_w):
    anyspec = pl.BlockSpec(memory_space=pl.ANY)
    V = pltpu.VMEM
    P = lambda r, c: V((r // 2, c), u32)
    out = pl.pallas_call(
        _kernel,
        out_shape=jax.ShapeDtypeStruct((S, D), bf16),
        in_specs=[anyspec] * 9,
        out_specs=anyspec,
        scratch_shapes=[
            [P(T, D) for _ in range(NC)],
            [[P(D, 128) for _ in range(NG)] for _ in range(3)],
            V((D, DH), bf16), P(D, D), V((D,), bf16), V((D,), bf16),
            [P(D, FC) for _ in range(NF)], [P(D, FC) for _ in range(NF)], [P(FC, D) for _ in range(NF)],
            [[P(128, HD) for _ in range(7)] for _ in range(NP)],
            [[P(256, HD) for _ in range(7)] for _ in range(NP)],
            [P(7 * 128, HD) for _ in range(NC)], P(7 * HD, HD),
            [P(2 * D, T) for _ in range(NC)],
            V((2 * NG, 80, 128), f32), P(2 * NG * 64, 128), V((2 * NG, 128, 128), f32),
            [P(T, D) for _ in range(NC - 1)], [[P(128, HD) for _ in range(2)] for _ in range(2)],
            V((D, 128), f32), V((NC, T, 128), f32), P(NG * 128, 128), V((16, D), f32), V((NB, 8, 128), f32),
            pltpu.SemaphoreType.DMA((10,)),
        ],
        compiler_params=pltpu.CompilerParams(vmem_limit_bytes=120 * 2**20),
    )(A_x.reshape(S, D), A_wqkv, A_w_phi.reshape(D, DH), A_wo,
      B_w_r, B_w_gate, B_w_up, B_w_down, gate_w)
    return out.reshape(1, S, D)
```

```python
import functools

import jax
import jax.numpy as jnp
from jax import lax
import jax.experimental.pallas as pl
import jax.experimental.pallas.tpu as pltpu

S, D, DH, F = 2048, 1024, 32, 3584
T = 256
NC = S // T
NG = 8
NP = NG // 2
HD = D // 2
FC = 512
NF = F // FC
NB = F // 128
NDOT = 28 * NC + 14
LAG = 5
SEL, SEL_LAG = 104, 6
GU0 = 2
GU1 = 114
W1, W2 = 147, 192
f32, bf16, u32 = jnp.float32, jnp.bfloat16, jnp.uint32
NT = (((1,), (1,)), ((), ()))
LOG2E = 1.4426950408889634
ALL = slice(None)


def _ld(ref, r0, r1, cols=ALL):
    if ref.dtype == bf16:
        return ref[r0:r1, cols]
    return pltpu.bitcast(ref[r0 // 2:r1 // 2, cols], bf16)


def _st(ref, r0, r1, cols, val):
    if ref.dtype == bf16:
        ref[r0:r1, cols] = val
    else:
        ref[r0 // 2:r1 // 2, cols] = pltpu.bitcast(val, u32)


def _rcp(x):
    r = pl.reciprocal(x, approx=True)
    return r * (2.0 - x * r)


def _heads(v, op):
    r = v[0]
    for j in range(1, v.shape[0]):
        r = op(r, v[j])
    r = op(r, pltpu.roll(r, 4, 0))
    return op(r, pltpu.roll(r, 2, 0))


def _feat(p):
    outs = []
    for h in range(2):
        ph = p[h * 64:(h + 1) * 64].reshape(8, 8, p.shape[1])
        e1 = jnp.exp2(ph - _heads(ph, jnp.maximum)[None])
        e2 = jnp.exp2(_heads(ph, jnp.minimum)[None] - ph)
        for e in (e1, e2):
            outs.append((e * _rcp(_heads(e, jnp.add))[None]).reshape(64, p.shape[1]))
    return jnp.concatenate(outs, axis=0)


def _left(a11, a12, a21, a22):
    return (a11 + a22, a21 + a22, a11, a22, a11 + a12, a21 - a11, a12 - a22)


def _right(k, b11, b12, b21, b22):
    if k == 1:
        return b11()
    if k == 4:
        return b22()
    p, q, sub = {0: (b11, b22, False), 2: (b12, b22, True), 3: (b21, b11, True),
                 5: (b11, b12, False), 6: (b21, b22, False)}[k]
    p, q = p().astype(f32), q().astype(f32)
    return (p - q if sub else p + q).astype(bf16)


def _kernel(x_hbm, wqkv_hbm, wphi_hbm, wo_hbm, wr_hbm, wg_hbm, wu_hbm, wd_hbm, gw_hbm,
            out_hbm,
            x_v, wraw_v, wphi_v, wo_v, wr_v, gw_v, wg_v, wu_v, wd_v,
            sq_v, skv_v, xt_v, wot_v, phiq_v, acc_v, kvz_v, zc_v, out_v, out0_v, xcol_v, gate_v, bd_v, rg_v, h_v,
            sems):
    cp = pltpu.make_async_copy
    c_wphi = cp(wphi_hbm, wphi_v, sems.at[0])
    c_wr = cp(wr_hbm, wr_v, sems.at[9])
    c_gw = cp(gw_hbm, gw_v, sems.at[9])
    wsem = lambda j, g: 1 + g // 2 if j else (5, 9)[g // 4]
    c_w = [[cp(wqkv_hbm.at[:, pl.ds(j * D + g * 128, 128)], wraw_v[j][g], sems.at[wsem(j, g)])
            for g in range(NG)] for j in range(3)]
    c_x = [cp(x_hbm.at[pl.ds(i * T, T)], x_v[i], sems.at[(1, 5, 9, 6)[min(i, 3)]])
           for i in range(NC)]
    c_gu = [cp(w.at[:, pl.ds(j * FC, FC)], v[j], sems.at[6 if j < GU0 else 7])
            for j in range(NF) for w, v in ((wg_hbm, wg_v), (wu_hbm, wu_v))]
    c_d = [cp(wd_hbm.at[pl.ds(j * FC, FC)], wd_v[j], sems.at[8]) for j in range(NF)]
    c_d.append(cp(wo_hbm, wo_v, sems.at[8]))
    c_o = [cp(out_v[i - 1], out_hbm.at[pl.ds(i * T, T)], sems.at[2]) for i in range(1, NC)]
    c_o0 = {(t, c): cp(out0_v[t][c], out_hbm.at[pl.ds(t * 128, 128), pl.ds(c * HD, HD)], sems.at[2])
            for t in range(2) for c in range(2)}

    for d in [c_wphi, c_w[1][0], c_w[1][1], c_w[2][0], c_w[2][1], c_x[0]]:
        d.start()
    for g in range(2, NG):
        c_w[1][g].start()
        c_w[2][g].start()
    for d in [c_x[1]] + c_w[0][:4] + [c_wr, c_gw] + c_w[0][4:] + c_x[2:] + c_gu + c_d:
        d.start()

    row = lax.broadcasted_iota(jnp.int32, (128, 128), 0)
    col = lax.broadcasted_iota(jnp.int32, (128, 128), 1)
    diag = (row // DH) == (col // 64) * 2 + col % 2
    rep = (((lax.broadcasted_iota(jnp.int32, (DH, 128), 1) % 64) // 2)
           == lax.broadcasted_iota(jnp.int32, (DH, 128), 0)).astype(bf16)
    acc_v[...] = jnp.zeros_like(acc_v)
    ones = jnp.ones((8, T), f32)
    c_wphi.wait()
    for g in range(NG):
        wt = jnp.dot(wphi_v[g * 128:(g + 1) * 128, :], rep, preferred_element_type=f32)
        _st(bd_v, g * 128, (g + 1) * 128, ALL, jnp.where(diag, wt, 0.0).T.astype(bf16))

    def prep(j, pp):
        w = []
        for g in (2 * pp, 2 * pp + 1):
            raw = _ld(wraw_v[j][g], 0, D)
            if j < 2:
                w.append(lax.dot_general(_ld(bd_v, g * 128, (g + 1) * 128), raw, NT,
                                         preferred_element_type=f32) * LOG2E)
            else:
                w.append(raw.T.astype(f32))
        dst, r0 = (sq_v, 0) if j == 0 else (skv_v, (j - 1) * 128)
        for k, s in enumerate(_left(w[0][:, :HD], w[0][:, HD:], w[1][:, :HD], w[1][:, HD:])):
            _st(dst[pp][k], r0, r0 + 128, ALL, s.astype(bf16))

    st = {"n": 0}

    def tie(a, dep):
        if dep is None:
            return a
        if a.dtype == f32:
            blk = jnp.where(st["never"], dep, a[0:8])
            return jnp.concatenate([blk, a[8:]], axis=0) if a.shape[0] > 8 else blk
        blk = pltpu.bitcast(jnp.where(st["never"], dep, pltpu.bitcast(a[0:16, 0:128], f32)), bf16)
        if a.shape[1] > 128:
            blk = jnp.concatenate([blk, a[0:16, 128:]], axis=1)
        return jnp.concatenate([blk, a[16:]], axis=0)

    def xright(i, k, fresh):
        blk = lambda r, c: (lambda: _ld(x_v[i], r * 128, (r + 1) * 128, slice(c * HD, (c + 1) * HD)))
        if k in (1, 4) or fresh:
            val = _right(k, blk(0, 0), blk(1, 0), blk(0, 1), blk(1, 1))
            if k not in (1, 4):
                _st(xt_v[i], k * 128, (k + 1) * 128, ALL, val)
            return val
        return _ld(xt_v[i], k * 128, (k + 1) * 128)

    jobs = {}
    after = {}
    ties = {}

    def project(lhs, i, fresh, use, mid):
        def m(k):
            n = st["n"]
            st["n"] = n + 1
            out = lax.dot_general(tie(lhs(k), ties.pop(n, None)), xright(i, k, fresh), NT,
                                  preferred_element_type=f32)
            if n in after:
                after.pop(n)()
            if n in jobs:
                res = jobs.pop(n)(out[0:8])
                lag = SEL_LAG if n == SEL else LAG
                if n + lag < NDOT:
                    assert n + lag not in ties
                    ties[n + lag] = res
            return out
        m5 = m(4)
        late()
        m3 = m(2)
        m2 = m(1)
        use(0, 1, m3 + m5)
        mid()
        m4 = m(3)
        m1 = m(0)
        use(1, 0, m2 + m4)
        c11 = m1 + m4 - m5
        c22 = m1 - m2 + m3
        c11 = c11 + m(6)
        m6 = m(5)
        use(0, 0, c11)
        st["late"] = lambda: use(1, 1, c22 + m6)

    def late():
        st.pop("late", lambda: None)()

    pend = []

    def kv_flush():
        for g, fk, vt in pend:
            fk = jnp.concatenate(fk, axis=1)
            vt = jnp.concatenate(vt, axis=1)
            for p in range(2):
                lhs = jnp.concatenate([vt[p * 64:(p + 1) * 64], ones], axis=0)
                acc_v[2 * g + p] += lax.dot_general(lhs, fk[p * 128:(p + 1) * 128], NT,
                                                    preferred_element_type=f32)
        pend.clear()

    def router(i, part, dep):
        best, bidx = st["best"], st["bidx"]
        for b in range(part * 4, part * 4 + 4):
            rows = slice(b * 16, (b + 1) * 16)
            xf = [_ld(x_v[i], b * 16, (b + 1) * 16, slice(k * 128, (k + 1) * 128)).astype(f32)
                  for k in range(D // 128)]
            acc = []
            for w in range(2):
                for hf in range(2):
                    a = None
                    for k in range(D // 128):
                        p = xf[k][hf * 8:(hf + 1) * 8] * rg_v[w * 8:(w + 1) * 8, k * 128:(k + 1) * 128]
                        a = tie(p, dep) if k == 0 else a + p
                    acc.append(a)
                    dep = a
            ra, ga = jnp.concatenate(acc[0:2], axis=0), jnp.concatenate(acc[2:4], axis=0)
            r = jnp.sum(ra, axis=1, keepdims=True).astype(bf16).astype(f32)
            gate_v[i, rows, :] = jnp.broadcast_to(jnp.sum(ga, axis=1, keepdims=True), (16, 128))
            r = jnp.broadcast_to(r, (16, 128))
            for k in range(2):
                rk = r[k * 8:(k + 1) * 8]
                if best is None:
                    best, bidx = rk, jnp.zeros((8, 128), jnp.int32)
                else:
                    better = rk > best
                    best = jnp.where(better, rk, best)
                    bidx = jnp.where(better, i * T + b * 16 + k * 8, bidx)
        st["best"], st["bidx"] = best, bidx
        return dep

    def select():
        best, bidx = st["best"], st["bidx"]
        m = jnp.max(best, axis=0, keepdims=True)
        cand = jnp.where(best == m, bidx + lax.broadcasted_iota(jnp.int32, (8, 128), 0), S)
        idxv = jnp.min(cand, axis=0, keepdims=True) & (S - 1)
        idx = idxv[0, 0]
        st["idxv"] = idxv
        st["rs"] = jax.nn.sigmoid(m)
        base = pl.multiple_of(((idx % T) // 16) * 16, 16)
        tile = x_v[0][pl.ds(base, 16), :].astype(f32)
        for i in range(1, NC):
            tile = jnp.where(idx // T == i, x_v[i][pl.ds(base, 16), :].astype(f32), tile)
        sel = lax.broadcasted_iota(jnp.int32, (16, D), 0) == (idx % 16)
        xs = jnp.sum(jnp.where(sel, tile, 0.0), axis=0, keepdims=True)
        for k in range(D // 128):
            xc = jnp.broadcast_to(xs[:, k * 128:(k + 1) * 128], (128, 128)).T
            xcol_v[k * 128:(k + 1) * 128, :] = xc
            best = jnp.maximum(best, xc[120:128])
        st["y"] = [None] * (D // 128)
        return best

    def chain(w_ref, r0, nblk, cols, col_of, dep):
        acc = None
        for k in range(nblk):
            p = _ld(w_ref, r0 + k * 16, r0 + (k + 1) * 16, cols).astype(f32) * col_of(k)
            acc = tie(p[0:8], dep) if acc is None else acc + p[0:8]
            acc = acc + p[8:16]
        return acc

    def ffn_in(w, c, dep):
        j, cc = divmod(c, FC // 128)
        acc = chain((wg_v, wu_v)[w][j], 0, D // 16, slice(cc * 128, (cc + 1) * 128),
                    lambda k: xcol_v[k * 16:(k + 1) * 16, :], dep)
        v = jnp.sum(acc, axis=0, keepdims=True)
        if w == 0:
            st["g", c] = v * jax.nn.sigmoid(v)
        else:
            h_v[c] = jnp.broadcast_to(st.pop(("g", c)) * v, (8, 128))
        return acc

    def ffn_down(c, dep):
        j, cc = divmod(c, FC // 128)
        hcol = jnp.concatenate([h_v[c]] * 16, axis=0).T
        ys = st["y"]
        for n in range(D // 128):
            dep = chain(wd_v[j], cc * 128, 128 // 16, slice(n * 128, (n + 1) * 128),
                        lambda k: hcol[k * 16:(k + 1) * 16], dep)
            ys[n] = dep if ys[n] is None else ys[n] + dep
        return dep

    def wo_job(r, e, dep):
        def blk(a, b):
            r0, c0 = b * HD + e * 128, a * HD + r * 128
            return _ld(wo_v, r0, r0 + 128, slice(c0, c0 + 128)).T.astype(f32)
        for k, v in enumerate(_left(blk(0, 0), blk(0, 1), blk(1, 0), blk(1, 1))):
            _st(wot_v, k * HD + r * 128, k * HD + (r + 1) * 128, slice(e * 128, (e + 1) * 128), v.astype(bf16))
            dep = jnp.maximum(dep, v[120:128])
        return dep

    def wait_kv(pp):
        for g in (2 * pp, 2 * pp + 1):
            c_w[1][g].wait()
            c_w[2][g].wait()
        if pp == 0:
            c_x[0].wait()
        prep(1, pp)
        prep(2, pp)

    def wait_q(half):
        for d in [c_x[1 + half]] + c_w[0][4 * half:4 * half + 4] + [c_wr, c_gw][:2 * half]:
            d.wait()
        prep(0, 2 * half)
        if half:
            wr = wr_v[...].reshape(1, D).astype(f32)
            rg_v[0:8, :] = jnp.broadcast_to(wr, (8, D))
            rg_v[8:16, :] = jnp.broadcast_to(gw_v[...].reshape(1, D).astype(f32), (8, D))
            st["best"] = st["bidx"] = None
            st["never"] = jnp.broadcast_to((pltpu.bitcast(wr[:, 0:128], jnp.int32) | 1) == 0, (8, 128))

    def wait_all(ds):
        for d in ds:
            d.wait()

    for pp in range(1, NP):
        after[7 * pp - 1] = functools.partial(wait_kv, pp)
    after[26] = functools.partial(wait_q, 0)
    after[33] = functools.partial(prep, 0, 1)
    after[40] = functools.partial(wait_q, 1)
    after[47] = functools.partial(prep, 0, 3)
    after[83] = functools.partial(wait_all, c_x[3:] + c_gu[:2 * GU0])
    for r in range(4 * NC):
        jobs[56 + 2 * r if r < 12 else 72 + r] = functools.partial(router, r // 4, r % 4)
    jobs[SEL] = lambda dep: select()
    n0 = 8 * GU0
    for u in range(2 * NB):
        pos = GU1 + (u * (W1 - LAG - GU1)) // n0 if u < n0 else W1 + 1 + ((u - n0) * (W2 - LAG - W1)) // (2 * NB - n0)
        assert pos not in jobs
        jobs[pos] = functools.partial(ffn_in, u % 2, u // 2)
    after[W1] = functools.partial(wait_all, c_gu[2 * GU0:])
    after[W2] = functools.partial(wait_all, c_d)
    tail = sorted([(c / NB, functools.partial(ffn_down, c)) for c in range(NB)]
                  + [((w + 0.5) / 16, functools.partial(wo_job, w // 4, w % 4)) for w in range(16)], key=lambda e: e[0])
    for pos, (_, job) in enumerate(tail):
        jobs[W2 + 1 + pos] = job

    wait_kv(0)
    for i, pp in [(i, pp) for i in range(NC) for pp in range(NP)]:
        new = [(2 * pp + a, [None, None], [None, None]) for a in range(2)]

        def use(a, t, c, new=new, i=i, pp=pp):
            g = 2 * pp + a
            if i >= 1:
                _st(phiq_v[i], g * 256, (g + 1) * 256, slice(t * 128, (t + 1) * 128), _feat(c[0:128]).astype(bf16))
            new[a][1][t] = _feat(c[-256:-128]).astype(bf16)
            new[a][2][t] = c[-128:]

        def lhs(k, i=i, pp=pp):
            kvw = _ld(skv_v[pp][k], 0, 256)
            return jnp.concatenate([_ld(sq_v[pp][k], 0, 128), kvw], axis=0) if i >= 1 else kvw

        project(lhs, i, pp == 0, use, kv_flush)
        pend.extend(new)

    def finalize():
        if pend:
            kv_flush()
            keep = (lax.broadcasted_iota(jnp.int32, (64, 128), 0) // 32
                    == lax.broadcasted_iota(jnp.int32, (64, 128), 1) % 2)
            for p in range(2 * NG):
                _st(kvz_v, p * 64, (p + 1) * 64, ALL, jnp.where(keep, acc_v[p, 0:64], 0.0).astype(bf16))
                zc_v[p] = jnp.concatenate([acc_v[p, 64:72]] * 16, axis=0).T

    for q in range(NP // 2):
        def use(a, t, c, q=q):
            for e in range(2):
                g = 2 * (2 * q + e) + a
                _st(phiq_v[0], g * 256, (g + 1) * 256, slice(t * 128, (t + 1) * 128),
                    _feat(c[e * 128:(e + 1) * 128]).astype(bf16))

        project(lambda k, q=q: jnp.concatenate([_ld(sq_v[2 * q][k], 0, 128), _ld(sq_v[2 * q + 1][k], 0, 128)], axis=0),
                0, False, use, finalize)

    late()
    yrow = jnp.concatenate([jnp.sum(y, axis=0, keepdims=True) * st["rs"] for y in st["y"]], axis=1)

    parity = lax.broadcasted_iota(jnp.int32, (8, T), 0) % 2

    def attn(i):
        ot = []
        for p in range(2 * NG):
            phi = _ld(phiq_v[i], p * 128, (p + 1) * 128)
            num = jnp.dot(_ld(kvz_v, p * 64, (p + 1) * 64), phi, preferred_element_type=f32)
            zc = zc_v[p]
            pz = (phi.astype(f32) * jnp.concatenate([zc] * (T // 128), axis=1)).reshape(16, 8, T)
            rden = _rcp(_heads(pz, jnp.add) + 1e-6)
            swapped = pltpu.roll(rden, 1, 0)
            for a in range(2):
                r = jnp.where(parity == a, rden, swapped)
                ot.append((num[32 * a:32 * a + 32].reshape(4, 8, T) * r[None]).reshape(32, T))
        ot = jnp.concatenate(ot, axis=0)
        b11, b12, b21, b22 = ot[:HD, :128], ot[:HD, 128:], ot[HD:, :128], ot[HD:, 128:]
        return [s.astype(bf16) for s in (b11 + b22, b11, b12 - b22, b21 - b11, b22, b11 + b12, b21 + b22)]

    def finish(i, o, nxt):
        def m(k):
            return jnp.dot(_ld(wot_v, k * HD, (k + 1) * HD), o[k], preferred_element_type=f32)

        def mix(c, t, a):
            a = a.T
            rows = slice(t * 128, (t + 1) * 128)
            gate = jax.nn.sigmoid(gate_v[i, rows, :])
            omg = 1.0 - gate
            hit = (lax.broadcasted_iota(jnp.int32, (128, 128), 0) + (i * T + t * 128)) == st["idxv"]
            for k in range(HD // 128):
                ks = slice(c * HD + k * 128, c * HD + (k + 1) * 128)
                xb = _ld(x_v[i], t * 128, (t + 1) * 128, ks).astype(f32)
                b = xb + (xb * 0.0 + jnp.where(hit, yrow[:, ks], 0.0))
                res = (gate * a[:, k * 128:(k + 1) * 128] + omg * b).astype(bf16)
                if i:
                    _st(out_v[i - 1], t * 128, (t + 1) * 128, ks, res)
                else:
                    _st(out0_v[t][c], 0, 128, slice(k * 128, (k + 1) * 128), res)
            if i == 0:
                c_o0[t, c].start()

        m5 = m(4)
        late()
        m3 = m(2)
        m2 = m(1)
        mix(0, 1, m3 + m5)
        m4 = m(3)
        o_next = None if nxt is None else attn(nxt)
        m1 = m(0)
        mix(1, 0, m2 + m4)
        c11 = m1 + m4 - m5
        c22 = m1 - m2 + m3
        c11 = c11 + m(6)
        m6 = m(5)
        mix(0, 0, c11)

        def last():
            mix(1, 1, c22 + m6)
            if i:
                c_o[i - 1].start()

        st["late"] = last
        return o_next

    order = list(range(1, NC)) + [0]
    o = attn(order[0])
    for n, i in enumerate(order):
        o = finish(i, o, order[n + 1] if n + 1 < NC else None)
    late()
    for d in c_o + list(c_o0.values()):
        d.wait()


@jax.jit
def pallas_gated_mix__linear_kernel_hedgehog__moe_arch_mod__prompt_kernel(
        A_x, A_wqkv, A_w_phi, A_wo, B_x, B_w_r, B_w_gate, B_w_up, B_w_down, gate_w):
    anyspec = pl.BlockSpec(memory_space=pl.ANY)
    V = pltpu.VMEM
    B = lambda r, c: V((r, c), bf16)
    P = lambda r, c: V((r // 2, c), u32)
    out = pl.pallas_call(
        _kernel,
        out_shape=jax.ShapeDtypeStruct((S, D), bf16),
        in_specs=[anyspec] * 9,
        out_specs=anyspec,
        scratch_shapes=[
            [B(T, D) for _ in range(NC)],
            [[B(D, 128) for _ in range(NG)] for _ in range(3)],
            V((D, DH), bf16), B(D, D), V((D,), bf16), V((D,), bf16),
            [B(D, FC) for _ in range(NF)], [B(D, FC) for _ in range(NF)], [B(FC, D) for _ in range(NF)],
            [[P(128, HD) for _ in range(7)] for _ in range(NP)],
            [[P(256, HD) for _ in range(7)] for _ in range(NP)],
            [P(7 * 128, HD) for _ in range(NC)], P(7 * HD, HD),
            [P(2 * D, T) for _ in range(NC)],
            V((2 * NG, 72, 128), f32), P(2 * NG * 64, 128), V((2 * NG, 128, 128), f32),
            [B(T, D) for _ in range(NC - 1)], [[B(128, HD) for _ in range(2)] for _ in range(2)],
            V((D, 128), f32), V((NC, T, 128), f32), P(NG * 128, 128), V((16, D), f32), V((NB, 8, 128), f32),
            pltpu.SemaphoreType.DMA((10,)),
        ],
        compiler_params=pltpu.CompilerParams(vmem_limit_bytes=120 * 2**20),
    )(A_x.reshape(S, D), A_wqkv, A_w_phi.reshape(D, DH), A_wo,
      B_w_r, B_w_gate, B_w_up, B_w_down, gate_w)
    return out.reshape(1, S, D)
```

```python
import functools

import jax
import jax.numpy as jnp
from jax import lax
import jax.experimental.pallas as pl
import jax.experimental.pallas.tpu as pltpu

S, D, DH, F = 2048, 1024, 32, 3584
T = 256
NC = S // T
NG = 8
NP = NG // 2
HD = D // 2
FC = 512
NF = F // FC
NB = F // 128
NDOT = 28 * NC + 14
LAG = 5
SEL, SEL_LAG = 105, 6
GU0 = 2
GU1 = 113
W1, W2 = 147, 193
f32, bf16, u32 = jnp.float32, jnp.bfloat16, jnp.uint32
NT = (((1,), (1,)), ((), ()))
LOG2E = 1.4426950408889634
ALL = slice(None)


def _ld(ref, r0, r1, cols=ALL):
    if ref.dtype == bf16:
        return ref[r0:r1, cols]
    return pltpu.bitcast(ref[r0 // 2:r1 // 2, cols], bf16)


def _st(ref, r0, r1, cols, val):
    if ref.dtype == bf16:
        ref[r0:r1, cols] = val
    else:
        ref[r0 // 2:r1 // 2, cols] = pltpu.bitcast(val, u32)


def _rcp(x):
    r = pl.reciprocal(x, approx=True)
    return r * (2.0 - x * r)


def _heads(v, op):
    r = v[0]
    for j in range(1, v.shape[0]):
        r = op(r, v[j])
    r = op(r, pltpu.roll(r, 4, 0))
    return op(r, pltpu.roll(r, 2, 0))


def _feat(p):
    outs = []
    for h in range(2):
        ph = p[h * 64:(h + 1) * 64].reshape(8, 8, p.shape[1])
        e1 = jnp.exp2(ph - _heads(ph, jnp.maximum)[None])
        e2 = jnp.exp2(_heads(ph, jnp.minimum)[None] - ph)
        for e in (e1, e2):
            outs.append((e * _rcp(_heads(e, jnp.add))[None]).reshape(64, p.shape[1]))
    return jnp.concatenate(outs, axis=0)


def _left(a11, a12, a21, a22):
    return (a11 + a22, a21 + a22, a11, a22, a11 + a12, a21 - a11, a12 - a22)


def _right(k, b11, b12, b21, b22):
    if k == 1:
        return b11()
    if k == 4:
        return b22()
    p, q, sub = {0: (b11, b22, False), 2: (b12, b22, True), 3: (b21, b11, True),
                 5: (b11, b12, False), 6: (b21, b22, False)}[k]
    p, q = p().astype(f32), q().astype(f32)
    return (p - q if sub else p + q).astype(bf16)


def _kernel(x_hbm, wqkv_hbm, wphi_hbm, wo_hbm, wr_hbm, wg_hbm, wu_hbm, wd_hbm, gw_hbm,
            out_hbm,
            x_v, wraw_v, wphi_v, wo_v, wr_v, gw_v, wg_v, wu_v, wd_v,
            sq_v, skv_v, xt_v, wot_v, phiq_v, acc_v, kvz_v, zc_v, out_v, out0_v, xcol_v, gate_v, bd_v, rg_v, h_v,
            sems):
    cp = pltpu.make_async_copy
    c_wphi = cp(wphi_hbm, wphi_v, sems.at[0])
    c_wr = cp(wr_hbm, wr_v, sems.at[9])
    c_gw = cp(gw_hbm, gw_v, sems.at[9])
    wsem = lambda j, g: 1 + g // 2 if j else (5, 9)[g // 4]
    c_w = [[cp(wqkv_hbm.at[:, pl.ds(j * D + g * 128, 128)], wraw_v[j][g], sems.at[wsem(j, g)])
            for g in range(NG)] for j in range(3)]
    c_x = [cp(x_hbm.at[pl.ds(i * T, T)], x_v[i], sems.at[(1, 5, 9, 6)[min(i, 3)]])
           for i in range(NC)]
    c_gu = [cp(w.at[:, pl.ds(j * FC, FC)], v[j], sems.at[6 if j < GU0 else 7])
            for j in range(NF) for w, v in ((wg_hbm, wg_v), (wu_hbm, wu_v))]
    c_d = [cp(wd_hbm.at[pl.ds(j * FC, FC)], wd_v[j], sems.at[8]) for j in range(NF)]
    c_d.append(cp(wo_hbm, wo_v, sems.at[8]))
    c_o = [cp(out_v[i - 1], out_hbm.at[pl.ds(i * T, T)], sems.at[2]) for i in range(1, NC)]
    c_o0 = {(t, c): cp(out0_v[t][c], out_hbm.at[pl.ds(t * 128, 128), pl.ds(c * HD, HD)], sems.at[2])
            for t in range(2) for c in range(2)}

    for d in [c_wphi, c_w[1][0], c_w[1][1], c_w[2][0], c_w[2][1], c_x[0]]:
        d.start()
    for g in range(2, NG):
        c_w[1][g].start()
        c_w[2][g].start()
    for d in [c_x[1]] + c_w[0][:4] + [c_wr, c_gw] + c_w[0][4:] + c_x[2:] + c_gu + c_d:
        d.start()

    row = lax.broadcasted_iota(jnp.int32, (128, 128), 0)
    col = lax.broadcasted_iota(jnp.int32, (128, 128), 1)
    diag = (row // DH) == (col // 64) * 2 + col % 2
    rep = (((lax.broadcasted_iota(jnp.int32, (DH, 128), 1) % 64) // 2)
           == lax.broadcasted_iota(jnp.int32, (DH, 128), 0)).astype(bf16)
    acc_v[...] = jnp.zeros_like(acc_v)
    ones = jnp.ones((8, T), f32)
    c_wphi.wait()
    for g in range(NG):
        wt = jnp.dot(wphi_v[g * 128:(g + 1) * 128, :], rep, preferred_element_type=f32)
        _st(bd_v, g * 128, (g + 1) * 128, ALL, jnp.where(diag, wt, 0.0).T.astype(bf16))

    def prep(j, pp):
        w = []
        for g in (2 * pp, 2 * pp + 1):
            raw = _ld(wraw_v[j][g], 0, D)
            if j < 2:
                w.append(lax.dot_general(_ld(bd_v, g * 128, (g + 1) * 128), raw, NT,
                                         preferred_element_type=f32) * LOG2E)
            else:
                w.append(raw.T.astype(f32))
        dst, r0 = (sq_v, 0) if j == 0 else (skv_v, (j - 1) * 128)
        for k, s in enumerate(_left(w[0][:, :HD], w[0][:, HD:], w[1][:, :HD], w[1][:, HD:])):
            _st(dst[pp][k], r0, r0 + 128, ALL, s.astype(bf16))

    st = {"n": 0}

    def tie(a, dep):
        if dep is None:
            return a
        if a.dtype == f32:
            blk = jnp.where(st["never"], dep, a[0:8])
            return jnp.concatenate([blk, a[8:]], axis=0) if a.shape[0] > 8 else blk
        blk = pltpu.bitcast(jnp.where(st["never"], dep, pltpu.bitcast(a[0:16, 0:128], f32)), bf16)
        if a.shape[1] > 128:
            blk = jnp.concatenate([blk, a[0:16, 128:]], axis=1)
        return jnp.concatenate([blk, a[16:]], axis=0)

    def xright(i, k, fresh):
        blk = lambda r, c: (lambda: _ld(x_v[i], r * 128, (r + 1) * 128, slice(c * HD, (c + 1) * HD)))
        if k in (1, 4) or fresh:
            val = _right(k, blk(0, 0), blk(1, 0), blk(0, 1), blk(1, 1))
            if k not in (1, 4):
                _st(xt_v[i], k * 128, (k + 1) * 128, ALL, val)
            return val
        return _ld(xt_v[i], k * 128, (k + 1) * 128)

    jobs = {}
    after = {}
    ties = {}

    def project(lhs, i, fresh, use, mid):
        def m(k):
            n = st["n"]
            st["n"] = n + 1
            out = lax.dot_general(tie(lhs(k), ties.pop(n, None)), xright(i, k, fresh), NT,
                                  preferred_element_type=f32)
            if n in after:
                after.pop(n)()
            if n in jobs:
                res = jobs.pop(n)(out[0:8])
                lag = SEL_LAG if n == SEL else LAG
                if n + lag < NDOT:
                    assert n + lag not in ties
                    ties[n + lag] = res
            return out
        m5 = m(4)
        m3 = m(2)
        late()
        m2 = m(1)
        use(0, 1, m3 + m5)
        mid()
        m4 = m(3)
        m1 = m(0)
        use(1, 0, m2 + m4)
        c11 = m1 + m4 - m5
        c22 = m1 - m2 + m3
        c11 = c11 + m(6)
        m6 = m(5)
        use(0, 0, c11)
        st["late"] = lambda: use(1, 1, c22 + m6)

    def late():
        st.pop("late", lambda: None)()

    pend = []

    def kv_flush():
        for g, fk, vt in pend:
            fk = jnp.concatenate(fk, axis=1)
            vt = jnp.concatenate(vt, axis=1)
            for p in range(2):
                lhs = jnp.concatenate([vt[p * 64:(p + 1) * 64], ones], axis=0)
                acc_v[2 * g + p] += lax.dot_general(lhs, fk[p * 128:(p + 1) * 128], NT,
                                                    preferred_element_type=f32)
        pend.clear()

    def router(i, part, dep):
        best, bidx = st["best"], st["bidx"]
        for b in range(part * 4, part * 4 + 4):
            rows = slice(b * 16, (b + 1) * 16)
            xf = [_ld(x_v[i], b * 16, (b + 1) * 16, slice(k * 128, (k + 1) * 128)).astype(f32)
                  for k in range(D // 128)]
            acc = []
            for w in range(2):
                for hf in range(2):
                    a = None
                    for k in range(D // 128):
                        p = xf[k][hf * 8:(hf + 1) * 8] * rg_v[w * 8:(w + 1) * 8, k * 128:(k + 1) * 128]
                        a = tie(p, dep) if k == 0 else a + p
                    acc.append(a)
                    dep = a
            ra, ga = jnp.concatenate(acc[0:2], axis=0), jnp.concatenate(acc[2:4], axis=0)
            r = jnp.sum(ra, axis=1, keepdims=True).astype(bf16).astype(f32)
            gate_v[i, rows, :] = jnp.broadcast_to(jnp.sum(ga, axis=1, keepdims=True), (16, 128))
            r = jnp.broadcast_to(r, (16, 128))
            for k in range(2):
                rk = r[k * 8:(k + 1) * 8]
                if best is None:
                    best, bidx = rk, jnp.zeros((8, 128), jnp.int32)
                else:
                    better = rk > best
                    best = jnp.where(better, rk, best)
                    bidx = jnp.where(better, i * T + b * 16 + k * 8, bidx)
        st["best"], st["bidx"] = best, bidx
        return dep

    def select():
        best, bidx = st["best"], st["bidx"]
        m = jnp.max(best, axis=0, keepdims=True)
        cand = jnp.where(best == m, bidx + lax.broadcasted_iota(jnp.int32, (8, 128), 0), S)
        idxv = jnp.min(cand, axis=0, keepdims=True) & (S - 1)
        idx = idxv[0, 0]
        st["idxv"] = idxv
        st["rs"] = jax.nn.sigmoid(m)
        base = pl.multiple_of(((idx % T) // 16) * 16, 16)
        tile = x_v[0][pl.ds(base, 16), :].astype(f32)
        for i in range(1, NC):
            tile = jnp.where(idx // T == i, x_v[i][pl.ds(base, 16), :].astype(f32), tile)
        sel = lax.broadcasted_iota(jnp.int32, (16, D), 0) == (idx % 16)
        xs = jnp.sum(jnp.where(sel, tile, 0.0), axis=0, keepdims=True)
        for k in range(D // 128):
            xc = jnp.broadcast_to(xs[:, k * 128:(k + 1) * 128], (128, 128)).T
            xcol_v[k * 128:(k + 1) * 128, :] = xc
            best = jnp.maximum(best, xc[120:128])
        st["y"] = [None] * (D // 128)
        return best

    def chain(w_ref, r0, nblk, cols, col_of, dep):
        acc = None
        for k in range(nblk):
            p = _ld(w_ref, r0 + k * 16, r0 + (k + 1) * 16, cols).astype(f32) * col_of(k)
            acc = tie(p[0:8], dep) if acc is None else acc + p[0:8]
            acc = acc + p[8:16]
        return acc

    def ffn_in(w, c, dep):
        j, cc = divmod(c, FC // 128)
        acc = chain((wg_v, wu_v)[w][j], 0, D // 16, slice(cc * 128, (cc + 1) * 128),
                    lambda k: xcol_v[k * 16:(k + 1) * 16, :], dep)
        v = jnp.sum(acc, axis=0, keepdims=True)
        if w == 0:
            st["g", c] = v * jax.nn.sigmoid(v)
        else:
            h_v[c] = jnp.broadcast_to(st.pop(("g", c)) * v, (8, 128))
        return acc

    def ffn_down(c, dep):
        j, cc = divmod(c, FC // 128)
        hcol = jnp.concatenate([h_v[c]] * 16, axis=0).T
        ys = st["y"]
        for n in range(D // 128):
            dep = chain(wd_v[j], cc * 128, 128 // 16, slice(n * 128, (n + 1) * 128),
                        lambda k: hcol[k * 16:(k + 1) * 16], dep)
            ys[n] = dep if ys[n] is None else ys[n] + dep
        return dep

    def wo_job(r, e, dep):
        def blk(a, b):
            r0, c0 = b * HD + e * 128, a * HD + r * 128
            return _ld(wo_v, r0, r0 + 128, slice(c0, c0 + 128)).T.astype(f32)
        for k, v in enumerate(_left(blk(0, 0), blk(0, 1), blk(1, 0), blk(1, 1))):
            _st(wot_v, k * HD + r * 128, k * HD + (r + 1) * 128, slice(e * 128, (e + 1) * 128), v.astype(bf16))
            dep = jnp.maximum(dep, v[120:128])
        return dep

    def wait_kv(pp):
        for g in (2 * pp, 2 * pp + 1):
            c_w[1][g].wait()
            c_w[2][g].wait()
        if pp == 0:
            c_x[0].wait()
        prep(1, pp)
        prep(2, pp)

    def wait_q(half):
        for d in [c_x[1 + half]] + c_w[0][4 * half:4 * half + 4] + [c_wr, c_gw][:2 * half]:
            d.wait()
        prep(0, 2 * half)
        if half:
            wr = wr_v[...].reshape(1, D).astype(f32)
            rg_v[0:8, :] = jnp.broadcast_to(wr, (8, D))
            rg_v[8:16, :] = jnp.broadcast_to(gw_v[...].reshape(1, D).astype(f32), (8, D))
            st["best"] = st["bidx"] = None
            st["never"] = jnp.broadcast_to((pltpu.bitcast(wr[:, 0:128], jnp.int32) | 1) == 0, (8, 128))

    def wait_all(ds):
        for d in ds:
            d.wait()

    for pp in range(1, NP):
        after[7 * pp - 1] = functools.partial(wait_kv, pp)
    after[25] = functools.partial(wait_q, 0)
    after[32] = functools.partial(prep, 0, 1)
    after[39] = functools.partial(wait_q, 1)
    after[46] = functools.partial(prep, 0, 3)
    after[83] = functools.partial(wait_all, c_x[3:] + c_gu[:2 * GU0])
    for r in range(4 * NC):
        jobs[56 + 2 * r if r < 12 else 72 + r] = functools.partial(router, r // 4, r % 4)
    jobs[SEL] = lambda dep: select()
    n0 = 8 * GU0
    for u in range(2 * NB):
        pos = GU1 + (u * (W1 - LAG - GU1)) // n0 if u < n0 else W1 + 1 + ((u - n0) * (W2 - LAG - W1)) // (2 * NB - n0)
        assert pos not in jobs
        jobs[pos] = functools.partial(ffn_in, u % 2, u // 2)
    after[W1] = functools.partial(wait_all, c_gu[2 * GU0:])
    after[W2] = functools.partial(wait_all, c_d)
    tail = sorted([(c / NB, functools.partial(ffn_down, c)) for c in range(NB)]
                  + [((w + 0.5) / 16, functools.partial(wo_job, w // 4, w % 4)) for w in range(16)], key=lambda e: e[0])
    for pos, (_, job) in enumerate(tail):
        jobs[W2 + 1 + pos] = job

    wait_kv(0)
    for i, pp in [(i, pp) for i in range(NC) for pp in range(NP)]:
        new = [(2 * pp + a, [None, None], [None, None]) for a in range(2)]

        def use(a, t, c, new=new, i=i, pp=pp):
            g = 2 * pp + a
            if i >= 1:
                _st(phiq_v[i], g * 256, (g + 1) * 256, slice(t * 128, (t + 1) * 128), _feat(c[0:128]).astype(bf16))
            new[a][1][t] = _feat(c[-256:-128]).astype(bf16)
            new[a][2][t] = c[-128:]

        def lhs(k, i=i, pp=pp):
            kvw = _ld(skv_v[pp][k], 0, 256)
            return jnp.concatenate([_ld(sq_v[pp][k], 0, 128), kvw], axis=0) if i >= 1 else kvw

        project(lhs, i, pp == 0, use, kv_flush)
        pend.extend(new)

    def finalize():
        if pend:
            kv_flush()
            keep = (lax.broadcasted_iota(jnp.int32, (64, 128), 0) // 32
                    == lax.broadcasted_iota(jnp.int32, (64, 128), 1) % 2)
            for p in range(2 * NG):
                _st(kvz_v, p * 64, (p + 1) * 64, ALL, jnp.where(keep, acc_v[p, 0:64], 0.0).astype(bf16))
                zc_v[p] = jnp.concatenate([acc_v[p, 64:72]] * 16, axis=0).T

    for q in range(NP // 2):
        def use(a, t, c, q=q):
            for e in range(2):
                g = 2 * (2 * q + e) + a
                _st(phiq_v[0], g * 256, (g + 1) * 256, slice(t * 128, (t + 1) * 128),
                    _feat(c[e * 128:(e + 1) * 128]).astype(bf16))

        project(lambda k, q=q: jnp.concatenate([_ld(sq_v[2 * q][k], 0, 128), _ld(sq_v[2 * q + 1][k], 0, 128)], axis=0),
                0, False, use, finalize)

    late()
    yrow = jnp.concatenate([jnp.sum(y, axis=0, keepdims=True) * st["rs"] for y in st["y"]], axis=1)

    parity = lax.broadcasted_iota(jnp.int32, (8, T), 0) % 2

    def attn(i):
        ot = []
        for p in range(2 * NG):
            phi = _ld(phiq_v[i], p * 128, (p + 1) * 128)
            num = jnp.dot(_ld(kvz_v, p * 64, (p + 1) * 64), phi, preferred_element_type=f32)
            zc = zc_v[p]
            pz = (phi.astype(f32) * jnp.concatenate([zc] * (T // 128), axis=1)).reshape(16, 8, T)
            rden = _rcp(_heads(pz, jnp.add) + 1e-6)
            swapped = pltpu.roll(rden, 1, 0)
            for a in range(2):
                r = jnp.where(parity == a, rden, swapped)
                ot.append((num[32 * a:32 * a + 32].reshape(4, 8, T) * r[None]).reshape(32, T))
        ot = jnp.concatenate(ot, axis=0)
        b11, b12, b21, b22 = ot[:HD, :128], ot[:HD, 128:], ot[HD:, :128], ot[HD:, 128:]
        return [s.astype(bf16) for s in (b11 + b22, b11, b12 - b22, b21 - b11, b22, b11 + b12, b21 + b22)]

    def finish(i, o, nxt):
        def m(k):
            return jnp.dot(_ld(wot_v, k * HD, (k + 1) * HD), o[k], preferred_element_type=f32)

        def mix(c, t, a):
            a = a.T
            rows = slice(t * 128, (t + 1) * 128)
            gate = jax.nn.sigmoid(gate_v[i, rows, :])
            omg = 1.0 - gate
            hit = (lax.broadcasted_iota(jnp.int32, (128, 128), 0) + (i * T + t * 128)) == st["idxv"]
            for k in range(HD // 128):
                ks = slice(c * HD + k * 128, c * HD + (k + 1) * 128)
                xb = _ld(x_v[i], t * 128, (t + 1) * 128, ks).astype(f32)
                b = xb + (xb * 0.0 + jnp.where(hit, yrow[:, ks], 0.0))
                res = (gate * a[:, k * 128:(k + 1) * 128] + omg * b).astype(bf16)
                if i:
                    _st(out_v[i - 1], t * 128, (t + 1) * 128, ks, res)
                else:
                    _st(out0_v[t][c], 0, 128, slice(k * 128, (k + 1) * 128), res)
            if i == 0:
                c_o0[t, c].start()

        m5 = m(4)
        late()
        m3 = m(2)
        m2 = m(1)
        mix(0, 1, m3 + m5)
        o_next = None if nxt is None else attn(nxt)
        m4 = m(3)
        m1 = m(0)
        mix(1, 0, m2 + m4)
        c11 = m1 + m4 - m5
        c22 = m1 - m2 + m3
        c11 = c11 + m(6)
        m6 = m(5)
        mix(0, 0, c11)

        def last():
            mix(1, 1, c22 + m6)
            if i:
                c_o[i - 1].start()

        st["late"] = last
        return o_next

    order = list(range(1, NC)) + [0]
    o = attn(order[0])
    for n, i in enumerate(order):
        o = finish(i, o, order[n + 1] if n + 1 < NC else None)
    late()
    for d in c_o + list(c_o0.values()):
        d.wait()


@jax.jit
def pallas_gated_mix__linear_kernel_hedgehog__moe_arch_mod__prompt_kernel(
        A_x, A_wqkv, A_w_phi, A_wo, B_x, B_w_r, B_w_gate, B_w_up, B_w_down, gate_w):
    anyspec = pl.BlockSpec(memory_space=pl.ANY)
    V = pltpu.VMEM
    B = lambda r, c: V((r, c), bf16)
    P = lambda r, c: V((r // 2, c), u32)
    out = pl.pallas_call(
        _kernel,
        out_shape=jax.ShapeDtypeStruct((S, D), bf16),
        in_specs=[anyspec] * 9,
        out_specs=anyspec,
        scratch_shapes=[
            [B(T, D) for _ in range(NC)],
            [[B(D, 128) for _ in range(NG)] for _ in range(3)],
            V((D, DH), bf16), B(D, D), V((D,), bf16), V((D,), bf16),
            [B(D, FC) for _ in range(NF)], [B(D, FC) for _ in range(NF)], [B(FC, D) for _ in range(NF)],
            [[P(128, HD) for _ in range(7)] for _ in range(NP)],
            [[P(256, HD) for _ in range(7)] for _ in range(NP)],
            [P(7 * 128, HD) for _ in range(NC)], P(7 * HD, HD),
            [P(2 * D, T) for _ in range(NC)],
            V((2 * NG, 72, 128), f32), P(2 * NG * 64, 128), V((2 * NG, 128, 128), f32),
            [B(T, D) for _ in range(NC - 1)], [[B(128, HD) for _ in range(2)] for _ in range(2)],
            V((D, 128), f32), V((NC, T, 128), f32), P(NG * 128, 128), V((16, D), f32), V((NB, 8, 128), f32),
            pltpu.SemaphoreType.DMA((10,)),
        ],
        compiler_params=pltpu.CompilerParams(vmem_limit_bytes=120 * 2**20),
    )(A_x.reshape(S, D), A_wqkv, A_w_phi.reshape(D, DH), A_wo,
      B_w_r, B_w_gate, B_w_up, B_w_down, gate_w)
    return out.reshape(1, S, D)
```
